```python
import jax
import jax.numpy as jnp

def _softmax(x, axis=-1):
    return jax.nn.softmax(x, axis=axis)

def _gelu(x):
    return jax.nn.gelu(x, approximate=True)

def _silu(x):
    return jax.nn.silu(x)

def _sigmoid(x):
    return jax.nn.sigmoid(x)

def _layernorm(x, axis=-1, eps=1e-05):
    m = jnp.mean(x, axis=axis, keepdims=True)
    v = jnp.var(x, axis=axis, keepdims=True)
    return (x - m) / jnp.sqrt(v + eps)

def _scatter_add(tgt, idx, src, axis=0):
    return tgt.at[idx].add(src)

def _segment_sum(src, seg, n):
    return jax.ops.segment_sum(src, seg, n)

class _Rng:

    def __init__(self, key):
        self._k = key

    def _next(self):
        self._k, sub = jax.random.split(self._k)
        return sub

    def normal(self, shape):
        return jax.random.normal(self._next(), shape, dtype=jnp.bfloat16)

    def randint(self, lo, hi, shape):
        return jax.random.randint(self._next(), shape, lo, hi, dtype=jnp.int32)

    def uniform(self, shape, lo=0.0, hi=1.0):
        return jax.random.uniform(self._next(), shape, jnp.bfloat16, lo, hi)

    def permutation(self, n):
        return jax.random.permutation(self._next(), n)
kernel_name = 'parallel_sum__memory_aug_recurrent_mem_tr__mixer_s_mlp__prompt'

def setup_inputs():
    _rng = _Rng(jax.random.key(int.from_bytes(__import__("os").urandom(4), "little")))
    _w = lambda a: (lambda t: t.astype(jnp.bfloat16) if jnp.issubdtype(t.dtype, jnp.floating) else t)(jnp.asarray(a))

    def _A_setup():
        B, S, Dm = (1, 2048, 1024)
        H, Dh = (32, 128)
        M, seg = (8, 32)
        seg = min(seg, S)
        S = S // seg * seg
        return {'x': _w((lambda *s: _rng.normal(s) * 0.05)(B, S, Dm)), 'mem0': _w((lambda *s: _rng.normal(s) * 0.05)(B, M, Dm)), 'Wq': _w((lambda *s: _rng.normal(s) * 0.05)(Dm, H, Dh) * Dm ** (-0.5)), 'Wk': _w((lambda *s: _rng.normal(s) * 0.05)(Dm, H, Dh) * Dm ** (-0.5)), 'Wv': _w((lambda *s: _rng.normal(s) * 0.05)(Dm, H, Dh) * Dm ** (-0.5)), 'Wo': _w((lambda *s: _rng.normal(s) * 0.05)(H, Dh, Dm) * (H * Dh) ** (-0.5)), 'seg_len': seg}
    _A_in = _A_setup()

    def _B_setup():
        B, S, D, F = (1, 2048, 1024, 3584)
        return {'x': _w((lambda *s: _rng.normal(s) * 0.05)(B, S, D)), 'w1': _w((lambda *s: _rng.normal(s) * 0.05)(D, D) * D ** (-0.5)), 'w2': _w((lambda *s: _rng.normal(s) * 0.05)(D, D) * D ** (-0.5)), 'w3': _w((lambda *s: _rng.normal(s) * 0.05)(D, F) * D ** (-0.5)), 'w4': _w((lambda *s: _rng.normal(s) * 0.05)(F, D) * F ** (-0.5))}
    _B_in = _B_setup()
    return {'A_x': _A_in['x'], 'A_mem0': _A_in['mem0'], 'A_Wq': _A_in['Wq'], 'A_Wk': _A_in['Wk'], 'A_Wv': _A_in['Wv'], 'A_Wo': _A_in['Wo'], 'A_seg_len': _A_in['seg_len'], 'B_x': _B_in['x'], 'B_w1': _B_in['w1'], 'B_w2': _B_in['w2'], 'B_w3': _B_in['w3'], 'B_w4': _B_in['w4']}

def reference(A_x, A_mem0, A_Wq, A_Wk, A_Wv, A_Wo, A_seg_len, B_x, B_w1, B_w2, B_w3, B_w4):

    def _A_ref(x, mem0, Wq, Wk, Wv, Wo, seg_len):
        B, S, Dm = x.shape
        H, Dh = (Wq.shape[1], Wq.shape[2])
        M = mem0.shape[1]
        scale = Dh ** (-0.5)
        n_seg = S // seg_len
        L = M + seg_len
        idx = jnp.arange(L)
        mask = (idx[:, None] < M) | (idx[:, None] >= idx[None, :])
        mem = mem0
        outs = []
        for s in range(n_seg):
            xs = x[:, s * seg_len:(s + 1) * seg_len, :].copy()
            h = jnp.concatenate([mem, xs], axis=1)
            q = jnp.einsum('btd,dhe->bhte', h, Wq)
            k = jnp.einsum('btd,dhe->bhte', h, Wk)
            v = jnp.einsum('btd,dhe->bhte', h, Wv)
            scores = jnp.einsum('bhqe,bhke->bhqk', q, k) * scale
            scores = jnp.where(mask[None, None], scores, -1000000000.0)
            p = _softmax(scores, axis=-1)
            o = jnp.einsum('bhqk,bhke->bhqe', p, v)
            o = jnp.einsum('bhte,hed->btd', o, Wo)
            mem = o[:, :M, :].copy()
            outs.append(o[:, M:, :])
        return jnp.concatenate(outs, axis=1)

    def _B_ref(x, w1, w2, w3, w4):
        B, S, D = x.shape
        h = _gelu(_layernorm(x, axis=-1) @ w1)
        c = D // 4
        g0 = jnp.pad(h[:, :, 0 * c:1 * c], ((0, 0), (1, 0), (0, 0)))[:, :S, :]
        g1 = jnp.pad(h[:, :, 1 * c:2 * c], ((0, 0), (0, 1), (0, 0)))[:, 1:, :]
        g2 = jnp.pad(h[:, :, 2 * c:3 * c], ((0, 0), (2, 0), (0, 0)))[:, :S, :]
        g3 = jnp.pad(h[:, :, 3 * c:], ((0, 0), (0, 2), (0, 0)))[:, 2:, :]
        hs = jnp.concatenate([g0, g1, g2, g3], axis=-1) @ w2
        x1 = x + hs
        h2 = _gelu(_layernorm(x1, axis=-1) @ w3) @ w4
        return x1 + h2
    x = A_x
    xn = _layernorm(x, axis=-1)
    return x + _A_ref(xn, A_mem0, A_Wq, A_Wk, A_Wv, A_Wo, A_seg_len) + _B_ref(xn, B_w1, B_w2, B_w3, B_w4)
```

```python
import functools

import jax
import jax.numpy as jnp
import numpy as np
from jax import lax
import jax.experimental.pallas as pl
import jax.experimental.pallas.tpu as pltpu

_F32 = jnp.float32
_BF16 = jnp.bfloat16
_U32 = jnp.uint32

_TM = 256
_FC = 512
_HG = 4
_PAD = 8


def _layernorm(x, eps=1e-5):
    m = jnp.mean(x, axis=-1, keepdims=True)
    c = x - m
    v = jnp.mean(c * c, axis=-1, keepdims=True)
    return c * lax.rsqrt(v + eps)


def _gelu(x):
    c0 = float(np.sqrt(2.0 / np.pi))
    c1 = c0 * 0.044715
    hx = 0.5 * x
    return hx + hx * jnp.tanh(x * (c0 + c1 * (x * x)))


def _dot(a, b):
    return lax.dot_general(a, b, (((1,), (0,)), ((), ())), preferred_element_type=_F32)


def _dot_nt(a, b):
    return lax.dot_general(a, b, (((1,), (1,)), ((), ())), preferred_element_type=_F32)


def _kernel(x_hbm, mem0_ref, wq_hbm, wk_hbm, wv_hbm, wo_hbm, w1_hbm, w2_hbm, w3_hbm, w4_hbm,
            out_hbm,
            x_v, w1_v, w2_v, w3_v, w4_v, stage_v, wqkv_v, wo_v, xn_v, h_v, base_v, att_v,
            sem_x, sem_w, sem_s, sem_o, sem_out, *, seg):
    S, D = x_v.shape
    F = w3_v.shape[1]
    n_mem = mem0_ref.shape[0]
    H = wqkv_v.shape[0] // 3
    E = wqkv_v.shape[2]
    nblk = S // _TM
    dch = D // nblk
    n_wo = D // 128

    def x_copy(i):
        rows = pl.ds(pl.multiple_of(i * _TM, _TM), _TM)
        return pltpu.make_async_copy(x_hbm.at[rows], x_v.at[rows], sem_x.at[i])

    def stage_copy(t, i):
        src = (wq_hbm, wk_hbm, wv_hbm)[t]
        rows = pl.ds(pl.multiple_of(i * (dch * H), dch * H), dch * H)
        return pltpu.make_async_copy(src.at[rows], stage_v.at[t, rows], sem_s.at[t, i])

    def wo_copy(j):
        return pltpu.make_async_copy(wo_hbm.at[:, pl.ds(j * 128, 128)], wo_v.at[j], sem_o.at[j])

    w_copies = [pltpu.make_async_copy(src, dst, sem_w.at[n]) for n, (src, dst) in enumerate(
        ((w1_hbm, w1_v), (w2_hbm, w2_v), (w3_hbm, w3_v), (w4_hbm, w4_v)))]

    x_copy(0).start()
    w_copies[0].start()
    for i in range(1, nblk):
        x_copy(i).start()
    for cp in w_copies[1:]:
        cp.start()
    for i in range(nblk):
        for t in range(3):
            stage_copy(t, i).start()
    for j in range(n_wo):
        wo_copy(j).start()

    h_v[pl.ds(0, _PAD), :] = jnp.zeros((_PAD, D), _F32)
    h_v[pl.ds(_PAD + S, _PAD), :] = jnp.zeros((_PAD, D), _F32)
    w_copies[0].wait()

    def b1(i, _):
        x_copy(i).wait()
        r0 = pl.multiple_of(i * _TM, _TM)
        xn = _layernorm(x_v[pl.ds(r0, _TM), :].astype(_F32))
        xn_v[pl.ds(r0, _TM), :] = xn
        y = _layernorm(xn).astype(_BF16)
        h_v[pl.ds(pl.multiple_of(r0 + _PAD, _PAD), _TM), :] = _gelu(_dot(y, w1_v[...]))
        return 0

    lax.fori_loop(0, nblk, b1, 0)

    for cp in w_copies[1:]:
        cp.wait()
    cq = D // 4

    def b2(i, _):
        for t in range(3):
            stage_copy(t, i).wait()
        r0 = pl.multiple_of(i * _TM, _TM)
        parts = []
        for n, sh in enumerate((-1, 1, -2, 2)):
            win = h_v[pl.ds(r0, _TM + 2 * _PAD), pl.ds(n * cq, cq)]
            parts.append(win[_PAD + sh:_PAD + sh + _TM].astype(_BF16))
        g = jnp.concatenate(parts, axis=1)
        x1 = xn_v[pl.ds(r0, _TM), :] + _dot(g, w2_v[...])
        y = _layernorm(x1).astype(_BF16)
        u = jnp.concatenate(
            [_gelu(_dot(y, w3_v[:, pl.ds(c * _FC, _FC)])).astype(_BF16) for c in range(F // _FC)],
            axis=1)
        base_v[pl.ds(r0, _TM), :] = (
            x_v[pl.ds(r0, _TM), :].astype(_F32) + x1 + _dot(u, w4_v[...]))

        s0 = pl.multiple_of(i * (dch * H), dch * H)
        o0 = pl.multiple_of(i * (dch // 2), dch // 2)
        for t in range(3):
            v = pltpu.bitcast(stage_v[t, pl.ds(s0, dch * H), :], _U32)
            v = jnp.swapaxes(v.reshape(dch // 2, H, E), 0, 1)
            for j in range(H // 2):
                a, b = v[j], v[H // 2 + j]
                wqkv_v[6 * j + t, pl.ds(o0, dch // 2), :] = (a & _U32(0xFFFF)) | (b << 16)
                wqkv_v[6 * j + 3 + t, pl.ds(o0, dch // 2), :] = (a >> 16) | (b & _U32(0xFFFF0000))
        return 0

    lax.fori_loop(0, nblk, b2, 0)

    for j in range(n_wo):
        wo_copy(j).wait()
    L = n_mem + seg
    row = lax.broadcasted_iota(jnp.int32, (L, L), 0)
    col = lax.broadcasted_iota(jnp.int32, (L, L), 1)
    mask = (row < n_mem) | (row >= col)
    scale = float(E) ** -0.5
    n_seg = S // seg

    def out_copy(s):
        rows = pl.ds(pl.multiple_of(s * seg, seg), seg)
        return pltpu.make_async_copy(x_v.at[rows], out_hbm.at[rows], sem_out.at[0])

    def step(s, mem):
        r0 = pl.multiple_of(s * seg, seg)
        hh = jnp.concatenate([mem, xn_v[pl.ds(r0, seg), :]], axis=0)
        ng = H // _HG
        qkv, sc = {}, {}
        for g in range(ng + 2):
            if g < ng:
                w = jnp.concatenate(
                    [pltpu.bitcast(wqkv_v[3 * _HG * g + n], _BF16) for n in range(3 * _HG)], axis=1)
                qkv[g] = _dot(hh, w)
            if 0 <= g - 1 < ng:
                y = qkv[g - 1]
                sc[g - 1] = [
                    _dot_nt(y[:, (3 * n) * E:(3 * n + 1) * E],
                            y[:, (3 * n + 1) * E:(3 * n + 2) * E].astype(_BF16))
                    for n in range(_HG)]
            if 0 <= g - 2 < ng:
                y = qkv[g - 2]
                for n in range(_HG):
                    z = jnp.where(mask, sc[g - 2][n] * scale, -1e9)
                    e = jnp.exp(z - jnp.max(z, axis=-1, keepdims=True))
                    r = 1.0 / jnp.sum(e, axis=-1, keepdims=True)
                    o = _dot(e, y[:, (3 * n + 2) * E:(3 * n + 3) * E].astype(_BF16)) * r
                    att_v[:, pl.ds(((g - 2) * _HG + n) * E, E)] = o
        wo = jnp.concatenate([wo_v[j] for j in range(n_wo)], axis=1)
        o = _dot(att_v[...], wo)
        x_v[pl.ds(r0, seg), :] = (base_v[pl.ds(r0, seg), :] + o[n_mem:]).astype(_BF16)
        out_copy(s).start()
        return o[:n_mem]

    lax.fori_loop(0, n_seg, step, mem0_ref[...].astype(_F32))
    pltpu.make_async_copy(x_v, out_hbm, sem_out.at[0]).wait()


@functools.partial(jax.jit, static_argnames=("A_seg_len",))
def pallas_parallel_sum__memory_aug_recurrent_mem_tr__mixer_s_mlp__prompt_kernel(
    A_x: jax.Array,
    A_mem0: jax.Array,
    A_Wq: jax.Array,
    A_Wk: jax.Array,
    A_Wv: jax.Array,
    A_Wo: jax.Array,
    A_seg_len: int,
    B_x: jax.Array,
    B_w1: jax.Array,
    B_w2: jax.Array,
    B_w3: jax.Array,
    B_w4: jax.Array,
):
    del B_x
    B, S, D = A_x.shape
    _, H, E = A_Wq.shape
    M = A_mem0.shape[1]
    F = B_w3.shape[1]
    seg = int(A_seg_len)
    assert B == 1 and S % _TM == 0 and S % seg == 0 and F % _FC == 0 and H % _HG == 0
    nblk = S // _TM

    hbm = pl.BlockSpec(memory_space=pltpu.HBM)
    out = pl.pallas_call(
        functools.partial(_kernel, seg=seg),
        out_shape=jax.ShapeDtypeStruct((S, D), A_x.dtype),
        in_specs=[hbm, pl.BlockSpec(memory_space=pltpu.VMEM)] + [hbm] * 8,
        out_specs=hbm,
        scratch_shapes=[
            pltpu.VMEM((S, D), _BF16),
            pltpu.VMEM((D, D), _BF16),
            pltpu.VMEM((D, D), _BF16),
            pltpu.VMEM((D, F), _BF16),
            pltpu.VMEM((F, D), _BF16),
            pltpu.VMEM((3, D * H, E), _BF16),
            pltpu.VMEM((3 * H, D // 2, E), _U32),
            pltpu.VMEM((D // 128, H * E, 128), _BF16),
            pltpu.VMEM((S, D), _F32),
            pltpu.VMEM((S + 2 * _PAD, D), _F32),
            pltpu.VMEM((S, D), _F32),
            pltpu.VMEM((M + seg, H * E), _F32),
            pltpu.SemaphoreType.DMA((nblk,)),
            pltpu.SemaphoreType.DMA((4,)),
            pltpu.SemaphoreType.DMA((3, nblk)),
            pltpu.SemaphoreType.DMA((D // 128,)),
            pltpu.SemaphoreType.DMA((1,)),
        ],
        compiler_params=pltpu.CompilerParams(vmem_limit_bytes=124 * 1024 * 1024),
    )(A_x.reshape(S, D), A_mem0.reshape(M, D),
      A_Wq.reshape(D * H, E), A_Wk.reshape(D * H, E), A_Wv.reshape(D * H, E),
      A_Wo.reshape(H * E, D), B_w1, B_w2, B_w3, B_w4)
    return out.reshape(B, S, D)
```

```python
import functools

import jax
import jax.numpy as jnp
import numpy as np
from jax import lax
import jax.experimental.pallas as pl
import jax.experimental.pallas.tpu as pltpu

_F32 = jnp.float32
_BF16 = jnp.bfloat16
_U32 = jnp.uint32

_TM = 256
_FC = 256
_HG = 4
_WO = (2, 4)
_PAD = 8
_NR = 16
_PW = 256
_SM = 64
_LA = 1
_NR0 = 32
_W0 = (0, 0.75)
_WS = (0.1, 0.9)
_WN = (0.02, 0.9)
_WP = (0.5, 0.98)
_SCOPES = False
_FLAGS = None


def _layernorm(x, eps=1e-5):
    m = jnp.mean(x, axis=-1, keepdims=True)
    c = x - m
    v = jnp.mean(c * c, axis=-1, keepdims=True)
    return c * lax.rsqrt(v + eps)


def _gelu(x):
    c0 = float(np.sqrt(2.0 / np.pi))
    c1 = c0 * 0.044715
    hx = 0.5 * x
    return hx + hx * jnp.tanh(x * (c0 + c1 * (x * x)))


def _dot(a, b):
    return lax.dot_general(a, b, (((1,), (0,)), ((), ())), preferred_element_type=_F32)


def _dot_nt(a, b):
    return lax.dot_general(a, b, (((1,), (1,)), ((), ())), preferred_element_type=_F32)


def _pack(x):
    return pltpu.bitcast(x.astype(_BF16), _U32)


def _unpack(w):
    return pltpu.bitcast(w, _BF16)


def _strassen_lhs(a11, a12, a21, a22):
    return a11 + a22, a21 + a22, a11, a22, a11 + a12, a21 - a11, a12 - a22


def _strassen_out(m):
    m1, m2, m3, m4, m5, m6, m7 = m
    return (m1 + m4) + (m7 - m5), m3 + m5, m2 + m4, (m1 - m2) + (m3 + m6)


def _strassen(prod, done):
    m1, m2 = prod(0), prod(1)
    c22 = m1 - m2
    m4 = prod(3)
    done(2, m2 + m4)
    c11 = m1 + m4
    c22 = prod(5) + c22
    c11 = prod(6) + c11
    m3 = prod(2)
    done(3, c22 + m3)
    m5 = prod(4)
    done(0, c11 - m5)
    done(1, m3 + m5)
    return m1, m2, m4, c22, c11, m3, m5


def _after(x, z):
    w = pltpu.bitcast(x, _U32)
    z = jnp.tile(z, (w.shape[0] // z.shape[0], w.shape[1] // z.shape[1]))
    return pltpu.bitcast(w | z, x.dtype)


class _scope:
    def __init__(self, name):
        self.c = jax.named_scope(name) if _SCOPES else None
    def __enter__(self):
        if self.c: self.c.__enter__()
    def __exit__(self, *a):
        if self.c: self.c.__exit__(*a)


def _ds(start, size, align):
    return pl.ds(start if isinstance(start, int) else pl.multiple_of(start, align), size)


def _kernel(x_hbm, mem0_ref, wq_hbm, wk_hbm, wv_hbm, wo_hbm, w1_hbm, w2_hbm, w3_hbm, w4_hbm,
            out_hbm,
            x_v, w1raw_v, w1_v, w2_v, w3_v, w4_v, stage_v, wqkv_v, wo_v,
            xn_v, h_v, y_v, g_v, base_v, att_v,
            sem_x, sem_w, sem_f, sem_s, sem_o, sem_out, *, seg):
    S, D = x_v.shape
    dh = D // 2
    fh = w3_v.shape[2]
    n_mem = mem0_ref.shape[0]
    H = wqkv_v.shape[0] // 3
    E = wqkv_v.shape[2]
    nblk = S // _TM
    th = _TM // 2
    nfc = fh // _FC
    dch = D // nblk
    n_wo = D // 128

    def x_copy(i):
        rows = _ds(i * _TM, _TM, _TM)
        return pltpu.make_async_copy(x_hbm.at[rows], x_v.at[rows], sem_x.at[i])

    quad = ((0, 0, 1), (0, 1, 2), (1, 0, 3), (1, 1, 4))

    def quad_copies(src, dst, r0, n, sems):
        _, rows, cols = dst.shape
        return [pltpu.make_async_copy(
            src.bitcast(_U32).at[_ds(r * rows + r0, n, 8), pl.ds(c * cols, cols)],
            dst.at[slot, _ds(r0, n, 8)], sems(k)) for k, (r, c, slot) in enumerate(quad)]

    def ffn_copies(c):
        cps = quad_copies(w4_hbm, w4_v, c * _FC // 2, _FC // 2, lambda k: sem_f.at[c, k])
        for k, (r, q, slot) in enumerate(quad):
            cps.append(pltpu.make_async_copy(
                w3_hbm.bitcast(_U32).at[pl.ds(r * dh // 2, dh // 2), pl.ds(q * fh + c * _FC, _FC)],
                w3_v.at[slot, :, pl.ds(c * _FC, _FC)], sem_f.at[c, 4 + k]))
        return cps

    def stage_copy(t, i):
        src = (wq_hbm, wk_hbm, wv_hbm)[t].bitcast(_U32)
        n = dch * H // 2
        return pltpu.make_async_copy(src.at[_ds(i * n, n, n)], stage_v.at[i % 2, t], sem_s.at[i % 2, t])

    def wo_copy(j):
        src = wo_hbm.bitcast(_U32).at[:, _ds(j * 128, 128, 128)]
        return pltpu.make_async_copy(src, wo_v.at[j], sem_o.at[j])

    w1_copy = pltpu.make_async_copy(w1_hbm.bitcast(_U32), w1raw_v, sem_w.at[4])
    w2_copies = quad_copies(w2_hbm, w2_v, 0, dh // 2, lambda k: sem_w.at[k])

    mem0 = mem0_ref[...].astype(_F32)
    zero = jnp.where(jnp.abs(mem0[:8, :128]) < 0.0, 1, 0).astype(_U32)

    def mark(v, r=0, c=0):
        return pltpu.bitcast(v[r:r + 8, c:c + 128], _U32) & zero

    def put_lhs(slot, r, y):
        n = y.shape[0] // 2
        ops = _strassen_lhs(y[:n, :dh], y[:n, dh:], y[n:, :dh], y[n:, dh:])
        for p in range(7):
            y_v[slot, p, _ds(r // 2, n // 2, 8), :] = _pack(ops[p])

    def put_rhs(w_v, idx, quads, z, seeds=False):
        high = jnp.tile(z | _U32(0xFFFF0000), (1, quads[0].shape[1] // 128))
        sums = []
        for b11, b12, b21, b22 in ([pltpu.bitcast(q << 16, _F32) for q in quads],
                                   [pltpu.bitcast(q & high, _F32) for q in quads]):
            sums.append((b11 + b22, b12 - b22, b21 - b11, b11 + b12, b21 + b22))
        for slot, even, odd in zip((0, 2, 3, 5, 6), *sums):
            w_v[(slot,) + idx] = pltpu.pack_elementwise([even, odd], packed_dtype=_BF16)
        if seeds:
            w_v[(1,) + idx] = quads[0]
            w_v[(4,) + idx] = quads[3]

    def prep(w_v, r0, c0, nc):
        idx = (_ds(r0, 8, 8), pl.ds(c0, nc))
        return lambda z: put_rhs(w_v, idx, [w_v[(slot,) + idx] for slot in (1, 2, 3, 4)], z)

    def spread(jobs, marks):
        prev = None
        for k, job in enumerate(jobs):
            z = marks[k * len(marks) // len(jobs)]
            prev = job(z if prev is None else z | prev)

    def halves(i, r, n):
        return _ds(i * _TM + r, n, 16), _ds(i * _TM + th + r, n, 16)

    def norm_jobs(i, slot, _NR):
        def job(r, z):
            top, bot = halves(i, r, _NR)
            x = _after(jnp.concatenate([x_v[top, :], x_v[bot, :]], axis=0), z)
            xn = _layernorm(x.astype(_F32))
            xn_v[top, :] = xn[:_NR]
            xn_v[bot, :] = xn[_NR:]
            y = _layernorm(xn)
            put_lhs(slot, r, y)
            return functools.reduce(jnp.bitwise_or, [mark(y, k) for k in range(0, y.shape[0], 8)])
        return [functools.partial(job, r) for r in range(0, th, _NR)]

    def ffn_norm_jobs(i, slot):
        def job(r, z):
            top, bot = halves(i, r, _NR)
            x1 = jnp.concatenate([base_v[top, :] + xn_v[top, :], base_v[bot, :] + xn_v[bot, :]], axis=0)
            y = _layernorm(_after(x1, z))
            put_lhs(slot, r, y)
            return functools.reduce(jnp.bitwise_or, [mark(y, k) for k in range(0, y.shape[0], 8)])
        return [functools.partial(job, r) for r in range(0, th, _NR)]

    def prep_jobs(c):
        return ([prep(w4_v, c * _FC // 2 + r, k, _PW)
                 for r in range(0, _FC // 2, 8) for k in range(0, dh, _PW)]
                + [prep(w3_v, r, c * _FC + k, _PW)
                   for r in range(0, dh // 2, 8) for k in range(0, _FC, _PW)])

    corners = [(r, c) for r in (0, th) for c in (0, dh)]
    tiles = [(r, c) for r in range(0, th, _SM) for c in range(0, dh, 128)]

    def shift_jobs(i):
        def job(r0, c0, z):
            a = []
            for r, c in corners:
                sh = (-1, 1, -2, 2)[(c + c0) // (D // 4)]
                lo = 0 if sh < 0 else _PAD
                win = _after(h_v[pl.ds(i * _TM + r + r0 + lo, _SM + _PAD), pl.ds(c + c0, 128)], z)
                a.append(win[_PAD - lo + sh:_PAD - lo + sh + _SM])
            for p, v in enumerate(_strassen_lhs(*a)):
                g_v[p, pl.ds(r0 // 2, _SM // 2), pl.ds(c0, 128)] = _pack(v)
        return [functools.partial(job, r0, c0) for r0, c0 in tiles]

    def mix(lhs, w_v, out_v, row, act):
        marks = []
        for r0, c0 in tiles:
            def prod(p):
                return _dot(_unpack(lhs[p, pl.ds(r0 // 2, _SM // 2), :]),
                            _unpack(w_v[p, :, pl.ds(c0, 128)]))

            def done(q, v):
                r, c = corners[q]
                out_v[pl.ds(row + r + r0, _SM), pl.ds(c + c0, 128)] = act(v)

            marks += [mark(v) for v in _strassen(prod, done)]
        return marks

    def window(marks, w):
        return marks[int(w[0] * len(marks)):int(w[1] * len(marks))]

    x_copy(0).start()
    w1_copy.start()
    x_copy(1).start()
    h_v[pl.ds(0, _PAD), :] = jnp.zeros((_PAD, D), _F32)
    h_v[pl.ds(_PAD + S, _PAD), :] = jnp.zeros((_PAD, D), _F32)
    x_copy(0).wait()
    xn = _layernorm(x_v[pl.ds(0, _TM), :].astype(_F32))
    xn_v[pl.ds(0, _TM), :] = xn
    y_v[0, pl.ds(0, 4)] = jnp.stack(
        [_pack(_layernorm(xn))[r // 2:(r + th) // 2, c:c + dh] for r, c in corners])
    w1_copy.wait()

    for i in range(nblk + 1):
      with _scope("mix%d" % i):
        c = i - 2
        if i == 0:
            for cp in w2_copies:
                cp.start()
        if i + 2 < nblk:
            x_copy(i + 2).start()
        if 0 <= c + _LA < nfc:
            for cp in ffn_copies(c + _LA):
                cp.start()
        if i == nblk - 1:
            for t in range(3):
                stage_copy(t, 0).start()
        if i + 1 < nblk:
            x_copy(i + 1).wait()
        if i == 1:
            for cp in w2_copies:
                cp.wait()
        if 0 <= c < nfc:
            for cp in ffn_copies(c):
                cp.wait()

        if i == 0:
            marks = []
            for r in range(0, _TM, _SM):
                q = 2 * (r // th)
                y = jnp.concatenate([_unpack(y_v[0, q + k, pl.ds(r % th // 2, _SM // 2), :])
                                     for k in range(2)], axis=1)
                for k in range(0, D, 128):
                    a = _dot(y, _unpack(w1raw_v[:, pl.ds(k, 128)]))
                    h_v[pl.ds(_PAD + r, _SM), pl.ds(k, 128)] = _gelu(a)
                    marks.append(mark(a))

            def first(k, z):
                quads = [w1raw_v[pl.ds(r * dh // 2 + k, 8), pl.ds(q * dh, dh)] for r, q, _ in quad]
                put_rhs(w1_v, (pl.ds(k, 8), slice(None)), quads, z, seeds=True)

            spread([functools.partial(first, k) for k in range(0, dh // 2, 8)], marks)
            spread(norm_jobs(1, 1, _NR0), window(marks, _W0))
            continue
        marks = []
        if i < nblk:
            marks += mix(y_v.at[i % 2], w1_v, h_v, _PAD + i * _TM, _gelu)
            spread(shift_jobs(i - 1), window(marks, _WS))
        else:
            for job in shift_jobs(i - 1):
                job(zero)
        if i == 1:
            spread([prep(w2_v, k, q, _PW) for q in range(0, dh, _PW) for k in range(0, dh // 2, 8)],
                   window(marks, (0, 0.9)))
        marks += mix(g_v, w2_v, base_v, (i - 1) * _TM, lambda v: v)
        if i + 1 < nblk:
            spread(norm_jobs(i + 1, (i + 1) % 2, _NR), window(marks, _WN))
        elif i + 1 == nblk:
            spread(ffn_norm_jobs(0, 0), window(marks, _WN))
        if 0 <= c < nfc:
            spread(prep_jobs(c), window(marks, _WP if i < nblk else (0, 0.97)))

    def ffn(i, _):
        @pl.when(i + 1 < nblk)
        def _():
            for t in range(3):
                stage_copy(t, i + 1).start()
        wo_copy(i).start()
        for t in range(3):
            stage_copy(t, i).wait()

        def retile(n, z):
            n, odd = divmod(n, 2)
            t, r, jh = n // (dch // 8), (n // 2) % (dch // 16), n % 2
            v = stage_v[i % 2, t, pl.ds(r * 8 * H, 8 * H), :].reshape(8, H, E)
            a, b = v[:, 8 * jh:8 * jh + 8], v[:, H // 2 + 8 * jh:H // 2 + 8 * jh + 8]
            low = (z | _U32(0xFFFF))[None]
            w = ((a >> 16) | (b & ~low)) if odd else ((a & low) | (b << 16))
            w = jnp.swapaxes(w, 0, 1)
            rows = _ds(i * (dch // 2) + 8 * r, 8, 8)
            for j in range(8):
                wqkv_v[6 * (8 * jh + j) + 3 * odd + t, rows, :] = w[j]

        pieces = list(range(3 * (dch // 16) * 4))
        u = []
        for c in range(nfc):
            g = [_dot(_unpack(y_v[i % 2, p]), _unpack(w3_v[p, :, pl.ds(c * _FC, _FC)]))
                 for p in range(7)]
            for p in range(7):
                for k in range(0, _FC, 128):
                    if pieces:
                        retile(pieces.pop(0), mark(g[p], 0, k))
            u.append([o.astype(_BF16) for o in _strassen_lhs(*[_gelu(q) for q in _strassen_out(g)])])
        assert not pieces
        m = [_dot(jnp.concatenate([uc[p] for uc in u], axis=1), _unpack(w4_v[p])) for p in range(7)]
        spread(ffn_norm_jobs(jnp.minimum(i + 1, nblk - 1), (i + 1) % 2),
               [mark(m[p], 0, k) for p in range(1, 5) for k in (0, 256)])
        for (r, c), v in zip(corners, _strassen_out(m)):
            base_v[_ds(i * _TM + r, th, th), pl.ds(c, dh)] += v
        return 0

    with _scope("ffn"):
        lax.fori_loop(0, nblk, ffn, 0)

    for j in range(n_wo):
        wo_copy(j).wait()
    L = n_mem + seg
    row = lax.broadcasted_iota(jnp.int32, (L, L), 0)
    col = lax.broadcasted_iota(jnp.int32, (L, L), 1)
    mask = (row < n_mem) | (row >= col)
    scale = float(E) ** -0.5
    n_seg = S // seg

    def step(s, mem):
        rows = _ds(s * seg, seg, seg)
        hh = jnp.concatenate([mem, xn_v[rows, :]], axis=0)
        ng = H // _HG
        qkv, sc = {}, {}

        def proj(g):
            w = jnp.concatenate([_unpack(wqkv_v[3 * _HG * g + n]) for n in range(3 * _HG)], axis=1)
            qkv[g] = _dot(hh, w)

        def scores(g):
            y = qkv[g]
            sc[g] = [_dot_nt(y[:, (3 * n) * E:(3 * n + 1) * E],
                             y[:, (3 * n + 1) * E:(3 * n + 2) * E].astype(_BF16))
                     for n in range(_HG)]

        def attend(g):
            y = qkv[g]
            for n in range(_HG):
                z = jnp.where(mask, sc[g][n] * scale, -1e9)
                e = jnp.exp(z - jnp.max(z, axis=-1, keepdims=True))
                r = 1.0 / jnp.sum(e, axis=-1, keepdims=True)
                o = _dot(e * r, y[:, (3 * n + 2) * E:(3 * n + 3) * E].astype(_BF16))
                att_v[:, pl.ds((g * _HG + n) * E, E)] = o

        def outproj(g0, g1):
            k0, kn = g0 * _HG * E, (g1 - g0) * _HG * E
            wo = jnp.concatenate(
                [_unpack(wo_v[j, pl.ds(k0 // 2, kn // 2), :]) for j in range(n_wo)], axis=1)
            return _dot(att_v[:, pl.ds(k0, kn)], wo)

        for g in range(ng):
            proj(g)
            if g >= 1:
                scores(g - 1)
            if g >= 2:
                attend(g - 2)
        o = outproj(0, _WO[0])
        scores(ng - 1)
        attend(ng - 2)
        o = outproj(_WO[0], _WO[1]) + o
        attend(ng - 1)
        o = outproj(_WO[1], ng) + o
        x_v[rows, :] = ((x_v[rows, :].astype(_F32) + (hh[n_mem:] + base_v[rows, :])) + o[n_mem:]).astype(_BF16)
        pltpu.make_async_copy(x_v.at[rows], out_hbm.at[rows], sem_out.at[0]).start()
        return o[:n_mem]

    with _scope("A"):
        lax.fori_loop(0, n_seg, step, mem0)
    pltpu.make_async_copy(x_v, out_hbm, sem_out.at[0]).wait()


@functools.partial(jax.jit, static_argnames=("A_seg_len",))
def pallas_parallel_sum__memory_aug_recurrent_mem_tr__mixer_s_mlp__prompt_kernel(
    A_x: jax.Array,
    A_mem0: jax.Array,
    A_Wq: jax.Array,
    A_Wk: jax.Array,
    A_Wv: jax.Array,
    A_Wo: jax.Array,
    A_seg_len: int,
    B_x: jax.Array,
    B_w1: jax.Array,
    B_w2: jax.Array,
    B_w3: jax.Array,
    B_w4: jax.Array,
):
    del B_x
    B, S, D = A_x.shape
    _, H, E = A_Wq.shape
    M = A_mem0.shape[1]
    F = B_w3.shape[1]
    seg = int(A_seg_len)
    nblk = S // _TM
    assert B == 1 and S % _TM == 0 and S % seg == 0 and F % (2 * _FC) == 0 and H % _HG == 0
    assert nblk == D // 128

    hbm = pl.BlockSpec(memory_space=pltpu.HBM)
    out = pl.pallas_call(
        functools.partial(_kernel, seg=seg),
        out_shape=jax.ShapeDtypeStruct((S, D), A_x.dtype),
        in_specs=[hbm, pl.BlockSpec(memory_space=pltpu.VMEM)] + [hbm] * 8,
        out_specs=hbm,
        scratch_shapes=[
            pltpu.VMEM((S, D), _BF16),
            pltpu.VMEM((D // 2, D), _U32),
            pltpu.VMEM((7, D // 4, D // 2), _U32),
            pltpu.VMEM((7, D // 4, D // 2), _U32),
            pltpu.VMEM((7, D // 4, F // 2), _U32),
            pltpu.VMEM((7, F // 4, D // 2), _U32),
            pltpu.VMEM((2, 3, D // nblk * H // 2, E), _U32),
            pltpu.VMEM((3 * H, D // 2, E), _U32),
            pltpu.VMEM((D // 128, H * E // 2, 128), _U32),
            pltpu.VMEM((S, D), _F32),
            pltpu.VMEM((S + 2 * _PAD, D), _F32),
            pltpu.VMEM((2, 7, _TM // 4, D // 2), _U32),
            pltpu.VMEM((7, _TM // 4, D // 2), _U32),
            pltpu.VMEM((S, D), _F32),
            pltpu.VMEM((M + seg, H * E), _F32),
            pltpu.SemaphoreType.DMA((nblk,)),
            pltpu.SemaphoreType.DMA((5,)),
            pltpu.SemaphoreType.DMA((nblk, 8)),
            pltpu.SemaphoreType.DMA((2, 3)),
            pltpu.SemaphoreType.DMA((D // 128,)),
            pltpu.SemaphoreType.DMA((1,)),
        ],
        compiler_params=pltpu.CompilerParams(vmem_limit_bytes=124 * 1024 * 1024, flags=_FLAGS),
    )(A_x.reshape(S, D), A_mem0.reshape(M, D),
      A_Wq.reshape(D * H, E), A_Wk.reshape(D * H, E), A_Wv.reshape(D * H, E),
      A_Wo.reshape(H * E, D), B_w1, B_w2, B_w3, B_w4)
    return out.reshape(B, S, D)
```

```python
import functools

import jax
import jax.numpy as jnp
import numpy as np
from jax import lax
import jax.experimental.pallas as pl
import jax.experimental.pallas.tpu as pltpu

_F32 = jnp.float32
_BF16 = jnp.bfloat16
_U32 = jnp.uint32

_TM = 256
_FC = 256
_HG = 4
_WO = (2, 4)
_PAD = 8
_NR = 16
_PW = 256
_LATE = 8
_PU = 8
_AU = 2
_PM = 64
_PR = 16
_SM = 64
_LA = 1
_NR0 = 32
_W0 = (0, 0.75)
_WS = (0.1, 0.9)
_WN = (0.02, 0.9)
_WP = (0.5, 0.98)
_SCOPES = False
_FLAGS = None


def _layernorm(x, eps=1e-5):
    m = jnp.mean(x, axis=-1, keepdims=True)
    c = x - m
    v = jnp.mean(c * c, axis=-1, keepdims=True)
    return c * lax.rsqrt(v + eps)


def _gelu(x):
    c0 = float(np.sqrt(2.0 / np.pi))
    c1 = c0 * 0.044715
    hx = 0.5 * x
    return hx + hx * jnp.tanh(x * (c0 + c1 * (x * x)))


def _dot(a, b):
    return lax.dot_general(a, b, (((1,), (0,)), ((), ())), preferred_element_type=_F32)


def _dot_nt(a, b):
    return lax.dot_general(a, b, (((1,), (1,)), ((), ())), preferred_element_type=_F32)


def _pack(x):
    return pltpu.bitcast(x.astype(_BF16), _U32)


def _unpack(w):
    return pltpu.bitcast(w, _BF16)


def _strassen_lhs(a11, a12, a21, a22):
    return a11 + a22, a21 + a22, a11, a22, a11 + a12, a21 - a11, a12 - a22


def _strassen_out(m):
    m1, m2, m3, m4, m5, m6, m7 = m
    return (m1 + m4) + (m7 - m5), m3 + m5, m2 + m4, (m1 - m2) + (m3 + m6)


def _strassen(prod, done):
    m1, m2 = prod(0), prod(1)
    c22 = m1 - m2
    m4 = prod(3)
    done(2, m2 + m4)
    c11 = m1 + m4
    c22 = prod(5) + c22
    c11 = prod(6) + c11
    m3 = prod(2)
    done(3, c22 + m3)
    m5 = prod(4)
    done(0, c11 - m5)
    done(1, m3 + m5)
    return m1, m2, m4, c22, c11, m3, m5


def _after(x, z):
    w = pltpu.bitcast(x, _U32)
    z = jnp.tile(z, (w.shape[0] // z.shape[0], w.shape[1] // z.shape[1]))
    return pltpu.bitcast(w | z, x.dtype)


class _scope:
    def __init__(self, name):
        self.c = jax.named_scope(name) if _SCOPES else None
    def __enter__(self):
        if self.c: self.c.__enter__()
    def __exit__(self, *a):
        if self.c: self.c.__exit__(*a)


def _ds(start, size, align):
    return pl.ds(start if isinstance(start, int) else pl.multiple_of(start, align), size)


def _kernel(x_hbm, mem0_ref, wq_hbm, wk_hbm, wv_hbm, wo_hbm, w1_hbm, w2_hbm, w3_hbm, w4_hbm,
            out_hbm,
            x_v, wqkv_v, wo_v, xn_v, base_v, *, seg):
    S, D = x_v.shape
    F = w3_hbm.shape[1]
    H, E = wqkv_v.shape[0] // 3, wqkv_v.shape[2]
    nblk, n_late = S // _TM, S // seg * _LATE
    mem0 = mem0_ref[...].astype(_F32)
    zero = jnp.where(jnp.abs(mem0[:8, :128]) < 0.0, 1, 0).astype(_U32)
    pl.run_scoped(
        functools.partial(_mixer, x_hbm, wq_hbm, wk_hbm, wv_hbm, wo_hbm, w1_hbm, w2_hbm, w3_hbm,
                          w4_hbm, x_v, wqkv_v, wo_v, xn_v, base_v, zero),
        pltpu.VMEM((D // 2, D), _U32),
        pltpu.VMEM((7, D // 4, D // 2), _U32),
        pltpu.VMEM((7, D // 4, D // 2), _U32),
        pltpu.VMEM((7, D // 4, F // 2), _U32),
        pltpu.VMEM((7, F // 4, D // 2), _U32),
        pltpu.VMEM((2, 3, D // nblk * H // 2, E), _U32),
        pltpu.VMEM((S + 2 * _PAD, D), _F32),
        pltpu.VMEM((2, 7, _TM // 4, D // 2), _U32),
        pltpu.VMEM((7, _TM // 4, D // 2), _U32),
        pltpu.SemaphoreType.DMA((nblk,)),
        pltpu.SemaphoreType.DMA((5,)),
        pltpu.SemaphoreType.DMA((nblk, 8)),
        pltpu.SemaphoreType.DMA((2, 3)),
        pltpu.SemaphoreType.DMA((D // 128,)))
    pl.run_scoped(
        functools.partial(_memory, out_hbm, x_v, wqkv_v, wo_v, xn_v, base_v, mem0, zero, seg),
        pltpu.VMEM((7, n_late // 4, D // 2), _U32),
        pltpu.VMEM((7, n_late // 4, D // 2), _U32),
        pltpu.VMEM((3 * H, n_late, E), _F32),
        pltpu.VMEM((n_late, H * E), _F32),
        pltpu.VMEM((n_late, D), _F32),
        pltpu.VMEM(((mem0.shape[0] + seg - _LATE) // 2, H * E), _U32),
        pltpu.VMEM((5, D // 4, 128), _U32),
        pltpu.VMEM((5, D // 4, 128), _U32),
        pltpu.SemaphoreType.DMA((1,)))


def _mixer(x_hbm, wq_hbm, wk_hbm, wv_hbm, wo_hbm, w1_hbm, w2_hbm, w3_hbm, w4_hbm,
           x_v, wqkv_v, wo_v, xn_v, base_v, zero,
           w1raw_v, w1_v, w2_v, w3_v, w4_v, stage_v, h_v, y_v, g_v,
           sem_x, sem_w, sem_f, sem_s, sem_o):
    S, D = x_v.shape
    dh = D // 2
    fh = w3_v.shape[2]
    H = wqkv_v.shape[0] // 3
    E = wqkv_v.shape[2]
    nblk = S // _TM
    th = _TM // 2
    nfc = fh // _FC
    dch = D // nblk
    n_wo = D // 128

    def x_copy(i):
        rows = _ds(i * _TM, _TM, _TM)
        return pltpu.make_async_copy(x_hbm.at[rows], x_v.at[rows], sem_x.at[i])

    quad = ((0, 0, 1), (0, 1, 2), (1, 0, 3), (1, 1, 4))

    def quad_copies(src, dst, r0, n, sems):
        _, rows, cols = dst.shape
        return [pltpu.make_async_copy(
            src.bitcast(_U32).at[_ds(r * rows + r0, n, 8), pl.ds(c * cols, cols)],
            dst.at[slot, _ds(r0, n, 8)], sems(k)) for k, (r, c, slot) in enumerate(quad)]

    def ffn_copies(c):
        cps = quad_copies(w4_hbm, w4_v, c * _FC // 2, _FC // 2, lambda k: sem_f.at[c, k])
        for k, (r, q, slot) in enumerate(quad):
            cps.append(pltpu.make_async_copy(
                w3_hbm.bitcast(_U32).at[pl.ds(r * dh // 2, dh // 2), pl.ds(q * fh + c * _FC, _FC)],
                w3_v.at[slot, :, pl.ds(c * _FC, _FC)], sem_f.at[c, 4 + k]))
        return cps

    def stage_copy(t, i):
        src = (wq_hbm, wk_hbm, wv_hbm)[t].bitcast(_U32)
        n = dch * H // 2
        return pltpu.make_async_copy(src.at[_ds(i * n, n, n)], stage_v.at[i % 2, t], sem_s.at[i % 2, t])

    def wo_copy(j):
        src = wo_hbm.bitcast(_U32).at[:, _ds(j * 128, 128, 128)]
        return pltpu.make_async_copy(src, wo_v.at[j], sem_o.at[j])

    w1_copy = pltpu.make_async_copy(w1_hbm.bitcast(_U32), w1raw_v, sem_w.at[4])
    w2_copies = quad_copies(w2_hbm, w2_v, 0, dh // 2, lambda k: sem_w.at[k])

    def mark(v, r=0, c=0):
        return pltpu.bitcast(v[r:r + 8, c:c + 128], _U32) & zero

    def put_lhs(slot, r, y):
        n = y.shape[0] // 2
        ops = _strassen_lhs(y[:n, :dh], y[:n, dh:], y[n:, :dh], y[n:, dh:])
        for p in range(7):
            y_v[slot, p, _ds(r // 2, n // 2, 8), :] = _pack(ops[p])

    def put_rhs(w_v, idx, quads, z, seeds=False):
        high = jnp.tile(z | _U32(0xFFFF0000), (1, quads[0].shape[1] // 128))
        sums = []
        for b11, b12, b21, b22 in ([pltpu.bitcast(q << 16, _F32) for q in quads],
                                   [pltpu.bitcast(q & high, _F32) for q in quads]):
            sums.append((b11 + b22, b12 - b22, b21 - b11, b11 + b12, b21 + b22))
        for slot, even, odd in zip((0, 2, 3, 5, 6), *sums):
            w_v[(slot,) + idx] = pltpu.pack_elementwise([even, odd], packed_dtype=_BF16)
        if seeds:
            w_v[(1,) + idx] = quads[0]
            w_v[(4,) + idx] = quads[3]

    def prep(w_v, r0, c0, nc):
        idx = (_ds(r0, 8, 8), pl.ds(c0, nc))
        return lambda z: put_rhs(w_v, idx, [w_v[(slot,) + idx] for slot in (1, 2, 3, 4)], z)

    def spread(jobs, marks):
        prev = None
        for k, job in enumerate(jobs):
            z = marks[k * len(marks) // len(jobs)]
            prev = job(z if prev is None else z | prev)

    def halves(i, r, n):
        return _ds(i * _TM + r, n, 16), _ds(i * _TM + th + r, n, 16)

    def norm_jobs(i, slot, _NR):
        def job(r, z):
            top, bot = halves(i, r, _NR)
            x = _after(jnp.concatenate([x_v[top, :], x_v[bot, :]], axis=0), z)
            xn = _layernorm(x.astype(_F32))
            xn_v[top, :] = xn[:_NR]
            xn_v[bot, :] = xn[_NR:]
            y = _layernorm(xn)
            put_lhs(slot, r, y)
            return functools.reduce(jnp.bitwise_or, [mark(y, k) for k in range(0, y.shape[0], 8)])
        return [functools.partial(job, r) for r in range(0, th, _NR)]

    def ffn_norm_jobs(i, slot):
        def job(r, z):
            top, bot = halves(i, r, _NR)
            x1 = jnp.concatenate([base_v[top, :] + xn_v[top, :], base_v[bot, :] + xn_v[bot, :]], axis=0)
            y = _layernorm(_after(x1, z))
            put_lhs(slot, r, y)
            return functools.reduce(jnp.bitwise_or, [mark(y, k) for k in range(0, y.shape[0], 8)])
        return [functools.partial(job, r) for r in range(0, th, _NR)]

    def prep_jobs(c):
        return ([prep(w4_v, c * _FC // 2 + r, k, _PW)
                 for r in range(0, _FC // 2, 8) for k in range(0, dh, _PW)]
                + [prep(w3_v, r, c * _FC + k, _PW)
                   for r in range(0, dh // 2, 8) for k in range(0, _FC, _PW)])

    corners = [(r, c) for r in (0, th) for c in (0, dh)]
    tiles = [(r, c) for r in range(0, th, _SM) for c in range(0, dh, 128)]

    def shift_jobs(i):
        def job(r0, c0, z):
            a = []
            for r, c in corners:
                sh = (-1, 1, -2, 2)[(c + c0) // (D // 4)]
                lo = 0 if sh < 0 else _PAD
                win = _after(h_v[pl.ds(i * _TM + r + r0 + lo, _SM + _PAD), pl.ds(c + c0, 128)], z)
                a.append(win[_PAD - lo + sh:_PAD - lo + sh + _SM])
            for p, v in enumerate(_strassen_lhs(*a)):
                g_v[p, pl.ds(r0 // 2, _SM // 2), pl.ds(c0, 128)] = _pack(v)
        return [functools.partial(job, r0, c0) for r0, c0 in tiles]

    def mix(lhs, w_v, out_v, row, act):
        marks = []
        for r0, c0 in tiles:
            def prod(p):
                return _dot(_unpack(lhs[p, pl.ds(r0 // 2, _SM // 2), :]),
                            _unpack(w_v[p, :, pl.ds(c0, 128)]))

            def done(q, v):
                r, c = corners[q]
                out_v[pl.ds(row + r + r0, _SM), pl.ds(c + c0, 128)] = act(v)

            marks += [mark(v) for v in _strassen(prod, done)]
        return marks

    def window(marks, w):
        return marks[int(w[0] * len(marks)):int(w[1] * len(marks))]

    x_copy(0).start()
    w1_copy.start()
    x_copy(1).start()
    h_v[pl.ds(0, _PAD), :] = jnp.zeros((_PAD, D), _F32)
    h_v[pl.ds(_PAD + S, _PAD), :] = jnp.zeros((_PAD, D), _F32)
    x_copy(0).wait()
    xn = _layernorm(x_v[pl.ds(0, _TM), :].astype(_F32))
    xn_v[pl.ds(0, _TM), :] = xn
    y_v[0, pl.ds(0, 4)] = jnp.stack(
        [_pack(_layernorm(xn))[r // 2:(r + th) // 2, c:c + dh] for r, c in corners])
    w1_copy.wait()

    for i in range(nblk + 1):
      with _scope("mix%d" % i):
        c = i - 2
        if i == 0:
            for cp in w2_copies:
                cp.start()
        if i + 2 < nblk:
            x_copy(i + 2).start()
        if 0 <= c + _LA < nfc:
            for cp in ffn_copies(c + _LA):
                cp.start()
        if i == nblk - 1:
            for t in range(3):
                stage_copy(t, 0).start()
        if i + 1 < nblk:
            x_copy(i + 1).wait()
        if i == 1:
            for cp in w2_copies:
                cp.wait()
        if 0 <= c < nfc:
            for cp in ffn_copies(c):
                cp.wait()

        if i == 0:
            marks = []
            for r in range(0, _TM, _SM):
                q = 2 * (r // th)
                y = jnp.concatenate([_unpack(y_v[0, q + k, pl.ds(r % th // 2, _SM // 2), :])
                                     for k in range(2)], axis=1)
                for k in range(0, D, 128):
                    a = _dot(y, _unpack(w1raw_v[:, pl.ds(k, 128)]))
                    h_v[pl.ds(_PAD + r, _SM), pl.ds(k, 128)] = _gelu(a)
                    marks.append(mark(a))

            def first(k, z):
                quads = [w1raw_v[pl.ds(r * dh // 2 + k, 8), pl.ds(q * dh, dh)] for r, q, _ in quad]
                put_rhs(w1_v, (pl.ds(k, 8), slice(None)), quads, z, seeds=True)

            spread([functools.partial(first, k) for k in range(0, dh // 2, 8)], marks)
            spread(norm_jobs(1, 1, _NR0), window(marks, _W0))
            continue
        marks = []
        if i < nblk:
            marks += mix(y_v.at[i % 2], w1_v, h_v, _PAD + i * _TM, _gelu)
            spread(shift_jobs(i - 1), window(marks, _WS))
        else:
            for job in shift_jobs(i - 1):
                job(zero)
        if i == 1:
            spread([prep(w2_v, k, q, _PW) for q in range(0, dh, _PW) for k in range(0, dh // 2, 8)],
                   window(marks, (0, 0.9)))
        marks += mix(g_v, w2_v, base_v, (i - 1) * _TM, lambda v: v)
        if i + 1 < nblk:
            spread(norm_jobs(i + 1, (i + 1) % 2, _NR), window(marks, _WN))
        elif i + 1 == nblk:
            spread(ffn_norm_jobs(0, 0), window(marks, _WN))
        if 0 <= c < nfc:
            spread(prep_jobs(c), window(marks, _WP if i < nblk else (0, 0.97)))

    def ffn(i, _):
        @pl.when(i + 1 < nblk)
        def _():
            for t in range(3):
                stage_copy(t, i + 1).start()
        wo_copy(i).start()
        for t in range(3):
            stage_copy(t, i).wait()

        def retile(n, z):
            n, odd = divmod(n, 2)
            t, r, jh = n // (dch // 8), (n // 2) % (dch // 16), n % 2
            v = stage_v[i % 2, t, pl.ds(r * 8 * H, 8 * H), :].reshape(8, H, E)
            a, b = v[:, 8 * jh:8 * jh + 8], v[:, H // 2 + 8 * jh:H // 2 + 8 * jh + 8]
            low = (z | _U32(0xFFFF))[None]
            w = ((a >> 16) | (b & ~low)) if odd else ((a & low) | (b << 16))
            w = jnp.swapaxes(w, 0, 1)
            rows = _ds(i * (dch // 2) + 8 * r, 8, 8)
            for j in range(8):
                wqkv_v[6 * (8 * jh + j) + 3 * odd + t, rows, :] = w[j]

        pieces = list(range(3 * (dch // 16) * 4))
        u = []
        for c in range(nfc):
            g = [_dot(_unpack(y_v[i % 2, p]), _unpack(w3_v[p, :, pl.ds(c * _FC, _FC)]))
                 for p in range(7)]
            for p in range(7):
                for k in range(0, _FC, 128):
                    if pieces:
                        retile(pieces.pop(0), mark(g[p], 0, k))
            u.append([o.astype(_BF16) for o in _strassen_lhs(*[_gelu(q) for q in _strassen_out(g)])])
        assert not pieces
        m = [_dot(jnp.concatenate([uc[p] for uc in u], axis=1), _unpack(w4_v[p])) for p in range(7)]
        spread(ffn_norm_jobs(jnp.minimum(i + 1, nblk - 1), (i + 1) % 2),
               [mark(m[p], 0, k) for p in range(1, 5) for k in (0, 256)])
        for (r, c), v in zip(corners, _strassen_out(m)):
            base_v[_ds(i * _TM + r, th, th), pl.ds(c, dh)] += v
        return 0

    with _scope("ffn"):
        lax.fori_loop(0, nblk, ffn, 0)

    for j in range(n_wo):
        wo_copy(j).wait()


def _rhs_sums(quads, z):
    high = jnp.tile(z | _U32(0xFFFF0000), (quads[0].shape[0] // 8, quads[0].shape[1] // 128))
    sums = []
    for f11, f12, f21, f22 in ([pltpu.bitcast(q << 16, _F32) for q in quads],
                               [pltpu.bitcast(q & high, _F32) for q in quads]):
        sums.append((f11 + f22, f12 - f22, f21 - f11, f11 + f12, f21 + f22))
    return [pltpu.pack_elementwise([e, o], packed_dtype=_BF16) for e, o in zip(*sums)]


def _memory(out_hbm, x_v, wqkv_v, wo_v, xn_v, base_v, mem0, zero, seg,
            a_v, a2_v, pre_v, post_v, acc_v, att_v, b0_v, b1_v, sem_out):
    S, D = x_v.shape
    dh = D // 2
    H, E = wqkv_v.shape[0] // 3, wqkv_v.shape[2]
    n_wo = wo_v.shape[0]
    n_mem = mem0.shape[0]
    n_seg = S // seg
    early = seg - _LATE
    hl = n_seg * _LATE // 2

    for r in range(0, n_seg // 2, 2):
        top, bot = (jnp.concatenate([xn_v[pl.ds((r0 + k) * seg + early, _LATE), :] for k in range(2)],
                                    axis=0) for r0 in (r, r + n_seg // 2))
        for p, v in enumerate(_strassen_lhs(top[:, :dh], top[:, dh:], bot[:, :dh], bot[:, dh:])):
            a_v[p, pl.ds(r * _LATE // 2, _LATE), :] = _pack(v)

    def mark(v):
        return pltpu.bitcast(v[:8, :128], _U32) & zero

    def fill(b_v, quad, marks):
        n = b_v.shape[1] // _PR
        for k in range(n):
            rows = pl.ds(k * _PR, _PR)
            quads = [quad(r, c, k * _PR) for r in range(2) for c in range(2)]
            for j, w in enumerate(_rhs_sums(quads, marks[k * len(marks) // n])):
                b_v[j, rows, :] = w

    def operands(b_v, quad):
        n = b_v.shape[1]
        return lambda p: _unpack(quad(0, 0, 0, n) if p == 1 else quad(1, 1, 0, n) if p == 4
                                 else b_v[(0, 2, 3, 5, 6).index(p)])

    def qkv_quad(n):
        return lambda r, c, k, rows=_PR: wqkv_v[n + c, pl.ds(r * dh // 2 + k, rows), :]

    fill(b0_v, qkv_quad(0), [zero])

    def pre(i, _):
        for j in range(_PU):
            n = 2 * (i * _PU + j)
            b = operands((b0_v, b1_v)[j % 2], qkv_quad(n))
            marks = []
            for r0 in range(0, hl, _PM):
                def prod(p):
                    return _dot(_unpack(a_v[p, pl.ds(r0 // 2, _PM // 2), :]), b(p))

                def done(q, v):
                    pre_v[n + q % 2, pl.ds(q // 2 * hl + r0, _PM), :] = v

                marks += [mark(v) for v in _strassen(prod, done)]
            fill((b1_v, b0_v)[j % 2], qkv_quad(jnp.minimum(n + 2, 3 * H - 2)), marks[:-4])
        return 0

    with _scope("pre"):
        lax.fori_loop(0, 3 * H // 2 // _PU, pre, 0)

    L = n_mem + seg
    row = lax.broadcasted_iota(jnp.int32, (L, L), 0)
    col = lax.broadcasted_iota(jnp.int32, (L, L), 1)
    mask = (row < n_mem) | (row >= col)
    scale = float(E) ** -0.5

    def step(s, mem):
        rows = _ds(s * seg, early, seg)
        late = _ds(s * _LATE, _LATE, _LATE)
        hh = jnp.concatenate([mem, xn_v[rows, :]], axis=0)
        hb = hh.astype(_BF16)
        ng = H // _HG
        qkv, sc = {}, {}

        def proj(g):
            tiles = range(3 * _HG * g, 3 * _HG * (g + 1))
            w = jnp.concatenate([_unpack(wqkv_v[n]) for n in tiles], axis=1)
            if g == 0:
                y = _dot(hb[:, :dh], w[:dh])
                y = _dot(hb[:, dh:], w[dh:]) + y
            else:
                y = _dot(hb, w)
            qkv[g] = jnp.concatenate(
                [y, jnp.concatenate([pre_v[n, late, :] for n in tiles], axis=1)], axis=0)

        def scores(g):
            y = qkv[g]
            sc[g] = [_dot_nt(y[:, (3 * n) * E:(3 * n + 1) * E],
                             y[:, (3 * n + 1) * E:(3 * n + 2) * E].astype(_BF16))
                     for n in range(_HG)]

        def attend(g):
            y = qkv[g]
            for n in range(_HG):
                z = jnp.where(mask, sc[g][n] * scale, -1e9)
                e = jnp.exp(z - jnp.max(z, axis=-1, keepdims=True))
                r = 1.0 / jnp.sum(e, axis=-1, keepdims=True)
                o = _dot(e * r, y[:, (3 * n + 2) * E:(3 * n + 3) * E].astype(_BF16))
                cols = pl.ds((g * _HG + n) * E, E)
                att_v[:, cols] = _pack(o[:L - _LATE])
                post_v[late, cols] = o[L - _LATE:]

        def outproj(g0, g1):
            k0, kn = g0 * _HG * E, (g1 - g0) * _HG * E
            wo = jnp.concatenate(
                [_unpack(wo_v[j, pl.ds(k0 // 2, kn // 2), :]) for j in range(n_wo)], axis=1)
            return _dot(_unpack(att_v[:, pl.ds(k0, kn)]), wo)

        for g in range(ng):
            proj(g)
            if g >= 1:
                scores(g - 1)
            if g >= 2:
                attend(g - 2)
        o = outproj(0, _WO[0])
        scores(ng - 1)
        attend(ng - 2)
        o = outproj(_WO[0], _WO[1]) + o
        attend(ng - 1)
        o = outproj(_WO[1], ng) + o
        x_v[rows, :] = ((x_v[rows, :].astype(_F32) + (hh[n_mem:] + base_v[rows, :])) + o[n_mem:]).astype(_BF16)
        return o[:n_mem]

    with _scope("A"):
        def steps(i, mem):
            for j in range(_AU):
                mem = step(i * _AU + j, mem)
            rows = [_ds((i * _AU + j) * seg, early, seg) for j in range(_AU)]
            for r in rows:
                pltpu.make_async_copy(x_v.at[r], out_hbm.at[r], sem_out.at[0]).start()
            return mem

        lax.fori_loop(0, n_seg // _AU, steps, mem0)

    kh = H * E // 2
    def wo_quad(i, j):
        return lambda r, c, k, rows=_PR: wo_v[c * n_wo // 2 + j, pl.ds((r * kh + i * dh) // 2 + k, rows), :]

    def post_lhs(i, r, c, z):
        ops = _strassen_lhs(*[_after(post_v[pl.ds(a * hl + r, 32), pl.ds(b * kh + i * dh + c, 256)], z)
                              for a in range(2) for b in range(2)])
        for p in range(7):
            (a_v, a2_v)[i % 2][p, pl.ds(r // 2, 16), pl.ds(c, 256)] = _pack(ops[p])

    lhs_tiles = [(r, c) for r in range(0, hl, 32) for c in range(0, dh, 256)]
    with _scope("post"):
      fill(b0_v, wo_quad(0, 0), [zero])
      for r, c in lhs_tiles:
        post_lhs(0, r, c, zero)
      jobs = [(i, j) for i in range(kh // dh) for j in range(n_wo // 2)]
      for n, (i, j) in enumerate(jobs):
        b = operands((b0_v, b1_v)[n % 2], wo_quad(i, j))
        marks = []
        for r0 in range(0, hl, _PM):
            def prod(p):
                return _dot(_unpack((a_v, a2_v)[i % 2][p, pl.ds(r0 // 2, _PM // 2), :]), b(p))

            def done(q, v):
                idx = (pl.ds(q // 2 * hl + r0, _PM), pl.ds(q % 2 * dh + j * 128, 128))
                if i > 0:
                    v = v + acc_v[idx]
                if i + 1 < kh // dh:
                    acc_v[idx] = v
                    return
                for k in range(0, _PM, _LATE):
                    at = (pl.ds((q // 2 * hl + r0 + k) // _LATE * seg + early, _LATE), idx[1])
                    rest = x_v[at].astype(_F32) + (xn_v[at] + base_v[at])
                    x_v[at] = (rest + v[k:k + _LATE]).astype(_BF16)

            marks += [mark(v) for v in _strassen(prod, done)]
        if n + 1 < len(jobs):
            fill((b1_v, b0_v)[n % 2], wo_quad(*jobs[n + 1]), marks[:-4])
        if i + 1 < kh // dh:
            k = len(lhs_tiles) // (n_wo // 2)
            for (r, c), z in zip(lhs_tiles[j * k:(j + 1) * k], marks[3::len(marks) // k]):
                post_lhs(i + 1, r, c, z)
    for r in range(n_seg):
        rows = pl.ds(r * seg + early, _LATE)
        pltpu.make_async_copy(x_v.at[rows], out_hbm.at[rows], sem_out.at[0]).start()
    pltpu.make_async_copy(x_v, out_hbm, sem_out.at[0]).wait()


@functools.partial(jax.jit, static_argnames=("A_seg_len",))
def pallas_parallel_sum__memory_aug_recurrent_mem_tr__mixer_s_mlp__prompt_kernel(
    A_x: jax.Array,
    A_mem0: jax.Array,
    A_Wq: jax.Array,
    A_Wk: jax.Array,
    A_Wv: jax.Array,
    A_Wo: jax.Array,
    A_seg_len: int,
    B_x: jax.Array,
    B_w1: jax.Array,
    B_w2: jax.Array,
    B_w3: jax.Array,
    B_w4: jax.Array,
):
    del B_x
    B, S, D = A_x.shape
    _, H, E = A_Wq.shape
    M = A_mem0.shape[1]
    F = B_w3.shape[1]
    seg = int(A_seg_len)
    nblk = S // _TM
    assert B == 1 and S % _TM == 0 and S % seg == 0 and F % (2 * _FC) == 0 and H % _HG == 0
    assert nblk == D // 128

    hbm = pl.BlockSpec(memory_space=pltpu.HBM)
    out = pl.pallas_call(
        functools.partial(_kernel, seg=seg),
        out_shape=jax.ShapeDtypeStruct((S, D), A_x.dtype),
        in_specs=[hbm, pl.BlockSpec(memory_space=pltpu.VMEM)] + [hbm] * 8,
        out_specs=hbm,
        scratch_shapes=[
            pltpu.VMEM((S, D), _BF16),
            pltpu.VMEM((3 * H, D // 2, E), _U32),
            pltpu.VMEM((D // 128, H * E // 2, 128), _U32),
            pltpu.VMEM((S, D), _F32),
            pltpu.VMEM((S, D), _F32),
        ],
        compiler_params=pltpu.CompilerParams(vmem_limit_bytes=124 * 1024 * 1024, flags=_FLAGS),
    )(A_x.reshape(S, D), A_mem0.reshape(M, D),
      A_Wq.reshape(D * H, E), A_Wk.reshape(D * H, E), A_Wv.reshape(D * H, E),
      A_Wo.reshape(H * E, D), B_w1, B_w2, B_w3, B_w4)
    return out.reshape(B, S, D)
```

```python
import functools

import jax
import jax.numpy as jnp
import numpy as np
from jax import lax
import jax.experimental.pallas as pl
import jax.experimental.pallas.tpu as pltpu

_F32 = jnp.float32
_BF16 = jnp.bfloat16
_U32 = jnp.uint32

_TM = 256
_FC = 256
_HG = 4
_WO = (2, 4)
_PAD = 8
_NR = 16
_PW = 256
_LATE = 8
_PU = 4
_AU = 2
_PM = 64
_PR = 16
_SM = 64
_LA = 1
_NR0 = 32
_W0 = (0, 0.75)
_WS = (0.1, 0.9)
_WN = (0.02, 0.9)
_WP = (0.5, 0.98)
_SCOPES = False
_FLAGS = None


def _layernorm(x, eps=1e-5):
    m = jnp.mean(x, axis=-1, keepdims=True)
    c = x - m
    v = jnp.mean(c * c, axis=-1, keepdims=True)
    return c * lax.rsqrt(v + eps)


def _gelu(x):
    c0 = float(np.sqrt(2.0 / np.pi))
    c1 = c0 * 0.044715
    hx = 0.5 * x
    return hx + hx * jnp.tanh(x * (c0 + c1 * (x * x)))


def _dot(a, b):
    return lax.dot_general(a, b, (((1,), (0,)), ((), ())), preferred_element_type=_F32)


def _dot_nt(a, b):
    return lax.dot_general(a, b, (((1,), (1,)), ((), ())), preferred_element_type=_F32)


def _pack(x):
    return pltpu.bitcast(x.astype(_BF16), _U32)


def _unpack(w):
    return pltpu.bitcast(w, _BF16)


def _strassen_lhs(a11, a12, a21, a22):
    return a11 + a22, a21 + a22, a11, a22, a11 + a12, a21 - a11, a12 - a22


def _strassen_out(m):
    m1, m2, m3, m4, m5, m6, m7 = m
    return (m1 + m4) + (m7 - m5), m3 + m5, m2 + m4, (m1 - m2) + (m3 + m6)


def _strassen(prod, done):
    m1, m2 = prod(0), prod(1)
    c22 = m1 - m2
    m4 = prod(3)
    done(2, m2 + m4)
    c11 = m1 + m4
    c22 = prod(5) + c22
    c11 = prod(6) + c11
    m3 = prod(2)
    done(3, c22 + m3)
    m5 = prod(4)
    done(0, c11 - m5)
    done(1, m3 + m5)
    return m1, m2, m4, c22, c11, m3, m5


def _after(x, z):
    w = pltpu.bitcast(x, _U32)
    z = jnp.tile(z, (w.shape[0] // z.shape[0], w.shape[1] // z.shape[1]))
    return pltpu.bitcast(w | z, x.dtype)


class _scope:
    def __init__(self, name):
        self.c = jax.named_scope(name) if _SCOPES else None
    def __enter__(self):
        if self.c: self.c.__enter__()
    def __exit__(self, *a):
        if self.c: self.c.__exit__(*a)


def _wo_tile(heads, m, j):
    return 3 * heads + 16 * (j // 4) + 4 * m + j % 4


def _ds(start, size, align):
    return pl.ds(start if isinstance(start, int) else pl.multiple_of(start, align), size)


def _kernel(x_hbm, mem0_ref, wq_hbm, wk_hbm, wv_hbm, wo_hbm, w1_hbm, w2_hbm, w3_hbm, w4_hbm,
            out_hbm,
            x_v, wa_v, a_v, xn_v, base_v, *, seg):
    S, D = x_v.shape
    F = w3_hbm.shape[1]
    H, E = wa_v.shape[0] // 4, wa_v.shape[2]
    nblk, n_late = S // _TM, S // seg * _LATE
    mem0 = mem0_ref[...].astype(_F32)
    zero = jnp.where(jnp.abs(mem0[:8, :128]) < 0.0, 1, 0).astype(_U32)
    pl.run_scoped(
        functools.partial(_mixer, x_hbm, wq_hbm, wk_hbm, wv_hbm, wo_hbm, w1_hbm, w2_hbm, w3_hbm,
                          w4_hbm, x_v, wa_v, a_v, xn_v, base_v, zero, seg),
        pltpu.VMEM((D // 2, D), _U32),
        pltpu.VMEM((7, D // 4, D // 2), _U32),
        pltpu.VMEM((7, D // 4, D // 2), _U32),
        pltpu.VMEM((7, D // 4, F // 2), _U32),
        pltpu.VMEM((7, F // 4, D // 2), _U32),
        pltpu.VMEM((2, 3, D // nblk * H // 2, E), _U32),
        pltpu.VMEM((S + 2 * _PAD, D), _F32),
        pltpu.VMEM((2, 7, _TM // 4, D // 2), _U32),
        pltpu.VMEM((7, _TM // 4, D // 2), _U32),
        pltpu.SemaphoreType.DMA((nblk,)),
        pltpu.SemaphoreType.DMA((5,)),
        pltpu.SemaphoreType.DMA((nblk, 8)),
        pltpu.SemaphoreType.DMA((2, 3)),
        pltpu.SemaphoreType.DMA((D // 128, H * E // D)))
    pl.run_scoped(
        functools.partial(_memory, out_hbm, x_v, wa_v, a_v, xn_v, base_v, mem0, zero, seg),
        pltpu.VMEM((3 * H, 4, n_late // 4, E), _F32),
        pltpu.VMEM((4, _LATE, H * E), _F32),
        pltpu.VMEM((49, n_late // 4, H * E // 4), _F32),
        pltpu.VMEM((4, 4, n_late // 4, 128), _F32),
        pltpu.VMEM(((mem0.shape[0] + seg - _LATE) // 2, H * E), _U32),
        pltpu.VMEM((49, D // 8, 128), _U32),
        pltpu.VMEM((49, D // 8, 128), _U32),
        pltpu.VMEM((S, D), _BF16),
        pltpu.SemaphoreType.DMA((1,)))


def _mixer(x_hbm, wq_hbm, wk_hbm, wv_hbm, wo_hbm, w1_hbm, w2_hbm, w3_hbm, w4_hbm,
           x_v, wa_v, a_v, xn_v, base_v, zero, seg,
           w1raw_v, w1_v, w2_v, w3_v, w4_v, stage_v, h_v, y_v, g_v,
           sem_x, sem_w, sem_f, sem_s, sem_o):
    S, D = x_v.shape
    dh = D // 2
    fh = w3_v.shape[2]
    H, E = wa_v.shape[0] // 4, wa_v.shape[2]
    nblk = S // _TM
    th = _TM // 2
    nfc = fh // _FC
    dch = D // nblk
    n_wo = D // 128

    def x_copy(i):
        rows = _ds(i * _TM, _TM, _TM)
        return pltpu.make_async_copy(x_hbm.at[rows], x_v.at[rows], sem_x.at[i])

    quad = ((0, 0, 1), (0, 1, 2), (1, 0, 3), (1, 1, 4))

    def quad_copies(src, dst, r0, n, sems):
        _, rows, cols = dst.shape
        return [pltpu.make_async_copy(
            src.bitcast(_U32).at[_ds(r * rows + r0, n, 8), pl.ds(c * cols, cols)],
            dst.at[slot, _ds(r0, n, 8)], sems(k)) for k, (r, c, slot) in enumerate(quad)]

    def ffn_copies(c):
        cps = quad_copies(w4_hbm, w4_v, c * _FC // 2, _FC // 2, lambda k: sem_f.at[c, k])
        for k, (r, q, slot) in enumerate(quad):
            cps.append(pltpu.make_async_copy(
                w3_hbm.bitcast(_U32).at[pl.ds(r * dh // 2, dh // 2), pl.ds(q * fh + c * _FC, _FC)],
                w3_v.at[slot, :, pl.ds(c * _FC, _FC)], sem_f.at[c, 4 + k]))
        return cps

    def stage_copy(t, i):
        src = (wq_hbm, wk_hbm, wv_hbm)[t].bitcast(_U32)
        n = dch * H // 2
        return pltpu.make_async_copy(src.at[_ds(i * n, n, n)], stage_v.at[i % 2, t], sem_s.at[i % 2, t])

    def wo_copies(j):
        return [pltpu.make_async_copy(
            wo_hbm.bitcast(_U32).at[pl.ds(m * dh, dh), _ds(j * 128, 128, 128)],
            wa_v.at[_wo_tile(H, m, j)], sem_o.at[j, m]) for m in range(H * E // D)]

    w1_copy = pltpu.make_async_copy(w1_hbm.bitcast(_U32), w1raw_v, sem_w.at[4])
    w2_copies = quad_copies(w2_hbm, w2_v, 0, dh // 2, lambda k: sem_w.at[k])

    def mark(v, r=0, c=0):
        return pltpu.bitcast(v[r:r + 8, c:c + 128], _U32) & zero

    def put_lhs(slot, r, y):
        n = y.shape[0] // 2
        ops = _strassen_lhs(y[:n, :dh], y[:n, dh:], y[n:, :dh], y[n:, dh:])
        for p in range(7):
            y_v[slot, p, _ds(r // 2, n // 2, 8), :] = _pack(ops[p])

    def put_rhs(w_v, idx, quads, z, seeds=False):
        high = jnp.tile(z | _U32(0xFFFF0000), (1, quads[0].shape[1] // 128))
        sums = []
        for b11, b12, b21, b22 in ([pltpu.bitcast(q << 16, _F32) for q in quads],
                                   [pltpu.bitcast(q & high, _F32) for q in quads]):
            sums.append((b11 + b22, b12 - b22, b21 - b11, b11 + b12, b21 + b22))
        for slot, even, odd in zip((0, 2, 3, 5, 6), *sums):
            w_v[(slot,) + idx] = pltpu.pack_elementwise([even, odd], packed_dtype=_BF16)
        if seeds:
            w_v[(1,) + idx] = quads[0]
            w_v[(4,) + idx] = quads[3]

    def prep(w_v, r0, c0, nc):
        idx = (_ds(r0, 8, 8), pl.ds(c0, nc))
        return lambda z: put_rhs(w_v, idx, [w_v[(slot,) + idx] for slot in (1, 2, 3, 4)], z)

    def spread(jobs, marks):
        prev = None
        for k, job in enumerate(jobs):
            z = marks[k * len(marks) // len(jobs)]
            prev = job(z if prev is None else z | prev)

    def halves(i, r, n):
        return _ds(i * _TM + r, n, 16), _ds(i * _TM + th + r, n, 16)

    def norm_jobs(i, slot, _NR):
        def job(r, z):
            top, bot = halves(i, r, _NR)
            x = _after(jnp.concatenate([x_v[top, :], x_v[bot, :]], axis=0), z)
            xn = _layernorm(x.astype(_F32))
            xn_v[top, :] = xn[:_NR]
            xn_v[bot, :] = xn[_NR:]
            y = _layernorm(xn)
            put_lhs(slot, r, y)
            return functools.reduce(jnp.bitwise_or, [mark(y, k) for k in range(0, y.shape[0], 8)])
        return [functools.partial(job, r) for r in range(0, th, _NR)]

    def ffn_norm_jobs(i, slot):
        def job(r, z):
            top, bot = halves(i, r, _NR)
            x1 = jnp.concatenate([base_v[top, :] + xn_v[top, :], base_v[bot, :] + xn_v[bot, :]], axis=0)
            y = _layernorm(_after(x1, z))
            put_lhs(slot, r, y)
            return functools.reduce(jnp.bitwise_or, [mark(y, k) for k in range(0, y.shape[0], 8)])
        return [functools.partial(job, r) for r in range(0, th, _NR)]

    def prep_jobs(c):
        return ([prep(w4_v, c * _FC // 2 + r, k, _PW)
                 for r in range(0, _FC // 2, 8) for k in range(0, dh, _PW)]
                + [prep(w3_v, r, c * _FC + k, _PW)
                   for r in range(0, dh // 2, 8) for k in range(0, _FC, _PW)])

    corners = [(r, c) for r in (0, th) for c in (0, dh)]
    tiles = [(r, c) for r in range(0, th, _SM) for c in range(0, dh, 128)]

    def shift_jobs(i):
        def job(r0, c0, z):
            a = []
            for r, c in corners:
                sh = (-1, 1, -2, 2)[(c + c0) // (D // 4)]
                lo = 0 if sh < 0 else _PAD
                win = _after(h_v[pl.ds(i * _TM + r + r0 + lo, _SM + _PAD), pl.ds(c + c0, 128)], z)
                a.append(win[_PAD - lo + sh:_PAD - lo + sh + _SM])
            for p, v in enumerate(_strassen_lhs(*a)):
                g_v[p, pl.ds(r0 // 2, _SM // 2), pl.ds(c0, 128)] = _pack(v)
        return [functools.partial(job, r0, c0) for r0, c0 in tiles]

    def mix(lhs, w_v, out_v, row, act):
        marks = []
        for r0, c0 in tiles:
            def prod(p):
                return _dot(_unpack(lhs[p, pl.ds(r0 // 2, _SM // 2), :]),
                            _unpack(w_v[p, :, pl.ds(c0, 128)]))

            def done(q, v):
                r, c = corners[q]
                out_v[pl.ds(row + r + r0, _SM), pl.ds(c + c0, 128)] = act(v)

            marks += [mark(v) for v in _strassen(prod, done)]
        return marks

    def window(marks, w):
        return marks[int(w[0] * len(marks)):int(w[1] * len(marks))]

    x_copy(0).start()
    w1_copy.start()
    x_copy(1).start()
    h_v[pl.ds(0, _PAD), :] = jnp.zeros((_PAD, D), _F32)
    h_v[pl.ds(_PAD + S, _PAD), :] = jnp.zeros((_PAD, D), _F32)
    x_copy(0).wait()
    xn = _layernorm(x_v[pl.ds(0, _TM), :].astype(_F32))
    xn_v[pl.ds(0, _TM), :] = xn
    y_v[0, pl.ds(0, 4)] = jnp.stack(
        [_pack(_layernorm(xn))[r // 2:(r + th) // 2, c:c + dh] for r, c in corners])
    w1_copy.wait()

    for i in range(nblk + 1):
      with _scope("mix%d" % i):
        c = i - 2
        if i == 0:
            for cp in w2_copies:
                cp.start()
        if i + 2 < nblk:
            x_copy(i + 2).start()
        if 0 <= c + _LA < nfc:
            for cp in ffn_copies(c + _LA):
                cp.start()
        if i == nblk - 1:
            for t in range(3):
                stage_copy(t, 0).start()
        if i + 1 < nblk:
            x_copy(i + 1).wait()
        if i == 1:
            for cp in w2_copies:
                cp.wait()
        if 0 <= c < nfc:
            for cp in ffn_copies(c):
                cp.wait()

        if i == 0:
            marks = []
            for r in range(0, _TM, _SM):
                q = 2 * (r // th)
                y = jnp.concatenate([_unpack(y_v[0, q + k, pl.ds(r % th // 2, _SM // 2), :])
                                     for k in range(2)], axis=1)
                for k in range(0, D, 128):
                    a = _dot(y, _unpack(w1raw_v[:, pl.ds(k, 128)]))
                    h_v[pl.ds(_PAD + r, _SM), pl.ds(k, 128)] = _gelu(a)
                    marks.append(mark(a))

            def first(k, z):
                quads = [w1raw_v[pl.ds(r * dh // 2 + k, 8), pl.ds(q * dh, dh)] for r, q, _ in quad]
                put_rhs(w1_v, (pl.ds(k, 8), slice(None)), quads, z, seeds=True)

            spread([functools.partial(first, k) for k in range(0, dh // 2, 8)], marks)
            spread(norm_jobs(1, 1, _NR0), window(marks, _W0))
            continue
        marks = []
        if i < nblk:
            marks += mix(y_v.at[i % 2], w1_v, h_v, _PAD + i * _TM, _gelu)
            spread(shift_jobs(i - 1), window(marks, _WS))
        else:
            for job in shift_jobs(i - 1):
                job(zero)
        if i == 1:
            spread([prep(w2_v, k, q, _PW) for q in range(0, dh, _PW) for k in range(0, dh // 2, 8)],
                   window(marks, (0, 0.9)))
        marks += mix(g_v, w2_v, base_v, (i - 1) * _TM, lambda v: v)
        if i + 1 < nblk:
            spread(norm_jobs(i + 1, (i + 1) % 2, _NR), window(marks, _WN))
        elif i + 1 == nblk:
            spread(ffn_norm_jobs(0, 0), window(marks, _WN))
        if 0 <= c < nfc:
            spread(prep_jobs(c), window(marks, _WP if i < nblk else (0, 0.97)))

    def ffn(i, _):
        @pl.when(i + 1 < nblk)
        def _():
            for t in range(3):
                stage_copy(t, i + 1).start()
        for cp in wo_copies(i):
            cp.start()
        for t in range(3):
            stage_copy(t, i).wait()

        def retile(n, z):
            n, odd = divmod(n, 2)
            t, r, jh = n // (dch // 8), (n // 2) % (dch // 16), n % 2
            v = stage_v[i % 2, t, pl.ds(r * 8 * H, 8 * H), :].reshape(8, H, E)
            a, b = v[:, 8 * jh:8 * jh + 8], v[:, H // 2 + 8 * jh:H // 2 + 8 * jh + 8]
            low = (z | _U32(0xFFFF))[None]
            w = ((a >> 16) | (b & ~low)) if odd else ((a & low) | (b << 16))
            w = jnp.swapaxes(w, 0, 1)
            rows = _ds(i * (dch // 2) + 8 * r, 8, 8)
            for j in range(8):
                wa_v[6 * (8 * jh + j) + 3 * odd + t, rows, :] = w[j]

        pieces = list(range(3 * (dch // 16) * 4))
        u = []
        for c in range(nfc):
            g = [_dot(_unpack(y_v[i % 2, p]), _unpack(w3_v[p, :, pl.ds(c * _FC, _FC)]))
                 for p in range(7)]
            for p in range(7):
                for k in range(0, _FC, 128):
                    if pieces:
                        retile(pieces.pop(0), mark(g[p], 0, k))
            u.append([o.astype(_BF16) for o in _strassen_lhs(*[_gelu(q) for q in _strassen_out(g)])])
        assert not pieces
        m = [_dot(jnp.concatenate([uc[p] for uc in u], axis=1), _unpack(w4_v[p])) for p in range(7)]
        spread(ffn_norm_jobs(jnp.minimum(i + 1, nblk - 1), (i + 1) % 2),
               [mark(m[p], 0, k) for p in range(1, 5) for k in (0, 256)])
        for c in range(0, D // 4, 128):
            z = mark(m[5], 0, c)
            ops = _lhs49(lambda a, b: _after(jnp.concatenate(
                [xn_v[_ds(i * _TM + (4 * k + a + 1) * seg - _LATE, _LATE, _LATE), pl.ds(b * D // 4 + c, 128)]
                 for k in range(2)], axis=0), z))
            for p, v in enumerate(ops):
                a_v[p, _ds(i * _LATE, _LATE, _LATE), pl.ds(c, 128)] = _pack(v)
        for (r, c), v in zip(corners, _strassen_out(m)):
            base_v[_ds(i * _TM + r, th, th), pl.ds(c, dh)] += v
        return 0

    with _scope("ffn"):
        lax.fori_loop(0, nblk, ffn, 0)

    for j in range(n_wo):
        for cp in wo_copies(j):
            cp.wait()


class _Quad:
    def __init__(self, blocks):
        self.blocks = list(blocks)

    def __add__(self, other):
        return _Quad(a + b for a, b in zip(self.blocks, other.blocks))

    def __sub__(self, other):
        return _Quad(a - b for a, b in zip(self.blocks, other.blocks))


def _grid(get):
    return [_Quad(get(2 * i + r, 2 * j + c) for r in range(2) for c in range(2))
            for i in range(2) for j in range(2)]


_RHS_TERMS = ((0, 1, 3), (0, 0, 0), (1, -1, 3), (2, -1, 0), (3, 0, 3), (0, 1, 1), (2, 1, 3))


def _rhs_term(get, p):
    a, sign, b = _RHS_TERMS[p]
    return get(a) if sign == 0 else get(a) + get(b) if sign > 0 else get(a) - get(b)


def _lhs49(get):
    return [v for q in _strassen_lhs(*_grid(get)) for v in _strassen_lhs(*q.blocks)]


def _rhs7(word, p, z):
    words = [[word(2 * (n // 2) + k // 2, 2 * (n % 2) + k % 2) for k in range(4)]
             if n in (_RHS_TERMS[p][0], _RHS_TERMS[p][2]) else None for n in range(4)]
    shift, high = z | _U32(16), z | _U32(0xFFFF0000)
    halves = []
    for half in (lambda w: w << shift, lambda w: w & high):
        q = _rhs_term(lambda n: _Quad(pltpu.bitcast(half(w), _F32) for w in words[n]), p)
        halves.append([_rhs_term(lambda n: q.blocks[n], k) for k in range(7)])
    return [pltpu.pack_elementwise([e, o], packed_dtype=_BF16) for e, o in zip(*halves)]


def _strassen49(prod, done):
    seen = []

    def outer(p):
        out = [None] * 4
        seen.extend(_strassen(lambda k: prod(7 * p + k), out.__setitem__))
        return _Quad(out)

    def finish(n, q):
        for k, v in enumerate(q.blocks):
            done(2 * (n // 2) + k // 2, 2 * (n % 2) + k % 2, v)

    _strassen(outer, finish)
    return seen


def _memory(out_hbm, x_v, wa_v, a_v, xn_v, base_v, mem0, zero, seg,
            pre_v, post_v, a2_v, acc_v, att_v, b0_v, b1_v, fin_v, sem_out):
    S, D = x_v.shape
    dh, dq = D // 2, D // 4
    H, E = wa_v.shape[0] // 4, wa_v.shape[2]
    n_wo = D // 128
    n_mem = mem0.shape[0]
    n_seg = S // seg
    early = seg - _LATE
    ql = n_seg * _LATE // 4

    def mark(v):
        return pltpu.bitcast(v[:8, :128], _U32) & zero

    def spread(jobs, marks):
        for k, job in enumerate(jobs):
            job(marks[k * len(marks) // len(jobs)])

    def fill(b_v, n, marks):
        def job(p, k, z):
            word = lambda r, c: wa_v[n + c, pl.ds(r * dq // 2 + k, 8), :]
            for j, w in enumerate(_rhs7(word, p, z)):
                b_v[7 * p + j, pl.ds(k, 8), :] = w
        spread([functools.partial(job, p, k) for p in (0, 1, 3, 5, 6, 2, 4)
                for k in range(0, dq // 2, 8)], marks)

    def project(n0, lhs, done):
        for j in range(4):
            b_v, marks = (b0_v, b1_v)[j % 2], []
            for r0 in range(0, ql, _PM):
                marks += [mark(v) for v in _strassen49(
                    lambda p: _dot(lhs(j, p, r0), _unpack(b_v[p])),
                    lambda r, c, v: done(j, r, c, r0, v))]
            fill((b1_v, b0_v)[j % 2], jnp.minimum(n0 + 4 * j + 4, 4 * H - 4), marks[:-4])

    fill(b0_v, 0, [zero])

    def pre(i, _):
        def done(j, r, c, r0, v):
            pre_v[16 * i + 4 * j + c, r, pl.ds(r0, _PM), :] = v

        project(16 * i, lambda j, p, r0: _unpack(a_v[p, pl.ds(r0 // 2, _PM // 2), :]), done)
        return 0

    with _scope("pre"):
        lax.fori_loop(0, 3 * H // 16, pre, 0)

    L = n_mem + seg
    row = lax.broadcasted_iota(jnp.int32, (L, L), 0)
    col = lax.broadcasted_iota(jnp.int32, (L, L), 1)
    mask = (row < n_mem) | (row >= col)
    scale = float(E) ** -0.5

    def step(i, r, mem):
        rows = _ds((4 * i + r) * seg, early, seg)
        hh = jnp.concatenate([mem, xn_v[rows, :]], axis=0)
        hb = hh.astype(_BF16)
        ng = H // _HG
        qkv, sc = {}, {}

        def proj(g):
            tiles = range(3 * _HG * g, 3 * _HG * (g + 1))
            w = jnp.concatenate([_unpack(wa_v[n]) for n in tiles], axis=1)
            if g == 0:
                y = _dot(hb[:, :dh], w[:dh])
                y = _dot(hb[:, dh:], w[dh:]) + y
            else:
                y = _dot(hb, w)
            qkv[g] = jnp.concatenate(
                [y, jnp.concatenate([pre_v[n, r, _ds(i * _LATE, _LATE, _LATE), :] for n in tiles], axis=1)], axis=0)

        def scores(g):
            y = qkv[g]
            sc[g] = [_dot_nt(y[:, (3 * n) * E:(3 * n + 1) * E],
                             y[:, (3 * n + 1) * E:(3 * n + 2) * E].astype(_BF16))
                     for n in range(_HG)]

        def attend(g):
            y = qkv[g]
            for n in range(_HG):
                z = jnp.where(mask, sc[g][n] * scale, -1e9)
                e = jnp.exp(z - jnp.max(z, axis=-1, keepdims=True))
                inv = 1.0 / jnp.sum(e, axis=-1, keepdims=True)
                o = _dot(e * inv, y[:, (3 * n + 2) * E:(3 * n + 3) * E].astype(_BF16))
                cols = pl.ds((g * _HG + n) * E, E)
                att_v[:, cols] = _pack(o[:L - _LATE])
                post_v[r, :, cols] = o[L - _LATE:]

        def outproj(g0, g1):
            k0, kn, w = g0 * _HG * E, (g1 - g0) * _HG * E, _HG * E
            wo = jnp.concatenate([jnp.concatenate(
                [_unpack(wa_v[_wo_tile(H, k // D, j), pl.ds(k % D // 2, w // 2), :])
                 for k in range(k0, k0 + kn, w)], axis=0) for j in range(n_wo)], axis=1)
            return _dot(_unpack(att_v[:, pl.ds(k0, kn)]), wo)

        for g in range(ng):
            proj(g)
            if g >= 1:
                scores(g - 1)
            if g >= 2:
                attend(g - 2)
        o = outproj(0, _WO[0])
        scores(ng - 1)
        attend(ng - 2)
        o = outproj(_WO[0], _WO[1]) + o
        attend(ng - 1)
        o = outproj(_WO[1], ng) + o
        x_v[rows, :] = ((x_v[rows, :].astype(_F32) + (hh[n_mem:] + base_v[rows, :])) + o[n_mem:]).astype(_BF16)
        return o[:n_mem]

    with _scope("A"):
        def steps(i, mem):
            for r in range(4):
                mem = step(i, r, mem)
            for m in range(H * E // D):
                for c in range(0, dq, 128):
                    ops = _lhs49(lambda a, b: post_v[a, :, pl.ds(m * D + b * dq + c, 128)])
                    for p, v in enumerate(ops):
                        a2_v[p, _ds(i * _LATE, _LATE, _LATE), pl.ds(m * dq + c, 128)] = v
            for r in range(4):
                rows = _ds((4 * i + r) * seg, early, seg)
                pltpu.make_async_copy(x_v.at[rows], out_hbm.at[rows], sem_out.at[0]).start()
            return mem

        lax.fori_loop(0, n_seg // 4, steps, mem0)

    def post(i, _):
        def done(m, r, c, r0, v):
            idx = (r, c, pl.ds(r0, _PM), slice(None))
            if m > 0:
                v = v + acc_v[idx]
            if m < 3:
                acc_v[idx] = v
                return
            for k in range(0, _PM, _LATE):
                at = (pl.ds((4 * (r0 + k) // _LATE + r) * seg + early, _LATE),
                      _ds((4 * i + c) * 128, 128, 128))
                rest = x_v[at].astype(_F32) + (xn_v[at] + base_v[at])
                fin_v[at] = (rest + v[k:k + _LATE]).astype(_BF16)

        project(3 * H + 16 * i, lambda m, p, r0: a2_v[p, pl.ds(r0, _PM), pl.ds(m * dq, dq)], done)
        for r in range(n_seg):
            at = (pl.ds(r * seg + early, _LATE), _ds(i * dh, dh, dh))
            pltpu.make_async_copy(fin_v.at[at], out_hbm.at[at], sem_out.at[0]).start()
        return 0

    with _scope("post"):
        lax.fori_loop(0, 2, post, 0)
    pltpu.make_async_copy(x_v, out_hbm, sem_out.at[0]).wait()


@functools.partial(jax.jit, static_argnames=("A_seg_len",))
def pallas_parallel_sum__memory_aug_recurrent_mem_tr__mixer_s_mlp__prompt_kernel(
    A_x: jax.Array,
    A_mem0: jax.Array,
    A_Wq: jax.Array,
    A_Wk: jax.Array,
    A_Wv: jax.Array,
    A_Wo: jax.Array,
    A_seg_len: int,
    B_x: jax.Array,
    B_w1: jax.Array,
    B_w2: jax.Array,
    B_w3: jax.Array,
    B_w4: jax.Array,
):
    del B_x
    B, S, D = A_x.shape
    _, H, E = A_Wq.shape
    M = A_mem0.shape[1]
    F = B_w3.shape[1]
    seg = int(A_seg_len)
    nblk = S // _TM
    assert B == 1 and S % _TM == 0 and S % seg == 0 and F % (2 * _FC) == 0 and H % _HG == 0
    assert nblk == D // 128

    hbm = pl.BlockSpec(memory_space=pltpu.HBM)
    out = pl.pallas_call(
        functools.partial(_kernel, seg=seg),
        out_shape=jax.ShapeDtypeStruct((S, D), A_x.dtype),
        in_specs=[hbm, pl.BlockSpec(memory_space=pltpu.VMEM)] + [hbm] * 8,
        out_specs=hbm,
        scratch_shapes=[
            pltpu.VMEM((S, D), _BF16),
            pltpu.VMEM((4 * H, D // 2, E), _U32),
            pltpu.VMEM((49, S // seg * _LATE // 8, D // 4), _U32),
            pltpu.VMEM((S, D), _F32),
            pltpu.VMEM((S, D), _F32),
        ],
        compiler_params=pltpu.CompilerParams(vmem_limit_bytes=124 * 1024 * 1024, flags=_FLAGS),
    )(A_x.reshape(S, D), A_mem0.reshape(M, D),
      A_Wq.reshape(D * H, E), A_Wk.reshape(D * H, E), A_Wv.reshape(D * H, E),
      A_Wo.reshape(H * E, D), B_w1, B_w2, B_w3, B_w4)
    return out.reshape(B, S, D)
```

```python
import functools

import jax
import jax.numpy as jnp
import numpy as np
from jax import lax
import jax.experimental.pallas as pl
import jax.experimental.pallas.tpu as pltpu

_F32 = jnp.float32
_BF16 = jnp.bfloat16
_U32 = jnp.uint32

_TM = 256
_FC = 512
_HG = 4
_WO = (2, 4)
_PAD = 8
_NR = 16
_PW = 256
_LATE = 8
_PU = 4
_AU = 2
_PM = 64
_PR = 16
_SM = 64
_LA = 1
_NR0 = 16
_W0 = (0, 0.75)
_WS = (0.1, 0.9)
_WN = (0.02, 0.8)
_WP = (0.45, 0.95)
_WL = (0, 0.5)
_FR = 32
_RD = 160
_RS = 0.6
_CS = 1
_N1 = 5
_HS = 0.35
_TU = 0
_TP = 21
_HE = 2
_HM = 2
_SCOPES = False
_ONLYB = False
_FLAGS = None


def _layernorm(x, eps=1e-5):
    m = jnp.mean(x, axis=-1, keepdims=True)
    c = x - m
    v = jnp.mean(c * c, axis=-1, keepdims=True)
    return c * lax.rsqrt(v + eps)


def _layernorm_twice(load, eps=1e-5):
    m = jnp.mean(load(0), axis=-1, keepdims=True)
    c = load(1) - m
    mu = jnp.mean(c, axis=-1, keepdims=True)
    v = jnp.mean(c * c, axis=-1, keepdims=True)
    r = lax.rsqrt(v + eps)
    r2 = r * lax.rsqrt((r * r) * jnp.maximum(v - mu * mu, 0.0) + eps)
    c = load(2) - m
    return c * r, (c - mu) * r2


def _gelu(x):
    c0 = float(np.sqrt(2.0 / np.pi))
    c1 = c0 * 0.044715
    hx = 0.5 * x
    return hx + hx * jnp.tanh(x * (c0 + c1 * (x * x)))


def _dot(a, b):
    return lax.dot_general(a, b, (((1,), (0,)), ((), ())), preferred_element_type=_F32)


def _dot_nt(a, b):
    return lax.dot_general(a, b, (((1,), (1,)), ((), ())), preferred_element_type=_F32)


def _pack(x):
    return pltpu.bitcast(x.astype(_BF16), _U32)


def _unpack(w):
    return pltpu.bitcast(w, _BF16)


def _strassen_lhs(a11, a12, a21, a22):
    return a11 + a22, a21 + a22, a11, a22, a11 + a12, a21 - a11, a12 - a22


def _strassen_out(m):
    m1, m2, m3, m4, m5, m6, m7 = m
    return (m1 + m4) + (m7 - m5), m3 + m5, m2 + m4, (m1 - m2) + (m3 + m6)


def _strassen(prod, done):
    m1, m2 = prod(0), prod(1)
    c22 = m1 - m2
    m4 = prod(3)
    done(2, m2 + m4)
    c11 = m1 + m4
    c22 = prod(5) + c22
    c11 = prod(6) + c11
    m3 = prod(2)
    done(3, c22 + m3)
    m5 = prod(4)
    done(0, c11 - m5)
    done(1, m3 + m5)
    return m1, m2, m4, c22, c11, m3, m5


def _after(x, z):
    w = pltpu.bitcast(x, _U32)
    z = jnp.tile(z, (w.shape[0] // z.shape[0], w.shape[1] // z.shape[1]))
    return pltpu.bitcast(w | z, x.dtype)


class _scope:
    def __init__(self, name):
        self.c = jax.named_scope(name) if _SCOPES else None
    def __enter__(self):
        if self.c: self.c.__enter__()
    def __exit__(self, *a):
        if self.c: self.c.__exit__(*a)


def _pair(even, odd):
    return pltpu.pack_elementwise([even, odd], packed_dtype=_BF16)


def _split(w):
    return pltpu.bitcast(w << 16, _F32), pltpu.bitcast(w & _U32(0xFFFF0000), _F32)


def _get(ref, rows):
    return jnp.concatenate([ref[k, rows, :] for k in range(ref.shape[0])], axis=1)


def _put(ref, rows, c0, x):
    for c in range(0, x.shape[1], 128):
        ref[(c0 + c) // 128, rows, :] = x[:, c:c + 128]


def _wo_tile(heads, m, j):
    return 3 * heads + 16 * (j // 4) + 4 * m + j % 4


def _ds(start, size, align):
    return pl.ds(start if isinstance(start, int) else pl.multiple_of(start, align), size)


def _kernel(x_hbm, mem0_ref, wq_hbm, wk_hbm, wv_hbm, wo_hbm, w1_hbm, w2_hbm, w3_hbm, w4_hbm,
            out_hbm,
            x_v, wa_v, a_v, xn_v, ffn_v, b0_v, b1_v, *, seg):
    S, D = x_v.shape
    F = w3_hbm.shape[1]
    H, E = wa_v.shape[0] // 4, wa_v.shape[2]
    nblk, n_late = S // _TM, S // seg * _LATE
    mem0 = mem0_ref[...].astype(_F32)
    zero = jnp.where(jnp.abs(mem0[:8, :128]) < 0.0, 1, 0).astype(_U32)
    pl.run_scoped(
        functools.partial(_mixer, x_hbm, wq_hbm, wk_hbm, wv_hbm, wo_hbm, w1_hbm, w2_hbm, w3_hbm,
                          w4_hbm, x_v, wa_v, a_v, xn_v, ffn_v, b0_v, b1_v, zero, seg),
        pltpu.VMEM((7, D // 4, D // 2), _U32),
        pltpu.VMEM((7, D // 4, D // 2), _U32),
        pltpu.VMEM((2, D // 2, _FC), _U32),
        pltpu.VMEM((2, _FC // 2, D), _U32),
        pltpu.VMEM((49, S // 8, D // 4), _U32),
        pltpu.VMEM((2, 3, _RD * H // 2, E), _U32),
        pltpu.VMEM((D // 128, S + 2 * _PAD, 128), _F32),
        pltpu.VMEM((2, 7, _TM // 4, D // 2), _U32),
        pltpu.VMEM((7, _TM // 4, D // 2), _U32),
        pltpu.VMEM((D // 128, _TM, 128), _F32),
        pltpu.VMEM((D // 128, _TM, 128), _F32),
        pltpu.VMEM((D // 128, _TM, 128), _F32),
        pltpu.SMEM((1,), jnp.int32),
        pltpu.SemaphoreType.DMA((nblk,)),
        pltpu.SemaphoreType.DMA((6,)),
        pltpu.SemaphoreType.DMA((2, 2)),
        pltpu.SemaphoreType.DMA((2, 3)),
        pltpu.SemaphoreType.DMA((D // 128, H * E // D)))
    if _ONLYB:
        def keep(sem):
            k = lax.iota(jnp.int32, 1)[0] if False else 0
            def body(i, _):
                v = pltpu.bitcast(wa_v[i, :8, :] | a_v[i, :8, :128], _F32) + xn_v[i, :8, :] + ffn_v[i, 0, :8, :128]
                x_v[:8, :128] = v.astype(_BF16)
                return 0
            lax.fori_loop(0, 7, body, 0)
            c = pltpu.make_async_copy(x_v, out_hbm, sem); c.start(); c.wait()
        pl.run_scoped(keep, pltpu.SemaphoreType.DMA)
        return
    pl.run_scoped(
        functools.partial(_memory, out_hbm, x_v, wa_v, a_v, xn_v, ffn_v, b0_v, b1_v, mem0, zero, seg),
        pltpu.VMEM((3 * H, 2, n_late // 4, E), _U32),
        pltpu.VMEM((4, _LATE, H * E), _F32),
        pltpu.VMEM((49, n_late // 4, H * E // 4), _F32),
        pltpu.VMEM((4, 4, n_late // 4, 128), _F32),
        pltpu.VMEM(((mem0.shape[0] + seg - _LATE) // 2, H * E), _U32),
        pltpu.VMEM((S, D), _BF16),
        pltpu.SemaphoreType.DMA((1,)))


def _mixer(x_hbm, wq_hbm, wk_hbm, wv_hbm, wo_hbm, w1_hbm, w2_hbm, w3_hbm, w4_hbm,
           x_v, wa_v, a_v, xn_v, ffn_v, b0_v, b1_v, zero, seg,
           w1_v, w2_v, w3_v, w4_v, f_v, stage_v, h_v, y_v, g_v, t0_v, t1_v, t2_v, nil_s,
           sem_x, sem_w, sem_f, sem_s, sem_o):
    S, D = x_v.shape
    dh = D // 2
    dq, tq = D // 4, _TM // 4
    H, E = wa_v.shape[0] // 4, wa_v.shape[2]
    nblk = S // _TM
    th = _TM // 2
    nfc = w3_hbm.shape[1] // _FC
    n_wo = D // 128

    def x_copy(i):
        rows = _ds(i * _TM, _TM, _TM)
        return pltpu.make_async_copy(x_hbm.at[rows], x_v.at[rows], sem_x.at[i])

    quad = ((0, 0, 1), (0, 1, 2), (1, 0, 3), (1, 1, 4))

    def w3_copy(c):
        src = w3_hbm.bitcast(_U32).at[:, _ds(c * _FC, _FC, _FC)]
        return pltpu.make_async_copy(src, w3_v.at[c % 2], sem_f.at[c % 2, 0])

    def w4_copy(c):
        src = w4_hbm.bitcast(_U32).at[_ds(c * _FC // 2, _FC // 2, _FC // 2)]
        return pltpu.make_async_copy(src, w4_v.at[c % 2], sem_f.at[c % 2, 1])

    def retile_row(c):
        return jnp.minimum(c * _RD, D - _RD) if not isinstance(c, int) else min(c * _RD, D - _RD)

    def stage_copy(t, c):
        src = (wq_hbm, wk_hbm, wv_hbm)[t].bitcast(_U32)
        rows = _ds(retile_row(c) * H // 2, _RD * H // 2, 8 * H)
        return pltpu.make_async_copy(src.at[rows], stage_v.at[c % 2, t], sem_s.at[c % 2, t])

    def wo_copies(j):
        return [pltpu.make_async_copy(
            wo_hbm.bitcast(_U32).at[pl.ds(m * dh, dh), _ds(j * 128, 128, 128)],
            wa_v.at[_wo_tile(H, m, j)], sem_o.at[j, m]) for m in range(H * E // D)]

    w1_copies = [pltpu.make_async_copy(w1_hbm.bitcast(_U32).at[:, pl.ds(k * dh, dh)], w3_v.at[k],
                                       sem_w.at[4 + k]) for k in range(2)]
    w2_copies = [pltpu.make_async_copy(w2_hbm.bitcast(_U32).at[pl.ds(k * dq, dq)], w4_v.at[k],
                                       sem_w.at[k]) for k in range(2)]

    def mark(v, r=0, c=0):
        return pltpu.bitcast(v[r:r + 8, c:c + 128], _U32) & zero

    def put_rhs(w_v, idx, quads, z, seeds=False):
        high = jnp.tile(z | _U32(0xFFFF0000), (1, quads[0].shape[1] // 128))
        sums = []
        for b11, b12, b21, b22 in ([pltpu.bitcast(q << 16, _F32) for q in quads],
                                   [pltpu.bitcast(q & high, _F32) for q in quads]):
            sums.append((b11 + b22, b12 - b22, b21 - b11, b11 + b12, b21 + b22))
        for slot, even, odd in zip((0, 2, 3, 5, 6), *sums):
            w_v[(slot,) + idx] = pltpu.pack_elementwise([even, odd], packed_dtype=_BF16)
        if seeds:
            w_v[(1,) + idx] = quads[0]
            w_v[(4,) + idx] = quads[3]

    jobs_left = []

    def spread(jobs, marks, share=1.0, prev=None):
        if share < 1:
            jobs_left.append(jobs[int(share * len(jobs)):])
            jobs = jobs[:int(share * len(jobs))]
        for k, job in enumerate(jobs):
            z = marks[k * len(marks) // len(jobs)]
            prev = job(z if prev is None else z | prev)
        return prev

    def halves(i, r, n):
        return _ds(i * _TM + r, n, 16), _ds(i * _TM + th + r, n, 16)

    def norm(rows, z):
        nil = nil_s[0]

        def load(k):
            w = [pltpu.bitcast(x_v[_ds(r + 16 * k * nil, 16, 16), :], _U32) for r in rows]
            return jnp.concatenate([h for v in w for h in _split(v if k else _after(v, z))], axis=0)

        xn, y = _layernorm_twice(load)
        for k, r in enumerate(rows):
            for odd in range(2):
                _put(xn_v, pl.ds(r + odd, 8, stride=2), 0, xn[16 * k + 8 * odd:16 * k + 8 * odd + 8])
        return y

    def put_lhs(slot, r, y):
        even, odd = (_strassen_lhs(y[k:k + 8, :dh], y[k:k + 8, dh:], y[k + 16:k + 24, :dh],
                                   y[k + 16:k + 24, dh:]) for k in (0, 8))
        for p in range(7):
            y_v[slot, p, pl.ds(r // 2, 8), :] = _pair(even[p], odd[p])

    def norm_jobs(i, slot):
        def job(r, z):
            y = norm((i * _TM + r, i * _TM + th + r), z)
            put_lhs(slot, r, y)
            return functools.reduce(jnp.bitwise_or, [mark(y, k) for k in range(0, y.shape[0], 8)])
        return [functools.partial(job, r) for r in range(0, th, 16)]

    def ffn_norm_jobs(i):
        t_v, nil = (t0_v, t1_v)[i % 2], nil_s[0]

        def ln(r, z):
            def load(tag):
                return [t_v[c + nil * tag, pl.ds(r, _FR), :] for c in range(D // 128)]

            def mean(parts):
                return jnp.sum(functools.reduce(jnp.add, parts), axis=-1, keepdims=True) * (1.0 / D)

            x1 = load(1)
            m = mean([_after(x1[0], z)] + x1[1:])
            inv = lax.rsqrt(mean([(e - m) * (e - m) for e in load(2)]) + 1e-5)
            for c, e in enumerate(load(3)):
                e = (e - m) * inv
                t2_v[c, pl.ds(r, _FR), :] = e
            return _any([mark(e, k) for k in range(0, _FR, 8)])

        def sums(r, c, p, z):
            r0 = r // 32 * 32 + r % 32 // 16
            lo, hi = (list(_lhs7(lambda a, b: _after(
                t2_v[(b * dq + c) // 128, pl.ds(a * tq + r0 + k, 8, stride=4), :], z), p))
                for k in (0, 2))
            for k in range(7):
                lo[k] = _pair(lo[k], hi[k])
                f_v[7 * p + k, pl.ds((i * tq + r) // 2, 8), pl.ds(c, 128)] = lo[k]
            return _any(lo) & zero if _CS else None

        return ([functools.partial(ln, a * tq + r) for r in range(0, tq, _FR) for a in range(4)],
                [functools.partial(sums, r, c, p)
                 for r in range(0, tq, 16) for c in range(0, dq, 128) for p in range(7)])

    def late_jobs(i):
        def job(c, z):
            ops = _lhs49(lambda a, b: _after(jnp.concatenate(
                [xn_v[(b * dq + c) // 128, _ds(i * _TM + (4 * k + a + 1) * seg - _LATE, _LATE, _LATE), :]
                 for k in range(2)], axis=0), z))
            for p, v in enumerate(ops):
                a_v[p, _ds(i * _LATE, _LATE, _LATE), pl.ds(c, 128)] = _pack(v)
        return [functools.partial(job, c) for c in range(0, dq, 128)]

    def w3_jobs(c):
        return _fill_jobs(b0_v, lambda r, k, j: w3_v[c % 2, pl.ds(r * dq // 2 + j, 8), pl.ds(k * 128, 128)])

    def w4_jobs(c, log):
        return _fill_jobs(b1_v, lambda r, k, j: w4_v[c % 2, pl.ds(r * 64 + j % 64, 8),
                                                     pl.ds(k * dq + j // 64 * 128, 128)], log)

    corners = [(r, c) for r in (0, th) for c in (0, dh)]
    tiles = [(r, c) for r in range(0, th, _SM) for c in range(0, dh, 128)]

    def shift_jobs(i, combine=_strassen_lhs):
        def job(r0, c0, z):
            def load(r, c, odd):
                sh = (-1, 1, -2, 2)[(c + c0) // (D // 4)]
                rows = pl.ds(i * _TM + _PAD + r + r0 + sh + odd, _SM // 2, stride=2)
                return _after(h_v[(c + c0) // 128, rows, :], z)

            even, odd = (combine(*[load(r, c, k) for r, c in corners]) for k in range(2))
            for p in range(len(even)):
                g_v[p, pl.ds(r0 // 2, _SM // 2), pl.ds(c0, 128)] = _pair(even[p], odd[p])
        return [functools.partial(job, r0, c0) for r0, c0 in tiles]

    def mix(lhs, w_v, put):
        marks = []
        for r0, c0 in tiles:
            def prod(p):
                return _dot(_unpack(lhs[p, pl.ds(r0 // 2, _SM // 2), :]),
                            _unpack(w_v[p, :, pl.ds(c0, 128)]))

            def done(q, v):
                r, c = corners[q]
                put(r + r0, c + c0, v)

            marks += [mark(v) for v in _strassen(prod, done)]
        return marks

    def window(marks, w):
        return marks[int(w[0] * len(marks)):int(w[1] * len(marks))]

    def plain(lhs, rhs, put, c0, c1):
        marks = []
        for k in range(c0, c1, 128):
            for r0 in range(0, th, _SM):
                for q in (2, 0):
                    y = jnp.concatenate([_unpack(lhs[q + n, pl.ds(r0 // 2, _SM // 2), :])
                                         for n in range(2)], axis=1)
                    a = _dot(y, _unpack(rhs(k)))
                    put(q // 2 * th + r0, k, a)
                    marks.append(mark(a))
        return marks

    def rhs_jobs(w_v, word):
        def job(k, c, z):
            put_rhs(w_v, (pl.ds(k, 8), pl.ds(c, _PW)), [word(r, q, k, c) for r, q, _ in quad], z, True)
        return [functools.partial(job, k, c) for c in range(0, dh, _PW) for k in range(0, dh // 2, 8)]

    nil_s[0] = 0
    x_copy(0).start()
    w1_copies[0].start()

    for r in (0, _PAD + S):
        _put(h_v, pl.ds(r, _PAD), 0, jnp.zeros((_PAD, D), _F32))
    x_copy(0).wait()
    x_copy(1).start()
    w1_copies[1].start()
    y0 = norm(range(0, _TM, 16), zero)
    for r in range(0, _TM, 16):
        for k in range(2):
            y_v[0, 2 * (r // th) + k, pl.ds(r % th // 2, 8), :] = _pair(
                y0[r:r + 8, k * dh:(k + 1) * dh], y0[r + 8:r + 16, k * dh:(k + 1) * dh])

    def mix_stage(i):
      with _scope("mix%d" % i):
        def put_h(r, c, v):
            _put(h_v, pl.ds(_PAD + i * _TM + r, _SM), c, _gelu(v))

        if i == 0:
            w1_copies[0].wait()
            x_copy(1).wait()
            x_copy(2).start()
            marks = plain(y_v.at[0], lambda k: w3_v[0, :, pl.ds(k, 128)], put_h, 0, dh)
            jobs = norm_jobs(1, 1)
            spread(jobs[:_N1], marks[:12])
            w1_copies[1].wait()
            for cp in w2_copies:
                cp.start()
            x_copy(3).start()
            marks = plain(y_v.at[0], lambda k: w3_v[1, :, pl.ds(k - dh, 128)], put_h, dh, D)
            spread(rhs_jobs(w1_v, lambda r, q, k, c: w3_v[q, pl.ds(r * dq + k, 8), pl.ds(c, _PW)]), marks)
            spread(jobs[_N1:], marks[:12])
            return
        marks = []
        if i == 1:
            x_copy(2).wait()
        if i == 2:
            for k in range(4, nblk):
                x_copy(k).wait()
            w3_copy(0).wait()
            w3_copy(1).start()
            w4_copy(0).start()
            for t in range(3):
                stage_copy(t, 0).start()
            for j in range(n_wo):
                for cp in wo_copies(j):
                    cp.start()
        if i < nblk:
            marks += mix(y_v.at[i % 2], w1_v, put_h)
            spread(shift_jobs(i - 1, _strassen_lhs if i > 1 else lambda *q: q), window(marks, _WS))
        else:
            for job in shift_jobs(i - 1):
                job(zero)
        if i == 1:
            spread(norm_jobs(2, 0), window(marks, (0, 0.8)))
            for cp in w2_copies:
                cp.wait()
            x_copy(3).wait()
            for k in range(4, nblk):
                x_copy(k).start()
            w3_copy(0).start()

        held = {}

        def put_base(r, c, v):
            v = v + xn_v[c // 128, pl.ds((i - 1) * _TM + r, _SM), :]
            (t1_v, t0_v)[i % 2][c // 128, pl.ds(r, _SM), :] = v
            quadrant = 2 * (r // th) + c // dh
            key = (r % th, c % dh)
            held[key, quadrant] = v
            seeds = {0: [(6, v)], 1: [(2, v)], 2: [(1, v)], 3: []}[quadrant]
            if quadrant and all((key, n) in held for n in (1, 2, 3)):
                seeds.append((5, held[key, 3] + (held[key, 2] - held[key, 1])))
            for p, w in seeds:
                ffn_v[p, 2 * (r % th // tq) + c % dh // dq, pl.ds((i - 1) * tq + r % tq, _SM),
                      pl.ds(c % dq, 128)] = w

        if i == 1:
            marks = plain(g_v, lambda k: jnp.concatenate(
                [w4_v[n, :, pl.ds(k, 128)] for n in range(2)], axis=0), put_base, 0, D)
            spread(rhs_jobs(w2_v, lambda r, q, k, c: w4_v[r, pl.ds(k, 8), pl.ds(q * dh + c, _PW)]), marks)
            return
        marks += mix(g_v, w2_v, put_base)
        jobs = norm_jobs(i + 1, (i + 1) % 2) if i + 1 < nblk else []
        if i + 1 == nblk:
            spread(w3_jobs(0), window(marks, _WN))
        if i >= 2:
            ln, sums = ffn_norm_jobs(i - 2)
            jobs = [job for pair in zip(ln, jobs) for job in pair] if jobs else ln
        spread(jobs, window(marks, _WN if i + 1 < nblk else (0, 0.55)), prev=carry.pop())
        carry.append(spread(sums, window(marks, _WP)) if i >= 2 else None)

    carry = [None]
    for i in range(nblk + 1):
        mix_stage(i)
    for jobs in ffn_norm_jobs(nblk - 1):
        for job in jobs:
            job(zero)

    def ffn(c, _):
        @pl.when(c + 1 < nfc)
        def _():
            for t in range(3):
                stage_copy(t, c + 1).start()
            w4_copy(c + 1).start()
            w3_copy(c + 1).wait()

        @pl.when(c + 2 < nfc)
        def _():
            w3_copy(c + 2).start()

        w4_copy(c).wait()
        for t in range(3):
            stage_copy(t, c).wait()

        def retile(t, r, jh, odd, z):
            v = stage_v[c % 2, t, pl.ds(r * H, 8 * H), :].reshape(8, H, E)
            a, b = v[:, 8 * jh:8 * jh + 8], v[:, H // 2 + 8 * jh:H // 2 + 8 * jh + 8]
            low = (z | _U32(0xFFFF))[None]
            w = ((a >> 16) | (b & ~low)) if odd else ((a & low) | (b << 16))
            w = jnp.swapaxes(w, 0, 1)
            rows = _ds(retile_row(c) // 2 + r, 8, 8)
            for j in range(8):
                wa_v[6 * (8 * jh + j) + 3 * odd + t, rows, :] = w[j]

        def hidden_jobs(r0, hid):
            def act(a, b, z):
                hid[a, b] = _gelu(_after(hid[a, b], z))

            def put(r, p, z):
                r1 = r // 32 * 32 + r % 32 // 2
                even, odd = (_lhs7(lambda a, b: _after(hid[a, b][k:k + 8], z), p) for k in (r1, r1 + 16))
                for k in range(7):
                    h_v[p, pl.ds(k * S // 8 + (r0 + r) // 2, 8), :] = pltpu.bitcast(
                        _pair(even[k], odd[k]), _F32)

            return ([functools.partial(act, a, b) for a in range(_HE) for b in range(4)],
                    [functools.partial(put, r, p) for p in (0, 1, 3, 5, 6, 2, 4) for r in range(0, tq, 16)])

        def hidden(jobs, marks):
            spread(jobs[0], window(marks, (0.03, _HS)))
            spread(jobs[1], window(marks, (_HS, 0.98)))

        marks, jobs, log, wait = [], None, [], None
        fills = w4_jobs(c, log)
        for r0 in range(0, S // 4, tq):
            hid = {}

            def lhs(p):
                w = f_v[p, pl.ds(r0 // 2, tq // 2), :]
                return _unpack(w if p != _TP or wait is None else _after(w, wait))

            seen = [mark(v) for v in _strassen49(
                lambda p: _dot(lhs(p), _unpack(b0_v[p])),
                lambda a, b, v: hid.__setitem__((a, b), v if a < _HE else _gelu(v)))]
            if jobs:
                hidden(jobs, seen)
            n = len(fills) // 7
            if fills[r0 // tq * n:]:
                spread(fills[r0 // tq * n:][:n], seen)
            wait = _any(log) & zero if log and _TU else None
            log.clear()
            jobs = hidden_jobs(r0, hid)
            marks += seen
        spread([functools.partial(retile, t, r, jh, odd) for t in range(3)
                for r in range(0, _RD // 2, 8) for jh in range(H // 16) for odd in range(2)],
               window(marks, (0.004, 0.98)), _RS)
        rest = jobs_left.pop()
        marks = []
        for r0 in range(0, S // 4, tq):
            for j in range(2):
                for p in range(7):
                    def done(q, v):
                        idx = (p, q, pl.ds(r0, tq), pl.ds(j * 128, 128))
                        old = ffn_v[idx]
                        ffn_v[idx] = v + (jnp.where(c > 0, old, 0.0) if p in (0, 3, 4) else old)

                    marks += [mark(v) for v in _strassen(
                        lambda k: _dot(
                            _unpack(h_v[p, pl.ds(k * S // 8 + r0 // 2, tq // 2), :]),
                            _unpack(b1_v[7 * p + k, pl.ds(j * 64, 64), :])), done)]
            if jobs:
                hidden(jobs, marks)
                jobs = None
        spread(w3_jobs(jnp.minimum(c + 1, nfc - 1)), window(marks, (0, 0.98)))
        spread(rest, window(marks, (0.1, 0.97)))
        spread(late_jobs(c) + late_jobs(c + 1), window(marks, (0.5, 0.9)))
        return 0

    with _scope("ffn"):
        lax.fori_loop(0, nfc, ffn, 0)

    for j in range(n_wo):
        for cp in wo_copies(j):
            cp.wait()


class _Quad:
    def __init__(self, blocks):
        self.blocks = list(blocks)

    def __add__(self, other):
        return _Quad(a + b for a, b in zip(self.blocks, other.blocks))

    def __sub__(self, other):
        return _Quad(a - b for a, b in zip(self.blocks, other.blocks))


def _grid(get):
    return [_Quad(get(2 * i + r, 2 * j + c) for r in range(2) for c in range(2))
            for i in range(2) for j in range(2)]


_RHS_TERMS = ((0, 1, 3), (0, 0, 0), (1, -1, 3), (2, -1, 0), (3, 0, 3), (0, 1, 1), (2, 1, 3))


def _rhs_term(get, p):
    a, sign, b = _RHS_TERMS[p]
    return get(a) if sign == 0 else get(a) + get(b) if sign > 0 else get(a) - get(b)


def _lhs49(get):
    return [v for q in _strassen_lhs(*_grid(get)) for v in _strassen_lhs(*q.blocks)]


_LHS_TERMS = ((0, 1, 3), (2, 1, 3), (0, 0, 0), (3, 0, 3), (0, 1, 1), (2, -1, 0), (1, -1, 3))


def _lhs7(get, p):
    a, sign, b = _LHS_TERMS[p]
    quad = lambda n: _Quad(get(2 * (n // 2) + k // 2, 2 * (n % 2) + k % 2) for k in range(4))
    q = quad(a) if sign == 0 else quad(a) + quad(b) if sign > 0 else quad(a) - quad(b)
    return _strassen_lhs(*q.blocks)


def _rhs7(word, p, z):
    words = [[word(2 * (n // 2) + k // 2, 2 * (n % 2) + k % 2) for k in range(4)]
             if n in (_RHS_TERMS[p][0], _RHS_TERMS[p][2]) else None for n in range(4)]
    shift, high = z | _U32(16), z | _U32(0xFFFF0000)
    halves = []
    for half in (lambda w: w << shift, lambda w: w & high):
        q = _rhs_term(lambda n: _Quad(pltpu.bitcast(half(w), _F32) for w in words[n]), p)
        halves.append([_rhs_term(lambda n: q.blocks[n], k) for k in range(7)])
    return [pltpu.pack_elementwise([e, o], packed_dtype=_BF16) for e, o in zip(*halves)]


def _any(words):
    while len(words) > 1:
        words = [functools.reduce(jnp.bitwise_or, words[k:k + 2]) for k in range(0, len(words), 2)]
    return words[0]


def _fill_jobs(b_v, word, log=None):
    def job(p, k, z):
        for j, w in enumerate(_rhs7(lambda r, c: word(r, c, k), p, z)):
            b_v[7 * p + j, pl.ds(k, 8), :] = w
            if log is not None:
                log.append(w)
    return [functools.partial(job, p, k) for p in (0, 1, 3, 5, 6, 2, 4)
            for k in range(0, b_v.shape[1], 8)]


def _strassen49(prod, done):
    seen = []

    def outer(p):
        out = [None] * 4
        seen.extend(_strassen(lambda k: prod(7 * p + k), out.__setitem__))
        return _Quad(out)

    def finish(n, q):
        for k, v in enumerate(q.blocks):
            done(2 * (n // 2) + k // 2, 2 * (n % 2) + k % 2, v)

    _strassen(outer, finish)
    return seen


def _memory(out_hbm, x_v, wa_v, a_v, xn_v, ffn_v, b0_v, b1_v, mem0, zero, seg,
            pre_v, post_v, a2_v, acc_v, att_v, fin_v, sem_out):
    S, D = x_v.shape
    dh, dq = D // 2, D // 4
    H, E = wa_v.shape[0] // 4, wa_v.shape[2]
    n_wo = D // 128
    n_mem = mem0.shape[0]
    n_seg = S // seg
    early = seg - _LATE
    ql = n_seg * _LATE // 4

    def mark(v):
        return pltpu.bitcast(v[:8, :128], _U32) & zero

    def spread(jobs, marks):
        for k, job in enumerate(jobs):
            job(marks[k * len(marks) // len(jobs)])

    def fill(b_v, n, marks):
        spread(_fill_jobs(b_v, lambda r, c, k: wa_v[n + c, pl.ds(r * dq // 2 + k, 8), :]), marks)

    def mixer_out(i, r, row, n, cols):
        b, c0, nc = cols
        a = 2 * (i % 2) + r // 2
        rows = _ds((i // 2) * (_TM // 4) + (r % 2) * seg + row, n, 8)
        q = 2 * (a % 2) + b % 2
        m = lambda p: ffn_v[p, q, rows, _ds(c0, nc, 128)]
        if isinstance(i, int) and isinstance(b, int):
            c11, c12, c21, c22 = (lambda: (m(0) + m(3)) + (m(6) - m(4)), lambda: m(2) + m(4),
                                  lambda: m(1) + m(3), lambda: (m(0) - m(1)) + (m(2) + m(5)))
            return (c11, c12, c21, c22)[2 * (a // 2) + b // 2]()
        c = _strassen_out([m(p) for p in range(7)])
        if isinstance(b, int):
            return jnp.where(a < 2, c[b // 2], c[2 + b // 2])
        return jnp.where(b < 2, c[2 * (a // 2)], c[2 * (a // 2) + 1])

    def project(n0, lhs, done):
        for j in range(4):
            b_v, marks = (b0_v, b1_v)[j % 2], []
            for r0 in range(0, ql, _PM):
                marks += [mark(v) for v in _strassen49(
                    lambda p: _dot(lhs(j, p, r0), _unpack(b_v[p])),
                    lambda r, c, v: done(j, r, c, r0, v))]
            fill((b1_v, b0_v)[j % 2], jnp.minimum(n0 + 4 * j + 4, 4 * H - 4), marks[:-4])

    fill(b0_v, 0, [zero])

    def pre(i, _):
        even = {}

        def done(j, r, c, r0, v):
            if r % 2 == 0:
                even[c] = v
            else:
                pre_v[16 * i + 4 * j + c, r // 2, pl.ds(r0, _PM), :] = pltpu.pack_elementwise(
                    [even[c], v], packed_dtype=_BF16)

        project(16 * i, lambda j, p, r0: _unpack(a_v[p, pl.ds(r0 // 2, _PM // 2), :]), done)
        return 0

    with _scope("pre"):
        lax.fori_loop(0, 3 * H // 16, pre, 0)

    L = n_mem + seg
    row = lax.broadcasted_iota(jnp.int32, (L, L), 0)
    col = lax.broadcasted_iota(jnp.int32, (L, L), 1)
    mask = (row < n_mem) | (row >= col)
    scale = float(E) ** -0.5

    def step(i, r, mem):
        rows = _ds((4 * i + r) * seg, early, seg)
        hh = jnp.concatenate([mem, _get(xn_v, rows)], axis=0)
        hb = hh.astype(_BF16)
        ng = H // _HG
        qkv, sc = {}, {}

        def proj(g):
            tiles = range(3 * _HG * g, 3 * _HG * (g + 1))
            w = jnp.concatenate([_unpack(wa_v[n]) for n in tiles], axis=1)
            if g == 0:
                y = _dot(hb[:, :dh], w[:dh])
                y = _dot(hb[:, dh:], w[dh:]) + y
            else:
                y = _dot(hb, w)
            w = jnp.concatenate([pre_v[n, r // 2, _ds(i * _LATE, _LATE, _LATE), :] for n in tiles], axis=1)
            qkv[g] = jnp.concatenate(
                [y, pltpu.bitcast(w & _U32(0xFFFF0000) if r % 2 else w << 16, _F32)], axis=0)

        def scores(g):
            y = qkv[g]
            sc[g] = [_dot_nt(y[:, (3 * n) * E:(3 * n + 1) * E],
                             y[:, (3 * n + 1) * E:(3 * n + 2) * E].astype(_BF16))
                     for n in range(_HG)]

        def attend(g):
            y = qkv[g]
            for n in range(_HG):
                z = jnp.where(mask, sc[g][n] * scale, -1e9)
                e = jnp.exp(z - jnp.max(z, axis=-1, keepdims=True))
                inv = 1.0 / jnp.sum(e, axis=-1, keepdims=True)
                o = _dot(e * inv, y[:, (3 * n + 2) * E:(3 * n + 3) * E].astype(_BF16))
                cols = pl.ds((g * _HG + n) * E, E)
                att_v[:, cols] = _pack(o[:L - _LATE])
                post_v[r, :, cols] = o[L - _LATE:]

        def outproj(g0, g1):
            k0, kn, w = g0 * _HG * E, (g1 - g0) * _HG * E, _HG * E
            wo = jnp.concatenate([jnp.concatenate(
                [_unpack(wa_v[_wo_tile(H, k // D, j), pl.ds(k % D // 2, w // 2), :])
                 for k in range(k0, k0 + kn, w)], axis=0) for j in range(n_wo)], axis=1)
            return _dot(_unpack(att_v[:, pl.ds(k0, kn)]), wo)

        for g in range(ng):
            proj(g)
            if g >= 1:
                scores(g - 1)
            if g >= 2:
                attend(g - 2)
        o = outproj(0, _WO[0])
        scores(ng - 1)
        attend(ng - 2)
        o = outproj(_WO[0], _WO[1]) + o
        attend(ng - 1)
        o = outproj(_WO[1], ng) + o
        rest = jnp.concatenate([mixer_out(i, r, 0, early, (b, 0, dq)) for b in range(4)], axis=1)
        x_v[rows, :] = ((x_v[rows, :].astype(_F32) + rest) + o[n_mem:]).astype(_BF16)
        return o[:n_mem]

    with _scope("A"):
        def steps(i, mem):
            for r in range(4):
                mem = step(i, r, mem)
            for m in range(H * E // D):
                for c in range(0, dq, 128):
                    ops = _lhs49(lambda a, b: post_v[a, :, pl.ds(m * D + b * dq + c, 128)])
                    for p, v in enumerate(ops):
                        a2_v[p, _ds(i * _LATE, _LATE, _LATE), pl.ds(m * dq + c, 128)] = v
            for r in range(4):
                rows = _ds((4 * i + r) * seg, early, seg)
                pltpu.make_async_copy(x_v.at[rows], out_hbm.at[rows], sem_out.at[0]).start()
            return mem

        lax.fori_loop(0, n_seg // 4, steps, mem0)

    def post(i, _):
        def done(m, r, c, r0, v):
            idx = (r, c, pl.ds(r0, _PM), slice(None))
            if m > 0:
                v = v + acc_v[idx]
            if m < 3:
                acc_v[idx] = v
                return
            for k in range(0, _PM, _LATE):
                at = (pl.ds((4 * (r0 + k) // _LATE + r) * seg + early, _LATE),
                      _ds((4 * i + c) * 128, 128, 128))
                ffn = mixer_out((r0 + k) // _LATE, r, early, _LATE, (2 * i + c // 2, c % 2 * 128, 128))
                fin_v[at] = ((x_v[at].astype(_F32) + ffn) + v[k:k + _LATE]).astype(_BF16)

        project(3 * H + 16 * i, lambda m, p, r0: a2_v[p, pl.ds(r0, _PM), pl.ds(m * dq, dq)], done)
        for r in range(n_seg):
            at = (pl.ds(r * seg + early, _LATE), _ds(i * dh, dh, dh))
            pltpu.make_async_copy(fin_v.at[at], out_hbm.at[at], sem_out.at[0]).start()
        return 0

    with _scope("post"):
        lax.fori_loop(0, 2, post, 0)
    pltpu.make_async_copy(x_v, out_hbm, sem_out.at[0]).wait()


@functools.partial(jax.jit, static_argnames=("A_seg_len",))
def pallas_parallel_sum__memory_aug_recurrent_mem_tr__mixer_s_mlp__prompt_kernel(
    A_x: jax.Array,
    A_mem0: jax.Array,
    A_Wq: jax.Array,
    A_Wk: jax.Array,
    A_Wv: jax.Array,
    A_Wo: jax.Array,
    A_seg_len: int,
    B_x: jax.Array,
    B_w1: jax.Array,
    B_w2: jax.Array,
    B_w3: jax.Array,
    B_w4: jax.Array,
):
    del B_x
    B, S, D = A_x.shape
    _, H, E = A_Wq.shape
    M = A_mem0.shape[1]
    F = B_w3.shape[1]
    seg = int(A_seg_len)
    nblk = S // _TM
    assert B == 1 and S % _TM == 0 and S % seg == 0 and F % _FC == 0 and H % _HG == 0
    assert nblk == D // 128

    hbm = pl.BlockSpec(memory_space=pltpu.HBM)
    out = pl.pallas_call(
        functools.partial(_kernel, seg=seg),
        out_shape=jax.ShapeDtypeStruct((S, D), A_x.dtype),
        in_specs=[hbm, pl.BlockSpec(memory_space=pltpu.VMEM)] + [hbm] * 8,
        out_specs=hbm,
        scratch_shapes=[
            pltpu.VMEM((S, D), _BF16),
            pltpu.VMEM((4 * H, D // 2, E), _U32),
            pltpu.VMEM((49, S // seg * _LATE // 8, D // 4), _U32),
            pltpu.VMEM((D // 128, S, 128), _F32),
            pltpu.VMEM((7, 4, S // 4, D // 4), _F32),
            pltpu.VMEM((49, D // 8, 128), _U32),
            pltpu.VMEM((49, D // 8, 128), _U32),
        ],
        compiler_params=pltpu.CompilerParams(vmem_limit_bytes=126 * 1024 * 1024, flags=_FLAGS),
    )(A_x.reshape(S, D), A_mem0.reshape(M, D),
      A_Wq.reshape(D * H, E), A_Wk.reshape(D * H, E), A_Wv.reshape(D * H, E),
      A_Wo.reshape(H * E, D), B_w1, B_w2, B_w3, B_w4)
    return out.reshape(B, S, D)
```

```python
import functools

import jax
import jax.numpy as jnp
import numpy as np
from jax import lax
import jax.experimental.pallas as pl
import jax.experimental.pallas.tpu as pltpu

_F32 = jnp.float32
_BF16 = jnp.bfloat16
_U32 = jnp.uint32

_TM = 256
_FC = 512
_HG = 4
_WO = (2, 4)
_PAD = 8
_LOG2E = float(np.log2(np.e))
_NR = 16
_PW = 256
_LATE = 8
_PU = 4
_AU = 2
_PM = 64
_PR = 16
_SM = 64
_LA = 1
_NR0 = 16
_W0 = (0, 0.75)
_WS = (0.1, 0.9)
_WN = (0.02, 0.8)
_WP = (0.45, 0.95)
_WL = (0, 0.5)
_FR = 32
_RD = 160
_RS = 0.3
_CS = 1
_N1 = 5
_HS = 0.9
_TU = 0
_TP = 21
_HE = 2
_HM = 2
_SCOPES = False
_ONLYB = False
_ONLYA = 0
_RC = 1
_AL = (1, 2)
_SP = 1
_PF = (0, -4, -4)
_PT = 0
_FLAGS = None


def _layernorm(x, eps=1e-5):
    m = jnp.mean(x, axis=-1, keepdims=True)
    c = x - m
    v = jnp.mean(c * c, axis=-1, keepdims=True)
    return c * lax.rsqrt(v + eps)


def _layernorm_twice(load, eps=1e-5):
    m = jnp.mean(load(0), axis=-1, keepdims=True)
    c = load(1) - m
    mu = jnp.mean(c, axis=-1, keepdims=True)
    v = jnp.mean(c * c, axis=-1, keepdims=True)
    r = lax.rsqrt(v + eps)
    r2 = r * lax.rsqrt((r * r) * jnp.maximum(v - mu * mu, 0.0) + eps)
    c = load(2) - m
    return c * r, (c - mu) * r2


def _gelu(x):
    c0 = float(np.sqrt(2.0 / np.pi))
    c1 = c0 * 0.044715
    hx = 0.5 * x
    return hx + hx * jnp.tanh(x * (c0 + c1 * (x * x)))


def _dot(a, b):
    return lax.dot_general(a, b, (((1,), (0,)), ((), ())), preferred_element_type=_F32)


def _dot_nt(a, b):
    return lax.dot_general(a, b, (((1,), (1,)), ((), ())), preferred_element_type=_F32)


def _pack(x):
    return pltpu.bitcast(x.astype(_BF16), _U32)


def _unpack(w):
    return pltpu.bitcast(w, _BF16)


def _strassen_lhs(a11, a12, a21, a22):
    return a11 + a22, a21 + a22, a11, a22, a11 + a12, a21 - a11, a12 - a22


def _strassen_out(m):
    m1, m2, m3, m4, m5, m6, m7 = m
    return (m1 + m4) + (m7 - m5), m3 + m5, m2 + m4, (m1 - m2) + (m3 + m6)


def _strassen(prod, done):
    m1, m2 = prod(0), prod(1)
    c22 = m1 - m2
    m4 = prod(3)
    done(2, m2 + m4)
    c11 = m1 + m4
    c22 = prod(5) + c22
    c11 = prod(6) + c11
    m3 = prod(2)
    done(3, c22 + m3)
    m5 = prod(4)
    done(0, c11 - m5)
    done(1, m3 + m5)
    return m1, m2, m4, c22, c11, m3, m5


def _after(x, z):
    w = pltpu.bitcast(x, _U32)
    z = jnp.tile(z, (w.shape[0] // z.shape[0], w.shape[1] // z.shape[1]))
    return pltpu.bitcast(w | z, x.dtype)


class _scope:
    def __init__(self, name):
        self.c = jax.named_scope(name) if _SCOPES else None
    def __enter__(self):
        if self.c: self.c.__enter__()
    def __exit__(self, *a):
        if self.c: self.c.__exit__(*a)


def _pair(even, odd):
    return pltpu.pack_elementwise([even, odd], packed_dtype=_BF16)


def _split(w):
    return pltpu.bitcast(w << 16, _F32), pltpu.bitcast(w & _U32(0xFFFF0000), _F32)


def _get(ref, rows):
    return jnp.concatenate([ref[k, rows, :] for k in range(ref.shape[0])], axis=1)


def _put(ref, rows, c0, x):
    for c in range(0, x.shape[1], 128):
        ref[(c0 + c) // 128, rows, :] = x[:, c:c + 128]


def _wo_tile(heads, m, j):
    return 3 * heads + 16 * (j // 4) + 4 * m + j % 4


def _ds(start, size, align):
    return pl.ds(start if isinstance(start, int) else pl.multiple_of(start, align), size)


def _kernel(x_hbm, mem0_ref, wq_hbm, wk_hbm, wv_hbm, wo_hbm, w1_hbm, w2_hbm, w3_hbm, w4_hbm,
            out_hbm,
            x_v, wa_v, a_v, xn_v, ffn_v, b0_v, b1_v, *, seg):
    S, D = x_v.shape
    F = w3_hbm.shape[1]
    H, E = wa_v.shape[0] // 4, wa_v.shape[2]
    nblk, n_late = S // _TM, S // seg * _LATE
    mem0 = mem0_ref[...].astype(_F32)
    zero = jnp.where(jnp.abs(mem0[:8, :128]) < 0.0, 1, 0).astype(_U32)
    if not _ONLYA: pl.run_scoped(
        functools.partial(_mixer, x_hbm, wq_hbm, wk_hbm, wv_hbm, wo_hbm, w1_hbm, w2_hbm, w3_hbm,
                          w4_hbm, x_v, wa_v, a_v, xn_v, ffn_v, b0_v, b1_v, zero, seg),
        pltpu.VMEM((7, D // 4, D // 2), _U32),
        pltpu.VMEM((7, D // 4, D // 2), _U32),
        pltpu.VMEM((2, D // 2, _FC), _U32),
        pltpu.VMEM((2, _FC // 2, D), _U32),
        pltpu.VMEM((49, S // 8, D // 4), _U32),
        pltpu.VMEM((2, 3, _RD * H // 2, E), _U32),
        pltpu.VMEM((D // 128, S + 2 * _PAD, 128), _F32),
        pltpu.VMEM((2, 7, _TM // 4, D // 2), _U32),
        pltpu.VMEM((7, _TM // 4, D // 2), _U32),
        pltpu.VMEM((D // 128, _TM, 128), _F32),
        pltpu.VMEM((D // 128, _TM, 128), _F32),
        pltpu.VMEM((D // 128, _TM, 128), _F32),
        pltpu.SMEM((1,), jnp.int32),
        pltpu.SemaphoreType.DMA((nblk,)),
        pltpu.SemaphoreType.DMA((6,)),
        pltpu.SemaphoreType.DMA((2, 2)),
        pltpu.SemaphoreType.DMA((2, 3)),
        pltpu.SemaphoreType.DMA((D // 128, H * E // D)))
    if _ONLYB:
        def keep(sem):
            k = lax.iota(jnp.int32, 1)[0] if False else 0
            def body(i, _):
                v = pltpu.bitcast(wa_v[i, :8, :] | a_v[i, :8, :128], _F32) + xn_v[i, :8, :] + ffn_v[i, 0, :8, :128]
                x_v[:8, :128] = v.astype(_BF16)
                return 0
            lax.fori_loop(0, 7, body, 0)
            c = pltpu.make_async_copy(x_v, out_hbm, sem); c.start(); c.wait()
        pl.run_scoped(keep, pltpu.SemaphoreType.DMA)
        return
    pl.run_scoped(
        functools.partial(_memory, out_hbm, x_v, wa_v, a_v, xn_v, ffn_v, b0_v, b1_v, mem0, zero, seg),
        pltpu.VMEM((3 * H, 2, n_late // 4, E), _U32),
        pltpu.VMEM((4, _LATE, H * E), _F32),
        pltpu.VMEM((49, n_late // 4, H * E // 4), _F32),
        pltpu.VMEM((4, D // 128, n_late // 4, 128), _F32),
        pltpu.VMEM(((mem0.shape[0] + seg - _LATE) // 2, H * E), _U32),
        pltpu.VMEM((4, n_late // 4, D), _BF16),
        pltpu.SemaphoreType.DMA((1,)))


def _mixer(x_hbm, wq_hbm, wk_hbm, wv_hbm, wo_hbm, w1_hbm, w2_hbm, w3_hbm, w4_hbm,
           x_v, wa_v, a_v, xn_v, ffn_v, b0_v, b1_v, zero, seg,
           w1_v, w2_v, w3_v, w4_v, f_v, stage_v, h_v, y_v, g_v, t0_v, t1_v, t2_v, nil_s,
           sem_x, sem_w, sem_f, sem_s, sem_o):
    S, D = x_v.shape
    dh = D // 2
    dq, tq = D // 4, _TM // 4
    H, E = wa_v.shape[0] // 4, wa_v.shape[2]
    nblk = S // _TM
    th = _TM // 2
    nfc = w3_hbm.shape[1] // _FC
    n_wo = D // 128

    def x_copy(i):
        rows = _ds(i * _TM, _TM, _TM)
        return pltpu.make_async_copy(x_hbm.at[rows], x_v.at[rows], sem_x.at[i])

    quad = ((0, 0, 1), (0, 1, 2), (1, 0, 3), (1, 1, 4))

    def w3_copy(c):
        src = w3_hbm.bitcast(_U32).at[:, _ds(c * _FC, _FC, _FC)]
        return pltpu.make_async_copy(src, w3_v.at[c % 2], sem_f.at[c % 2, 0])

    def w4_copy(c):
        src = w4_hbm.bitcast(_U32).at[_ds(c * _FC // 2, _FC // 2, _FC // 2)]
        return pltpu.make_async_copy(src, w4_v.at[c % 2], sem_f.at[c % 2, 1])

    def retile_row(c):
        return jnp.minimum(c * _RD, D - _RD) if not isinstance(c, int) else min(c * _RD, D - _RD)

    def stage_copy(t, c):
        src = (wq_hbm, wk_hbm, wv_hbm)[t].bitcast(_U32)
        rows = _ds(retile_row(c) * H // 2, _RD * H // 2, 8 * H)
        return pltpu.make_async_copy(src.at[rows], stage_v.at[c % 2, t], sem_s.at[c % 2, t])

    def wo_copies(j):
        return [pltpu.make_async_copy(
            wo_hbm.bitcast(_U32).at[pl.ds(m * dh, dh), _ds(j * 128, 128, 128)],
            wa_v.at[_wo_tile(H, m, j)], sem_o.at[j, m]) for m in range(H * E // D)]

    w1_copies = [pltpu.make_async_copy(w1_hbm.bitcast(_U32).at[:, pl.ds(k * dh, dh)], w3_v.at[k],
                                       sem_w.at[4 + k]) for k in range(2)]
    w2_copies = [pltpu.make_async_copy(w2_hbm.bitcast(_U32).at[pl.ds(k * dq, dq)], w4_v.at[k],
                                       sem_w.at[k]) for k in range(2)]

    def mark(v, r=0, c=0):
        return pltpu.bitcast(v[r:r + 8, c:c + 128], _U32) & zero

    def put_rhs(w_v, idx, quads, z, seeds=False):
        high = jnp.tile(z | _U32(0xFFFF0000), (1, quads[0].shape[1] // 128))
        sums = []
        for b11, b12, b21, b22 in ([pltpu.bitcast(q << 16, _F32) for q in quads],
                                   [pltpu.bitcast(q & high, _F32) for q in quads]):
            sums.append((b11 + b22, b12 - b22, b21 - b11, b11 + b12, b21 + b22))
        for slot, even, odd in zip((0, 2, 3, 5, 6), *sums):
            w_v[(slot,) + idx] = pltpu.pack_elementwise([even, odd], packed_dtype=_BF16)
        if seeds:
            w_v[(1,) + idx] = quads[0]
            w_v[(4,) + idx] = quads[3]

    jobs_left = []

    def spread(jobs, marks, share=1.0, prev=None):
        if share < 1:
            jobs_left.append(jobs[int(share * len(jobs)):])
            jobs = jobs[:int(share * len(jobs))]
        for k, job in enumerate(jobs):
            z = marks[k * len(marks) // len(jobs)]
            prev = job(z if prev is None else z | prev)
        return prev

    def halves(i, r, n):
        return _ds(i * _TM + r, n, 16), _ds(i * _TM + th + r, n, 16)

    def norm(rows, z):
        nil = nil_s[0]

        def load(k):
            w = [pltpu.bitcast(x_v[_ds(r + 16 * k * nil, 16, 16), :], _U32) for r in rows]
            return jnp.concatenate([h for v in w for h in _split(v if k else _after(v, z))], axis=0)

        xn, y = _layernorm_twice(load)
        for k, r in enumerate(rows):
            for odd in range(2):
                _put(xn_v, pl.ds(r + odd, 8, stride=2), 0, xn[16 * k + 8 * odd:16 * k + 8 * odd + 8])
        return y

    def put_lhs(slot, r, y):
        even, odd = (_strassen_lhs(y[k:k + 8, :dh], y[k:k + 8, dh:], y[k + 16:k + 24, :dh],
                                   y[k + 16:k + 24, dh:]) for k in (0, 8))
        for p in range(7):
            y_v[slot, p, pl.ds(r // 2, 8), :] = _pair(even[p], odd[p])

    def norm_jobs(i, slot):
        def job(r, z):
            y = norm((i * _TM + r, i * _TM + th + r), z)
            put_lhs(slot, r, y)
            return functools.reduce(jnp.bitwise_or, [mark(y, k) for k in range(0, y.shape[0], 8)])
        return [functools.partial(job, r) for r in range(0, th, 16)]

    def ffn_norm_jobs(i):
        t_v, nil = (t0_v, t1_v)[i % 2], nil_s[0]

        def ln(r, z):
            def load(tag):
                return [t_v[c + nil * tag, pl.ds(r, _FR), :] for c in range(D // 128)]

            def mean(parts):
                return jnp.sum(functools.reduce(jnp.add, parts), axis=-1, keepdims=True) * (1.0 / D)

            x1 = load(1)
            m = mean([_after(x1[0], z)] + x1[1:])
            inv = lax.rsqrt(mean([(e - m) * (e - m) for e in load(2)]) + 1e-5)
            for c, e in enumerate(load(3)):
                e = (e - m) * inv
                t2_v[c, pl.ds(r, _FR), :] = e
            return _any([mark(e, k) for k in range(0, _FR, 8)])

        def sums(r, c, p, z):
            r0 = r // 32 * 32 + r % 32 // 16
            lo, hi = (list(_lhs7(lambda a, b: _after(
                t2_v[(b * dq + c) // 128, pl.ds(a * tq + r0 + k, 8, stride=4), :], z), p))
                for k in (0, 2))
            for k in range(7):
                lo[k] = _pair(lo[k], hi[k])
                f_v[7 * p + k, pl.ds((i * tq + r) // 2, 8), pl.ds(c, 128)] = lo[k]
            return _any(lo) & zero if _CS else None

        return ([functools.partial(ln, a * tq + r) for r in range(0, tq, _FR) for a in range(4)],
                [functools.partial(sums, r, c, p)
                 for r in range(0, tq, 16) for c in range(0, dq, 128) for p in range(7)])

    def late_jobs(i):
        def job(c, p, z):
            def get(odd):
                def block(a, b):
                    rows = [_ds(i * _TM + (4 * k + a + 1) * seg - _LATE, _LATE, _LATE) for k in range(2)]
                    return _after(xn_v[(b * dq + c) // 128, rows[odd], :], z)
                return block

            for k, (lo, hi) in enumerate(zip(_lhs7(get(0), p), _lhs7(get(1), p))):
                a_v[7 * p + k, _ds(i * _LATE, _LATE, _LATE), pl.ds(c, 128)] = _pair(lo, hi)
        return [functools.partial(job, c, p) for c in range(0, dq, 128) for p in range(7)]

    def w3_jobs(c):
        return _fill_jobs(b0_v, lambda r, k, j: w3_v[c % 2, pl.ds(r * dq // 2 + j, 8), pl.ds(k * 128, 128)])

    def w4_jobs(c, log):
        return _fill_jobs(b1_v, lambda r, k, j: w4_v[c % 2, pl.ds(r * 64 + j % 64, 8),
                                                     pl.ds(k * dq + j // 64 * 128, 128)], log)

    corners = [(r, c) for r in (0, th) for c in (0, dh)]
    tiles = [(r, c) for r in range(0, th, _SM) for c in range(0, dh, 128)]

    def shift_jobs(i, combine=_strassen_lhs):
        def job(r0, c0, z):
            def load(r, c, odd):
                sh = (-1, 1, -2, 2)[(c + c0) // (D // 4)]
                rows = pl.ds(i * _TM + _PAD + r + r0 + sh + odd, _SM // 2, stride=2)
                return _after(h_v[(c + c0) // 128, rows, :], z)

            even, odd = (combine(*[load(r, c, k) for r, c in corners]) for k in range(2))
            for p in range(len(even)):
                g_v[p, pl.ds(r0 // 2, _SM // 2), pl.ds(c0, 128)] = _pair(even[p], odd[p])
        return [functools.partial(job, r0, c0) for r0, c0 in tiles]

    def mix(lhs, w_v, put):
        marks = []
        for r0, c0 in tiles:
            def prod(p):
                return _dot(_unpack(lhs[p, pl.ds(r0 // 2, _SM // 2), :]),
                            _unpack(w_v[p, :, pl.ds(c0, 128)]))

            def done(q, v):
                r, c = corners[q]
                put(r + r0, c + c0, v)

            marks += [mark(v) for v in _strassen(prod, done)]
        return marks

    def window(marks, w):
        return marks[int(w[0] * len(marks)):int(w[1] * len(marks))]

    def plain(lhs, rhs, put, c0, c1):
        marks = []
        for k in range(c0, c1, 128):
            for r0 in range(0, th, _SM):
                for q in (2, 0):
                    y = jnp.concatenate([_unpack(lhs[q + n, pl.ds(r0 // 2, _SM // 2), :])
                                         for n in range(2)], axis=1)
                    a = _dot(y, _unpack(rhs(k)))
                    put(q // 2 * th + r0, k, a)
                    marks.append(mark(a))
        return marks

    def rhs_jobs(w_v, word):
        def job(k, c, z):
            put_rhs(w_v, (pl.ds(k, 8), pl.ds(c, _PW)), [word(r, q, k, c) for r, q, _ in quad], z, True)
        return [functools.partial(job, k, c) for c in range(0, dh, _PW) for k in range(0, dh // 2, 8)]

    nil_s[0] = 0
    x_copy(0).start()
    w1_copies[0].start()

    for r in (0, _PAD + S):
        _put(h_v, pl.ds(r, _PAD), 0, jnp.zeros((_PAD, D), _F32))
    x_copy(0).wait()
    x_copy(1).start()
    w1_copies[1].start()
    y0 = norm(range(0, _TM, 16), zero)
    for r in range(0, _TM, 16):
        for k in range(2):
            y_v[0, 2 * (r // th) + k, pl.ds(r % th // 2, 8), :] = _pair(
                y0[r:r + 8, k * dh:(k + 1) * dh], y0[r + 8:r + 16, k * dh:(k + 1) * dh])

    def mix_stage(i):
      with _scope("mix%d" % i):
        def put_h(r, c, v):
            _put(h_v, pl.ds(_PAD + i * _TM + r, _SM), c, _gelu(v))

        if i == 0:
            w1_copies[0].wait()
            x_copy(1).wait()
            x_copy(2).start()
            marks = plain(y_v.at[0], lambda k: w3_v[0, :, pl.ds(k, 128)], put_h, 0, dh)
            jobs = norm_jobs(1, 1)
            spread(jobs[:_N1], marks[:12])
            w1_copies[1].wait()
            for cp in w2_copies:
                cp.start()
            x_copy(3).start()
            marks = plain(y_v.at[0], lambda k: w3_v[1, :, pl.ds(k - dh, 128)], put_h, dh, D)
            spread(rhs_jobs(w1_v, lambda r, q, k, c: w3_v[q, pl.ds(r * dq + k, 8), pl.ds(c, _PW)]), marks)
            spread(jobs[_N1:], marks[:12])
            return
        marks = []
        if i == 1:
            x_copy(2).wait()
        if i == 2:
            for k in range(4, nblk):
                x_copy(k).wait()
            w3_copy(0).wait()
            w3_copy(1).start()
            w4_copy(0).start()
            for t in range(3):
                stage_copy(t, 0).start()
            for j in range(n_wo):
                for cp in wo_copies(j):
                    cp.start()
        if i < nblk:
            marks += mix(y_v.at[i % 2], w1_v, put_h)
            spread(shift_jobs(i - 1, _strassen_lhs if i > 1 else lambda *q: q), window(marks, _WS))
        else:
            for job in shift_jobs(i - 1):
                job(zero)
        if i == 1:
            spread(norm_jobs(2, 0), window(marks, (0, 0.8)))
            for cp in w2_copies:
                cp.wait()
            x_copy(3).wait()
            for k in range(4, nblk):
                x_copy(k).start()
            w3_copy(0).start()

        held = {}

        def put_base(r, c, v):
            v = v + xn_v[c // 128, pl.ds((i - 1) * _TM + r, _SM), :]
            (t1_v, t0_v)[i % 2][c // 128, pl.ds(r, _SM), :] = v
            quadrant = 2 * (r // th) + c // dh
            key = (r % th, c % dh)
            held[key, quadrant] = v
            seeds = {0: [(6, v)], 1: [(2, v)], 2: [(1, v)], 3: []}[quadrant]
            if quadrant and all((key, n) in held for n in (1, 2, 3)):
                seeds.append((5, held[key, 3] + (held[key, 2] - held[key, 1])))
            for p, w in seeds:
                ffn_v[p, 2 * (r % th // tq) + c % dh // dq, pl.ds((i - 1) * tq + r % tq, _SM),
                      pl.ds(c % dq, 128)] = w

        if i == 1:
            marks = plain(g_v, lambda k: jnp.concatenate(
                [w4_v[n, :, pl.ds(k, 128)] for n in range(2)], axis=0), put_base, 0, D)
            spread(rhs_jobs(w2_v, lambda r, q, k, c: w4_v[r, pl.ds(k, 8), pl.ds(q * dh + c, _PW)]), marks)
            return
        marks += mix(g_v, w2_v, put_base)
        jobs = norm_jobs(i + 1, (i + 1) % 2) if i + 1 < nblk else []
        if i + 1 == nblk:
            spread(w3_jobs(0), window(marks, _WN))
        if i >= 2:
            ln, sums = ffn_norm_jobs(i - 2)
            jobs = [job for pair in zip(ln, jobs) for job in pair] if jobs else ln
        spread(jobs, window(marks, _WN if i + 1 < nblk else (0, 0.55)), prev=carry.pop())
        carry.append(spread(sums, window(marks, _WP)) if i >= 2 else None)

    carry = [None]
    for i in range(nblk + 1):
        mix_stage(i)
    for jobs in ffn_norm_jobs(nblk - 1):
        for job in jobs:
            job(zero)

    def ffn(c, _):
        @pl.when(c + 1 < nfc)
        def _():
            for t in range(3):
                stage_copy(t, c + 1).start()
            w4_copy(c + 1).start()
            w3_copy(c + 1).wait()

        @pl.when(c + 2 < nfc)
        def _():
            w3_copy(c + 2).start()

        w4_copy(c).wait()
        for t in range(3):
            stage_copy(t, c).wait()

        def retile(t, r, jh, odd, z):
            v = stage_v[c % 2, t, pl.ds(r * H, 8 * H), :].reshape(8, H, E)
            a, b = v[:, 8 * jh:8 * jh + 8], v[:, H // 2 + 8 * jh:H // 2 + 8 * jh + 8]
            low = (z | _U32(0xFFFF))[None]
            w = ((a >> 16) | (b & ~low)) if odd else ((a & low) | (b << 16))
            w = jnp.swapaxes(w, 0, 1)
            rows = _ds(retile_row(c) // 2 + r, 8, 8)
            for j in range(8):
                wa_v[6 * (8 * jh + j) + 3 * odd + t, rows, :] = w[j]

        def hidden_jobs(r0, hid):
            def act(a, b, z):
                hid[a, b] = _gelu(_after(hid[a, b], z))

            def put(r, p, z):
                r1 = r // 32 * 32 + r % 32 // 2
                even, odd = (_lhs7(lambda a, b: _after(hid[a, b][k:k + 8], z) if _PT == 1 or (_PT == 2 and a % 2 + b % 2 == 0) else hid[a, b][k:k + 8], p) for k in (r1, r1 + 16))
                for k in range(7):
                    h_v[p, pl.ds(k * S // 8 + (r0 + r) // 2, 8), :] = pltpu.bitcast(
                        _pair(even[k], odd[k]), _F32)

            return ([functools.partial(act, a, b) for a in range(_HE) for b in range(4)],
                    [functools.partial(put, r, p) for p in (0, 1, 3, 5, 6, 2, 4) for r in range(0, tq, 16)])

        def hidden(jobs, marks):
            spread(jobs[0], window(marks, (0.03, _HS)))
            spread(jobs[1], window(marks, (_HS, 0.98)))

        marks, jobs, log, wait = [], None, [], None
        fills = w4_jobs(c, log)
        for r0 in range(0, S // 4, tq):
            hid = {}

            def lhs(p):
                w = f_v[p, pl.ds(r0 // 2, tq // 2), :]
                return _unpack(w if p != _TP or wait is None else _after(w, wait))

            seen = [mark(v) for v in _strassen49(
                lambda p: _dot(lhs(p), _unpack(b0_v[p])),
                lambda a, b, v: hid.__setitem__((a, b), v if a < _HE else _gelu(v)))]
            if jobs:
                hidden(jobs, seen)
            n = len(fills) // 7
            if fills[r0 // tq * n:]:
                spread(fills[r0 // tq * n:][:n], seen)
            wait = _any(log) & zero if log and _TU else None
            log.clear()
            jobs = hidden_jobs(r0, hid)
            marks += seen
        spread([functools.partial(retile, t, r, jh, odd) for t in range(3)
                for r in range(0, _RD // 2, 8) for jh in range(H // 16) for odd in range(2)],
               window(marks, (0.004, 0.98)), _RS)
        rest = jobs_left.pop()
        marks = []
        for r0 in range(0, S // 4, tq):
            for j in range(2):
                for p in range(7):
                    def done(q, v):
                        idx = (p, q, pl.ds(r0, tq), pl.ds(j * 128, 128))
                        old = ffn_v[idx]
                        ffn_v[idx] = v + (jnp.where(c > 0, old, 0.0) if p in (0, 3, 4) else old)

                    marks += [mark(v) for v in _strassen(
                        lambda k: _dot(
                            _unpack(h_v[p, pl.ds(k * S // 8 + r0 // 2, tq // 2), :]),
                            _unpack(b1_v[7 * p + k, pl.ds(j * 64, 64), :])), done)]
            if jobs:
                hidden(jobs, marks)
                jobs = None
        spread(w3_jobs(jnp.minimum(c + 1, nfc - 1)), window(marks, (0, 0.98)))
        spread(rest, window(marks, (0.1, 0.97)))
        spread(late_jobs(c) + late_jobs(c + 1), window(marks, (0.3, 0.95)))
        return 0

    with _scope("ffn"):
        lax.fori_loop(0, nfc, ffn, 0)

    for j in range(n_wo):
        for cp in wo_copies(j):
            cp.wait()


class _Quad:
    def __init__(self, blocks):
        self.blocks = list(blocks)

    def __add__(self, other):
        return _Quad(a + b for a, b in zip(self.blocks, other.blocks))

    def __sub__(self, other):
        return _Quad(a - b for a, b in zip(self.blocks, other.blocks))


def _grid(get):
    return [_Quad(get(2 * i + r, 2 * j + c) for r in range(2) for c in range(2))
            for i in range(2) for j in range(2)]


_RHS_TERMS = ((0, 1, 3), (0, 0, 0), (1, -1, 3), (2, -1, 0), (3, 0, 3), (0, 1, 1), (2, 1, 3))


def _rhs_term(get, p):
    a, sign, b = _RHS_TERMS[p]
    return get(a) if sign == 0 else get(a) + get(b) if sign > 0 else get(a) - get(b)


def _lhs49(get):
    return [v for q in _strassen_lhs(*_grid(get)) for v in _strassen_lhs(*q.blocks)]


_LHS_TERMS = ((0, 1, 3), (2, 1, 3), (0, 0, 0), (3, 0, 3), (0, 1, 1), (2, -1, 0), (1, -1, 3))


def _lhs7(get, p):
    a, sign, b = _LHS_TERMS[p]
    quad = lambda n: _Quad(get(2 * (n // 2) + k // 2, 2 * (n % 2) + k % 2) for k in range(4))
    q = quad(a) if sign == 0 else quad(a) + quad(b) if sign > 0 else quad(a) - quad(b)
    return _strassen_lhs(*q.blocks)


def _rhs7(word, p, z):
    words = [[word(2 * (n // 2) + k // 2, 2 * (n % 2) + k % 2) for k in range(4)]
             if n in (_RHS_TERMS[p][0], _RHS_TERMS[p][2]) else None for n in range(4)]
    shift, high = z | _U32(16), z | _U32(0xFFFF0000)
    halves = []
    for half in (lambda w: w << shift, lambda w: w & high):
        q = _rhs_term(lambda n: _Quad(pltpu.bitcast(half(w), _F32) for w in words[n]), p)
        halves.append([_rhs_term(lambda n: q.blocks[n], k) for k in range(7)])
    return [pltpu.pack_elementwise([e, o], packed_dtype=_BF16) for e, o in zip(*halves)]


def _any(words):
    while len(words) > 1:
        words = [functools.reduce(jnp.bitwise_or, words[k:k + 2]) for k in range(0, len(words), 2)]
    return words[0]


def _fill_jobs(b_v, word, log=None):
    def job(p, k, z):
        for j, w in enumerate(_rhs7(lambda r, c: word(r, c, k), p, z)):
            b_v[7 * p + j, pl.ds(k, 8), :] = w
            if log is not None:
                log.append(w)
    return [functools.partial(job, p, k) for p in (0, 1, 3, 5, 6, 2, 4)
            for k in range(0, b_v.shape[1], 8)]


def _strassen49(prod, done):
    seen = []

    def outer(p):
        out = [None] * 4
        seen.extend(_strassen(lambda k: prod(7 * p + k), out.__setitem__))
        return _Quad(out)

    def finish(n, q):
        for k, v in enumerate(q.blocks):
            done(2 * (n // 2) + k // 2, 2 * (n % 2) + k % 2, v)

    _strassen(outer, finish)
    return seen


def _memory(out_hbm, x_v, wa_v, a_v, xn_v, ffn_v, b0_v, b1_v, mem0, zero, seg,
            pre_v, post_v, a2_v, acc_v, att_v, fin_v, sem_out):
    S, D = x_v.shape
    dh, dq = D // 2, D // 4
    H, E = wa_v.shape[0] // 4, wa_v.shape[2]
    n_wo = D // 128
    n_mem = mem0.shape[0]
    n_seg = S // seg
    early = seg - _LATE
    ql = n_seg * _LATE // 4

    def mark(v):
        return pltpu.bitcast(v[:8, :128], _U32) & zero

    def spread(jobs, marks):
        for k, job in enumerate(jobs):
            job(marks[k * len(marks) // len(jobs)])

    def fill(b_v, n, marks):
        spread(_fill_jobs(b_v, lambda r, c, k: wa_v[n + c, pl.ds(r * dq // 2 + k, 8), :]), marks)

    def mixer_out(i, r):
        rows = _ds((i // 2) * (_TM // 4) + (r % 2) * seg, seg, seg)
        cols = [None] * 4
        for b in range(2):
            c = _strassen_out([ffn_v[p, 2 * (r // 2) + b, rows, :] for p in range(7)])
            for k in range(2):
                cols[2 * k + b] = jnp.where(i % 2 == 0, c[k], c[2 + k])
        return jnp.concatenate(cols, axis=1)

    def project(n0, lhs, done):
        for j in range(4):
            b_v, marks = (b0_v, b1_v)[j % 2], []
            for r0 in range(0, ql, _PM):
                marks += [mark(v) for v in _strassen49(
                    lambda p: _dot(lhs(j, p, r0), _unpack(b_v[p])),
                    lambda r, c, v: done(j, r, c, r0, v))]
            fill((b1_v, b0_v)[j % 2], jnp.minimum(n0 + 4 * j + 4, 4 * H - 4), marks[_PF[0]:_PF[1] if j < 3 else _PF[2]])

    if _ONLYA != 1: fill(b0_v, 0, [zero])

    def pre(i, _):
        even = {}

        def done(j, r, c, r0, v):
            if r % 2 == 0:
                even[c] = v
            else:
                pre_v[16 * i + 4 * j + c, r // 2, pl.ds(r0, _PM), :] = pltpu.pack_elementwise(
                    [even[c], v], packed_dtype=_BF16)

        project(16 * i, lambda j, p, r0: _unpack(a_v[p, pl.ds(r0 // 2, _PM // 2), :]), done)
        return 0

    with _scope("pre"):
        if _ONLYA != 1: lax.fori_loop(0, 3 * H // 16, pre, 0)

    L = n_mem + seg
    row = lax.broadcasted_iota(jnp.int32, (L, L), 0)
    col = lax.broadcasted_iota(jnp.int32, (L, L), 1)
    mask = (row < n_mem) | (row >= col)
    scale = float(E) ** -0.5

    def step(i, r, mem):
        rows = _ds((4 * i + r) * seg, early, seg)
        hh = jnp.concatenate([mem, _get(xn_v, rows)], axis=0)
        hb = hh.astype(_BF16)
        ng = H // _HG
        qkv, sc = {}, {}

        def proj(g):
            tiles = range(3 * _HG * g, 3 * _HG * (g + 1))
            w = jnp.concatenate([_unpack(wa_v[n]) for n in tiles], axis=1)
            if g == 0:
                y = _dot(hb[:, :dh], w[:dh])
                y = _dot(hb[:, dh:], w[dh:]) + y
            else:
                y = _dot(hb, w)
            w = jnp.concatenate([pre_v[n, r // 2, pl.ds(i // 2 * 2 * _LATE + i % 2, _LATE, stride=2), :] for n in tiles], axis=1)
            qkv[g] = jnp.concatenate(
                [y, pltpu.bitcast(w & _U32(0xFFFF0000) if r % 2 else w << 16, _F32)], axis=0)

        def scores(g):
            y = qkv[g]
            sc[g] = [_dot_nt(y[:, (3 * n) * E:(3 * n + 1) * E],
                             y[:, (3 * n + 1) * E:(3 * n + 2) * E].astype(_BF16))
                     for n in range(_HG)]

        def attend(g):
            y = qkv[g]
            for n in range(_HG):
                z = jnp.where(mask, sc[g][n] * (scale * _LOG2E), -1e9 * _LOG2E)
                e = jnp.exp2(z - jnp.max(z, axis=-1, keepdims=True))
                tot = jnp.sum(e, axis=-1, keepdims=True)
                if _RC:
                    inv = pl.reciprocal(tot, approx=True)
                    inv = inv * (2.0 - tot * inv)
                else:
                    inv = 1.0 / tot
                o = _dot(e * inv, y[:, (3 * n + 2) * E:(3 * n + 3) * E].astype(_BF16))
                cols = pl.ds((g * _HG + n) * E, E)
                att_v[:, cols] = _pack(o[:L - _LATE])
                post_v[r, :, cols] = o[L - _LATE:]

        def outproj(g0, g1):
            k0, kn, w = g0 * _HG * E, (g1 - g0) * _HG * E, _HG * E
            wo = jnp.concatenate([jnp.concatenate(
                [_unpack(wa_v[_wo_tile(H, k // D, j), pl.ds(k % D // 2, w // 2), :])
                 for k in range(k0, k0 + kn, w)], axis=0) for j in range(n_wo)], axis=1)
            return _dot(_unpack(att_v[:, pl.ds(k0, kn)]), wo)

        o = None
        cuts = (0,) + _WO + (ng,)
        for t in range(ng + len(cuts) - 1):
            if t < ng:
                proj(t)
            else:
                d = outproj(cuts[t - ng], cuts[t - ng + 1])
                o = d if o is None else d + o
            if _SP and 0 <= t - _AL[1] < ng:
                attend(t - _AL[1])
            if 0 <= t - _AL[0] < ng:
                scores(t - _AL[0])
            if not _SP and 0 <= t - _AL[1] < ng:
                attend(t - _AL[1])
        rest = x_v[_ds((4 * i + r) * seg, seg, seg), :].astype(_F32) + mixer_out(i, r)
        x_v[rows, :] = (rest[:early] + o[n_mem:]).astype(_BF16)
        _put(acc_v.at[r], _ds(i * _LATE, _LATE, _LATE), 0, rest[early:])
        return o[:n_mem]

    with _scope("A"):
        def steps(i, mem):
            for r in range(4):
                mem = step(i, r, mem)
            for m in range(H * E // D):
                for c in range(0, dq, 128):
                    ops = _lhs49(lambda a, b: post_v[a, :, pl.ds(m * D + b * dq + c, 128)])
                    for p, v in enumerate(ops):
                        a2_v[p, _ds(i * _LATE, _LATE, _LATE), pl.ds(m * dq + c, 128)] = v
            for r in range(4):
                rows = _ds((4 * i + r) * seg, early, seg)
                pltpu.make_async_copy(x_v.at[rows], out_hbm.at[rows], sem_out.at[0]).start()
            return mem

        if _ONLYA != 2: lax.fori_loop(0, n_seg // 4, steps, mem0)

    def post(i, _):
        def done(m, r, c, r0, v):
            v = v + acc_v[r, 4 * i + c, pl.ds(r0, _PM), :] if m == 0 else v + part.pop((r, c, r0))
            if m < 3:
                part[r, c, r0] = v
                return
            for k in range(0, _PM, _LATE):
                fin_v[r, pl.ds(r0 + k, _LATE), _ds((4 * i + c) * 128, 128, 128)] = (
                    v[k:k + _LATE].astype(_BF16))

        part = {}
        project(3 * H + 16 * i, lambda m, p, r0: a2_v[p, pl.ds(r0, _PM), pl.ds(m * dq, dq)], done)
        for r in range(n_seg):
            cols = _ds(i * dh, dh, dh)
            pltpu.make_async_copy(fin_v.at[r % 4, pl.ds(r // 4 * _LATE, _LATE), cols],
                                  out_hbm.at[pl.ds(r * seg + early, _LATE), cols], sem_out.at[0]).start()
        return 0

    with _scope("post"):
        if _ONLYA != 1: lax.fori_loop(0, 2, post, 0)
    pltpu.make_async_copy(x_v, out_hbm, sem_out.at[0]).wait()


@functools.partial(jax.jit, static_argnames=("A_seg_len",))
def pallas_parallel_sum__memory_aug_recurrent_mem_tr__mixer_s_mlp__prompt_kernel(
    A_x: jax.Array,
    A_mem0: jax.Array,
    A_Wq: jax.Array,
    A_Wk: jax.Array,
    A_Wv: jax.Array,
    A_Wo: jax.Array,
    A_seg_len: int,
    B_x: jax.Array,
    B_w1: jax.Array,
    B_w2: jax.Array,
    B_w3: jax.Array,
    B_w4: jax.Array,
):
    del B_x
    B, S, D = A_x.shape
    _, H, E = A_Wq.shape
    M = A_mem0.shape[1]
    F = B_w3.shape[1]
    seg = int(A_seg_len)
    nblk = S // _TM
    assert B == 1 and S % _TM == 0 and S % seg == 0 and F % _FC == 0 and H % _HG == 0
    assert nblk == D // 128

    hbm = pl.BlockSpec(memory_space=pltpu.HBM)
    out = pl.pallas_call(
        functools.partial(_kernel, seg=seg),
        out_shape=jax.ShapeDtypeStruct((S, D), A_x.dtype),
        in_specs=[hbm, pl.BlockSpec(memory_space=pltpu.VMEM)] + [hbm] * 8,
        out_specs=hbm,
        scratch_shapes=[
            pltpu.VMEM((S, D), _BF16),
            pltpu.VMEM((4 * H, D // 2, E), _U32),
            pltpu.VMEM((49, S // seg * _LATE // 8, D // 4), _U32),
            pltpu.VMEM((D // 128, S, 128), _F32),
            pltpu.VMEM((7, 4, S // 4, D // 4), _F32),
            pltpu.VMEM((49, D // 8, 128), _U32),
            pltpu.VMEM((49, D // 8, 128), _U32),
        ],
        compiler_params=pltpu.CompilerParams(vmem_limit_bytes=126 * 1024 * 1024, flags=_FLAGS),
    )(A_x.reshape(S, D), A_mem0.reshape(M, D),
      A_Wq.reshape(D * H, E), A_Wk.reshape(D * H, E), A_Wv.reshape(D * H, E),
      A_Wo.reshape(H * E, D), B_w1, B_w2, B_w3, B_w4)
    return out.reshape(B, S, D)
```

```python
import functools

import jax
import jax.numpy as jnp
import numpy as np
from jax import lax
import jax.experimental.pallas as pl
import jax.experimental.pallas.tpu as pltpu

_F32 = jnp.float32
_BF16 = jnp.bfloat16
_U32 = jnp.uint32

_TM = 256
_FC = 512
_HG = 4
_WO = (2, 4)
_PAD = 8
_LOG2E = float(np.log2(np.e))
_NR = 16
_PW = 128
_LATE = 8
_PU = 4
_AU = 2
_PM = 64
_PR = 16
_SM = 64
_LA = 1
_NR0 = 16
_W0 = (0, 0.75)
_WS = (0.1, 0.9)
_WN = (0.02, 0.8)
_WP = (0.45, 0.95)
_WL = (0, 0.5)
_FR = 32
_RD = 160
_RS = 0.3
_CS = 1
_N1 = 5
_HS = 0.9
_TU = 0
_TP = 21
_HE = 2
_HM = 2
_SCOPES = False
_ONLYB = False
_ONLYA = 0
_RC = 1
_AL = (1, 2)
_SP = 1
_PF = (0, -4, -4)
_PT = 0
_FLAGS = None


def _layernorm(x, eps=1e-5):
    m = jnp.mean(x, axis=-1, keepdims=True)
    c = x - m
    v = jnp.mean(c * c, axis=-1, keepdims=True)
    return c * lax.rsqrt(v + eps)


def _layernorm_twice(load, eps=1e-5):
    m = jnp.mean(load(0), axis=-1, keepdims=True)
    c = load(1) - m
    mu = jnp.mean(c, axis=-1, keepdims=True)
    v = jnp.mean(c * c, axis=-1, keepdims=True)
    r = lax.rsqrt(v + eps)
    r2 = (0.5 * r) * lax.rsqrt((r * r) * jnp.maximum(v - mu * mu, 0.0) + eps)
    c = load(2) - m
    return c * r, (c - mu) * r2


def _gelu(hx):
    c0 = 2.0 * float(np.sqrt(2.0 / np.pi))
    c1 = 4.0 * 0.044715 * c0
    return hx + hx * jnp.tanh(hx * (c0 + c1 * (hx * hx)))


def _dot(a, b):
    return lax.dot_general(a, b, (((1,), (0,)), ((), ())), preferred_element_type=_F32)


def _dot_nt(a, b):
    return lax.dot_general(a, b, (((1,), (1,)), ((), ())), preferred_element_type=_F32)


def _pack(x):
    return pltpu.bitcast(x.astype(_BF16), _U32)


def _unpack(w):
    return pltpu.bitcast(w, _BF16)


def _strassen_lhs(a11, a12, a21, a22):
    return a11 + a22, a21 + a22, a11, a22, a11 + a12, a21 - a11, a12 - a22


def _strassen_out(m):
    m1, m2, m3, m4, m5, m6, m7 = m
    return (m1 + m4) + (m7 - m5), m3 + m5, m2 + m4, (m1 - m2) + (m3 + m6)


def _strassen(prod, done):
    m1, m2 = prod(0), prod(1)
    c22 = m1 - m2
    m4 = prod(3)
    done(2, m2 + m4)
    c11 = m1 + m4
    c22 = prod(5) + c22
    c11 = prod(6) + c11
    m3 = prod(2)
    done(3, c22 + m3)
    m5 = prod(4)
    done(0, c11 - m5)
    done(1, m3 + m5)
    return m1, m2, m4, c22, c11, m3, m5


def _zero_bits(ref):
    return jnp.where(jnp.abs(ref[:16, :128].astype(_F32)[:8]) < 0.0, 1, 0).astype(_U32)


def _after(x, z):
    w = pltpu.bitcast(x, _U32)
    z = jnp.tile(z, (w.shape[0] // z.shape[0], w.shape[1] // z.shape[1]))
    return pltpu.bitcast(w | z, x.dtype)


class _scope:
    def __init__(self, name):
        self.c = jax.named_scope(name) if _SCOPES else None
    def __enter__(self):
        if self.c: self.c.__enter__()
    def __exit__(self, *a):
        if self.c: self.c.__exit__(*a)


def _pair(even, odd):
    return pltpu.pack_elementwise([even, odd], packed_dtype=_BF16)


def _split(w):
    return pltpu.bitcast(w << 16, _F32), pltpu.bitcast(w & _U32(0xFFFF0000), _F32)


def _get(ref, rows):
    return jnp.concatenate([ref[k, rows, :] for k in range(ref.shape[0])], axis=1)


def _put(ref, rows, c0, x):
    for c in range(0, x.shape[1], 128):
        ref[(c0 + c) // 128, rows, :] = x[:, c:c + 128]


def _wo_tile(heads, m, j):
    return 3 * heads + 16 * (j // 4) + 4 * m + j % 4


def _ds(start, size, align):
    return pl.ds(start if isinstance(start, int) else pl.multiple_of(start, align), size)


def _kernel(x_hbm, mem0_hbm, wq_hbm, wk_hbm, wv_hbm, wo_hbm, w1_hbm, w2_hbm, w3_hbm, w4_hbm,
            out_hbm,
            x_v, wa_v, a_v, xn_v, ffn_v, b0_v, b1_v, *, seg):
    S, D = x_v.shape
    F = w3_hbm.shape[1]
    H, E = wa_v.shape[0] // 4, wa_v.shape[2]
    nblk, n_late = S // _TM, S // seg * _LATE
    n_mem = mem0_hbm.shape[0]
    if not _ONLYA: pl.run_scoped(
        functools.partial(_mixer, x_hbm, wq_hbm, wk_hbm, wv_hbm, wo_hbm, w1_hbm, w2_hbm, w3_hbm,
                          w4_hbm, x_v, wa_v, a_v, xn_v, ffn_v, b0_v, b1_v, seg),
        pltpu.VMEM((7, D // 4, D // 2), _U32),
        pltpu.VMEM((7, D // 4, D // 2), _U32),
        pltpu.VMEM((2, D // 2, _FC), _U32),
        pltpu.VMEM((2, _FC // 2, D), _U32),
        pltpu.VMEM((49, S // 8, D // 4), _U32),
        pltpu.VMEM((2, 3, _RD * H // 2, E), _U32),
        pltpu.VMEM((D // 128, S + 2 * _PAD, 128), _F32),
        pltpu.VMEM((2, 7, _TM // 4, D // 2), _U32),
        pltpu.VMEM((7, _TM // 4, D // 2), _U32),
        pltpu.VMEM((D // 128, _TM, 128), _F32),
        pltpu.VMEM((D // 128, _TM, 128), _F32),
        pltpu.VMEM((D // 128, _TM + _PAD, 128), _F32),
        pltpu.SMEM((1,), jnp.int32),
        pltpu.SemaphoreType.DMA((nblk,)),
        pltpu.SemaphoreType.DMA((6,)),
        pltpu.SemaphoreType.DMA((2, 2)),
        pltpu.SemaphoreType.DMA((2, 3)),
        pltpu.SemaphoreType.DMA((D // 128, H * E // D)))
    if _ONLYB:
        def keep(sem):
            k = lax.iota(jnp.int32, 1)[0] if False else 0
            def body(i, _):
                v = pltpu.bitcast(wa_v[i, :8, :] | a_v[i, :8, :128], _F32) + xn_v[i, :8, :] + ffn_v[i, 0, :8, :128]
                x_v[:8, :128] = v.astype(_BF16)
                return 0
            lax.fori_loop(0, 7, body, 0)
            c = pltpu.make_async_copy(x_v, out_hbm, sem); c.start(); c.wait()
        pl.run_scoped(keep, pltpu.SemaphoreType.DMA)
        return
    pl.run_scoped(
        functools.partial(_memory, out_hbm, x_v, wa_v, a_v, xn_v, ffn_v, b0_v, b1_v, mem0_hbm, seg),
        pltpu.VMEM((3 * H, 2, n_late // 4, E), _U32),
        pltpu.VMEM((4, _LATE, H * E), _F32),
        pltpu.VMEM((49, n_late // 4, H * E // 4), _F32),
        pltpu.VMEM((4, D // 128, n_late // 4, 128), _F32),
        pltpu.VMEM(((n_mem + seg - _LATE) // 2, H * E), _U32),
        pltpu.VMEM((4, n_late // 4, D), _BF16),
        pltpu.VMEM((n_mem, D), _BF16),
        pltpu.SemaphoreType.DMA((2,)))


def _mixer(x_hbm, wq_hbm, wk_hbm, wv_hbm, wo_hbm, w1_hbm, w2_hbm, w3_hbm, w4_hbm,
           x_v, wa_v, a_v, xn_v, ffn_v, b0_v, b1_v, seg,
           w1_v, w2_v, w3_v, w4_v, f_v, stage_v, h_v, y_v, g_v, t0_v, t1_v, t2_v, nil_s,
           sem_x, sem_w, sem_f, sem_s, sem_o):
    S, D = x_v.shape
    dh = D // 2
    dq, tq = D // 4, _TM // 4
    H, E = wa_v.shape[0] // 4, wa_v.shape[2]
    nblk = S // _TM
    th = _TM // 2
    nfc = w3_hbm.shape[1] // _FC
    n_wo = D // 128

    def x_copy(i):
        rows = _ds(i * _TM, _TM, _TM)
        return pltpu.make_async_copy(x_hbm.at[rows], x_v.at[rows], sem_x.at[i])

    quad = ((0, 0, 1), (0, 1, 2), (1, 0, 3), (1, 1, 4))

    def w3_copy(c):
        src = w3_hbm.bitcast(_U32).at[:, _ds(c * _FC, _FC, _FC)]
        return pltpu.make_async_copy(src, w3_v.at[c % 2], sem_f.at[c % 2, 0])

    def w4_copy(c):
        src = w4_hbm.bitcast(_U32).at[_ds(c * _FC // 2, _FC // 2, _FC // 2)]
        return pltpu.make_async_copy(src, w4_v.at[c % 2], sem_f.at[c % 2, 1])

    def retile_row(c):
        return jnp.minimum(c * _RD, D - _RD) if not isinstance(c, int) else min(c * _RD, D - _RD)

    def stage_copy(t, c):
        src = (wq_hbm, wk_hbm, wv_hbm)[t].bitcast(_U32)
        rows = _ds(retile_row(c) * H // 2, _RD * H // 2, 8 * H)
        return pltpu.make_async_copy(src.at[rows], stage_v.at[c % 2, t], sem_s.at[c % 2, t])

    def wo_copies(j):
        return [pltpu.make_async_copy(
            wo_hbm.bitcast(_U32).at[pl.ds(m * dh, dh), _ds(j * 128, 128, 128)],
            wa_v.at[_wo_tile(H, m, j)], sem_o.at[j, m]) for m in range(H * E // D)]

    w1_copies = [pltpu.make_async_copy(w1_hbm.bitcast(_U32).at[:, pl.ds(k * dh, dh)], w3_v.at[k],
                                       sem_w.at[4 + k]) for k in range(2)]
    w2_copies = [pltpu.make_async_copy(w2_hbm.bitcast(_U32).at[pl.ds(k * dq, dq)], w4_v.at[k],
                                       sem_w.at[k]) for k in range(2)]

    def mark(v, r=0, c=0):
        return pltpu.bitcast(v[r:r + 8, c:c + 128], _U32) & zero

    def put_rhs(w_v, idx, quads, z, seeds=False):
        high = jnp.tile(z | _U32(0xFFFF0000), (1, quads[0].shape[1] // 128))
        sums = []
        for b11, b12, b21, b22 in ([pltpu.bitcast(q << 16, _F32) for q in quads],
                                   [pltpu.bitcast(q & high, _F32) for q in quads]):
            sums.append((b11 + b22, b12 - b22, b21 - b11, b11 + b12, b21 + b22))
        for slot, even, odd in zip((0, 2, 3, 5, 6), *sums):
            w_v[(slot,) + idx] = pltpu.pack_elementwise([even, odd], packed_dtype=_BF16)
        if seeds:
            w_v[(1,) + idx] = quads[0]
            w_v[(4,) + idx] = quads[3]

    jobs_left = []

    def spread(jobs, marks, share=1.0, prev=None):
        if share < 1:
            jobs_left.append(jobs[int(share * len(jobs)):])
            jobs = jobs[:int(share * len(jobs))]
        for k, job in enumerate(jobs):
            z = marks[k * len(marks) // len(jobs)]
            prev = job(z if prev is None else z | prev)
        return prev

    def halves(i, r, n):
        return _ds(i * _TM + r, n, 16), _ds(i * _TM + th + r, n, 16)

    def norm(rows, z):
        nil = nil_s[0]

        def load(k):
            w = [pltpu.bitcast(x_v[_ds(r + 16 * k * nil, 16, 16), :], _U32) for r in rows]
            return jnp.concatenate([h for v in w for h in _split(v if k else _after(v, z))], axis=0)

        xn, y = _layernorm_twice(load)
        for k, r in enumerate(rows):
            for odd in range(2):
                _put(xn_v, pl.ds(r + odd, 8, stride=2), 0, xn[16 * k + 8 * odd:16 * k + 8 * odd + 8])
        return y

    def put_lhs(slot, r, y):
        even, odd = (_strassen_lhs(y[k:k + 8, :dh], y[k:k + 8, dh:], y[k + 16:k + 24, :dh],
                                   y[k + 16:k + 24, dh:]) for k in (0, 8))
        for p in range(7):
            y_v[slot, p, pl.ds(r // 2, 8), :] = _pair(even[p], odd[p])

    def norm_jobs(i, slot):
        def job(r, z):
            y = norm((i * _TM + r, i * _TM + th + r), z)
            put_lhs(slot, r, y)
            return functools.reduce(jnp.bitwise_or, [mark(y, k) for k in range(0, y.shape[0], 8)])
        return [functools.partial(job, r) for r in range(0, th, 16)]

    def ffn_norm_jobs(i):
        t_v, nil = (t0_v, t1_v)[i % 2], nil_s[0]

        def ln(r, z):
            def load(tag):
                return [t_v[c + nil * tag, pl.ds(r, _FR), :] for c in range(D // 128)]

            def mean(parts):
                return jnp.sum(functools.reduce(jnp.add, parts), axis=-1, keepdims=True) * (1.0 / D)

            x1 = load(1)
            m = mean([_after(x1[0], z)] + x1[1:])
            inv = 0.5 * lax.rsqrt(mean([(e - m) * (e - m) for e in load(2)]) + 1e-5)
            for c, e in enumerate(load(3)):
                e = (e - m) * inv
                t2_v[c, pl.ds(r, _FR), :] = e
            return _any([mark(e, k) for k in range(0, _FR, 8)])

        def sums(r, c, p, z):
            r0 = r // 32 * 32 + r % 32 // 16
            lo, hi = (list(_lhs7(lambda a, b: _after(
                t2_v[(b * dq + c) // 128, pl.ds(a * tq + r0 + k, 8, stride=4), :], z), p))
                for k in (0, 2))
            for k in range(7):
                lo[k] = _pair(lo[k], hi[k])
                f_v[7 * p + k, pl.ds((i * tq + r) // 2, 8), pl.ds(c, 128)] = lo[k]
            return _any(lo) & zero if _CS else None

        return ([functools.partial(ln, a * tq + r) for r in range(0, tq, _FR) for a in range(4)],
                [functools.partial(sums, r, c, p)
                 for r in range(0, tq, 16) for c in range(0, dq, 128) for p in range(7)])

    def late_jobs(i):
        def job(c, p, z):
            def get(odd):
                def block(a, b):
                    rows = [_ds(i * _TM + (4 * k + a + 1) * seg - _LATE, _LATE, _LATE) for k in range(2)]
                    return _after(xn_v[(b * dq + c) // 128, rows[odd], :], z)
                return block

            for k, (lo, hi) in enumerate(zip(_lhs7(get(0), p), _lhs7(get(1), p))):
                a_v[7 * p + k, _ds(i * _LATE, _LATE, _LATE), pl.ds(c, 128)] = _pack(
                    jnp.concatenate([lo, hi], axis=0))
        return [functools.partial(job, c, p) for c in range(0, dq, 128) for p in range(7)]

    def w3_jobs(c):
        return _fill_jobs(b0_v, lambda r, k, j: w3_v[c % 2, pl.ds(r * dq // 2 + j, 8), pl.ds(k * 128, 128)])

    def w4_jobs(c, log):
        return _fill_jobs(b1_v, lambda r, k, j: w4_v[c % 2, pl.ds(r * 64 + j % 64, 8),
                                                     pl.ds(k * dq + j // 64 * 128, 128)], log)

    corners = [(r, c) for r in (0, th) for c in (0, dh)]
    tiles = [(r, c) for r in range(0, th, _SM) for c in range(0, dh, 128)]

    def shift_jobs(i, combine=_strassen_lhs):
        def job(r0, c0, z):
            def load(r, c, odd):
                sh = (-1, 1, -2, 2)[(c + c0) // (D // 4)]
                rows = pl.ds(i * _TM + _PAD + r + r0 + sh + odd, _SM // 2, stride=2)
                return _after(h_v[(c + c0) // 128, rows, :], z)

            even, odd = (combine(*[load(r, c, k) for r, c in corners]) for k in range(2))
            for p in range(len(even)):
                g_v[p, pl.ds(r0 // 2, _SM // 2), pl.ds(c0, 128)] = _pair(even[p], odd[p])
        return [functools.partial(job, r0, c0) for r0, c0 in tiles]

    def mix(lhs, w_v, put):
        marks = []
        for r0, c0 in tiles:
            def prod(p):
                return _dot(_unpack(lhs[p, pl.ds(r0 // 2, _SM // 2), :]),
                            _unpack(w_v[p, :, pl.ds(c0, 128)]))

            def done(q, v):
                r, c = corners[q]
                put(r + r0, c + c0, v)

            marks += [mark(v) for v in _strassen(prod, done)]
        return marks

    def window(marks, w):
        return marks[int(w[0] * len(marks)):int(w[1] * len(marks))]

    def plain(lhs, rhs, put, c0, c1):
        marks = []
        for k in range(c0, c1, 128):
            for r0 in range(0, th, _SM):
                for q in (2, 0):
                    y = jnp.concatenate([_unpack(lhs[q + n, pl.ds(r0 // 2, _SM // 2), :])
                                         for n in range(2)], axis=1)
                    a = _dot(y, _unpack(rhs(k)))
                    put(q // 2 * th + r0, k, a)
                    marks.append(mark(a))
        return marks

    def rhs_jobs(w_v, word):
        def job(k, c, z):
            put_rhs(w_v, (pl.ds(k, 8), pl.ds(c, _PW)), [word(r, q, k, c) for r, q, _ in quad], z, True)
        return [functools.partial(job, k, c) for c in range(0, dh, _PW) for k in range(0, dh // 2, 8)]

    nil_s[0] = 0
    x_copy(0).start()
    x_copy(1).start()
    w1_copies[0].start()

    for r in (0, _PAD + S):
        _put(h_v, pl.ds(r, _PAD), 0, jnp.zeros((_PAD, D), _F32))
    x_copy(0).wait()
    zero = _zero_bits(x_v)
    y0 = norm(range(0, _TM, 16), zero)
    for r in range(0, _TM, 16):
        for k in range(2):
            y_v[0, 2 * (r // th) + k, pl.ds(r % th // 2, 8), :] = _pair(
                y0[r:r + 8, k * dh:(k + 1) * dh], y0[r + 8:r + 16, k * dh:(k + 1) * dh])

    def mix_stage(i):
      with _scope("mix%d" % i):
        def put_h(r, c, v):
            _put(h_v, pl.ds(_PAD + i * _TM + r, _SM), c, _gelu(v))

        if i == 0:
            x_copy(1).wait()
            w1_copies[1].start()
            w1_copies[0].wait()
            x_copy(2).start()
            marks = plain(y_v.at[0], lambda k: w3_v[0, :, pl.ds(k, 128)], put_h, 0, dh)
            jobs = norm_jobs(1, 1)
            spread(jobs[:_N1], marks[:12])
            w1_copies[1].wait()
            for cp in w2_copies:
                cp.start()
            x_copy(3).start()
            marks = plain(y_v.at[0], lambda k: w3_v[1, :, pl.ds(k - dh, 128)], put_h, dh, D)
            spread(rhs_jobs(w1_v, lambda r, q, k, c: w3_v[q, pl.ds(r * dq + k, 8), pl.ds(c, _PW)]), marks)
            spread(jobs[_N1:], marks[:12])
            return
        marks = []
        if i == 1:
            x_copy(2).wait()
            for k in range(4, nblk):
                x_copy(k).start()
            w3_copy(0).start()
        if i == 2:
            for k in range(4, nblk):
                x_copy(k).wait()
            w3_copy(0).wait()
            w3_copy(1).start()
            w4_copy(0).start()
            for t in range(3):
                stage_copy(t, 0).start()
            for j in range(n_wo):
                for cp in wo_copies(j):
                    cp.start()
        if i < nblk:
            marks += mix(y_v.at[i % 2], w1_v, put_h)
            spread(shift_jobs(i - 1, _strassen_lhs if i > 1 else lambda *q: q), window(marks, _WS))
        else:
            for job in shift_jobs(i - 1):
                job(zero)
        if i == 1:
            spread(norm_jobs(2, 0), window(marks, (0, 0.8)))
            for cp in w2_copies:
                cp.wait()
            x_copy(3).wait()

        held = {}

        def put_base(r, c, v):
            v = v + xn_v[c // 128, pl.ds((i - 1) * _TM + r, _SM), :]
            (t1_v, t0_v)[i % 2][c // 128, pl.ds(r, _SM), :] = v
            quadrant = 2 * (r // th) + c // dh
            key = (r % th, c % dh)
            held[key, quadrant] = v
            seeds = {0: [(6, v)], 1: [(2, v)], 2: [(1, v)], 3: []}[quadrant]
            if quadrant and all((key, n) in held for n in (1, 2, 3)):
                seeds.append((5, held[key, 3] + (held[key, 2] - held[key, 1])))
            for p, w in seeds:
                ffn_v[p, 2 * (r % th // tq) + c % dh // dq, pl.ds((i - 1) * tq + r % tq, _SM),
                      pl.ds(c % dq, 128)] = w

        if i == 1:
            marks = plain(g_v, lambda k: jnp.concatenate(
                [w4_v[n, :, pl.ds(k, 128)] for n in range(2)], axis=0), put_base, 0, D)
            spread(rhs_jobs(w2_v, lambda r, q, k, c: w4_v[r, pl.ds(k, 8), pl.ds(q * dh + c, _PW)]), marks)
            return
        marks += mix(g_v, w2_v, put_base)
        jobs = norm_jobs(i + 1, (i + 1) % 2) if i + 1 < nblk else []
        if i + 1 == nblk:
            spread(w3_jobs(0), window(marks, _WN))
        if i >= 2:
            ln, sums = ffn_norm_jobs(i - 2)
            jobs = [job for pair in zip(ln, jobs) for job in pair] if jobs else ln
        spread(jobs, window(marks, _WN if i + 1 < nblk else (0, 0.55)), prev=carry.pop())
        carry.append(spread(sums, window(marks, _WP)) if i >= 2 else None)

    carry = [None]
    for i in range(nblk + 1):
        mix_stage(i)
    for jobs in ffn_norm_jobs(nblk - 1):
        for job in jobs:
            job(zero)

    def ffn(c, _):
        @pl.when(c + 1 < nfc)
        def _():
            for t in range(3):
                stage_copy(t, c + 1).start()
            w4_copy(c + 1).start()
            w3_copy(c + 1).wait()

        @pl.when(c + 2 < nfc)
        def _():
            w3_copy(c + 2).start()

        w4_copy(c).wait()
        for t in range(3):
            stage_copy(t, c).wait()

        def retile(t, r, jh, odd, z):
            v = stage_v[c % 2, t, pl.ds(r * H, 8 * H), :].reshape(8, H, E)
            a, b = v[:, 8 * jh:8 * jh + 8], v[:, H // 2 + 8 * jh:H // 2 + 8 * jh + 8]
            low = (z | _U32(0xFFFF))[None]
            w = ((a >> 16) | (b & ~low)) if odd else ((a & low) | (b << 16))
            w = jnp.swapaxes(w, 0, 1)
            rows = _ds(retile_row(c) // 2 + r, 8, 8)
            for j in range(8):
                wa_v[6 * (8 * jh + j) + 3 * odd + t, rows, :] = w[j]

        def hidden_jobs(r0, hid):
            def act(a, b, z):
                hid[a, b] = _gelu(_after(hid[a, b], z))

            def put(r, p, z):
                r1 = r // 32 * 32 + r % 32 // 2
                even, odd = (_lhs7(lambda a, b: _after(hid[a, b][k:k + 8], z) if _PT == 1 or (_PT == 2 and a % 2 + b % 2 == 0) else hid[a, b][k:k + 8], p) for k in (r1, r1 + 16))
                for k in range(7):
                    h_v[p, pl.ds(k * S // 8 + (r0 + r) // 2, 8), :] = pltpu.bitcast(
                        _pair(even[k], odd[k]), _F32)

            return ([functools.partial(act, a, b) for a in range(_HE) for b in range(4)],
                    [functools.partial(put, r, p) for p in (0, 1, 3, 5, 6, 2, 4) for r in range(0, tq, 16)])

        def hidden(jobs, marks):
            spread(jobs[0], window(marks, (0.03, _HS)))
            spread(jobs[1], window(marks, (_HS, 0.98)))

        marks, jobs, log, wait = [], None, [], None
        fills = w4_jobs(c, log)
        for r0 in range(0, S // 4, tq):
            hid = {}

            def lhs(p):
                w = f_v[p, pl.ds(r0 // 2, tq // 2), :]
                return _unpack(w if p != _TP or wait is None else _after(w, wait))

            seen = [mark(v) for v in _strassen49(
                lambda p: _dot(lhs(p), _unpack(b0_v[p])),
                lambda a, b, v: hid.__setitem__((a, b), v if a < _HE else _gelu(v)))]
            if jobs:
                hidden(jobs, seen)
            n = len(fills) // 7
            if fills[r0 // tq * n:]:
                spread(fills[r0 // tq * n:][:n], seen)
            wait = _any(log) & zero if log and _TU else None
            log.clear()
            jobs = hidden_jobs(r0, hid)
            marks += seen
        spread([functools.partial(retile, t, r, jh, odd) for t in range(3)
                for r in range(0, _RD // 2, 8) for jh in range(H // 16) for odd in range(2)],
               window(marks, (0.004, 0.98)), _RS)
        rest = jobs_left.pop()
        marks = []
        for r0 in range(0, S // 4, tq):
            for j in range(2):
                for p in range(7):
                    def done(q, v):
                        idx = (p, q, pl.ds(r0, tq), pl.ds(j * 128, 128))
                        old = ffn_v[idx]
                        ffn_v[idx] = v + (jnp.where(c > 0, old, 0.0) if p in (0, 3, 4) else old)

                    marks += [mark(v) for v in _strassen(
                        lambda k: _dot(
                            _unpack(h_v[p, pl.ds(k * S // 8 + r0 // 2, tq // 2), :]),
                            _unpack(b1_v[7 * p + k, pl.ds(j * 64, 64), :])), done)]
            if jobs:
                hidden(jobs, marks)
                jobs = None
        spread(w3_jobs(jnp.minimum(c + 1, nfc - 1)), window(marks, (0, 0.98)))
        spread(rest, window(marks, (0.1, 0.97)))
        spread(late_jobs(c) + late_jobs(c + 1), window(marks, (0.3, 0.95)))
        return 0

    with _scope("ffn"):
        lax.fori_loop(0, nfc, ffn, 0)

    for j in range(n_wo):
        for cp in wo_copies(j):
            cp.wait()


class _Quad:
    def __init__(self, blocks):
        self.blocks = list(blocks)

    def __add__(self, other):
        return _Quad(a + b for a, b in zip(self.blocks, other.blocks))

    def __sub__(self, other):
        return _Quad(a - b for a, b in zip(self.blocks, other.blocks))


def _grid(get):
    return [_Quad(get(2 * i + r, 2 * j + c) for r in range(2) for c in range(2))
            for i in range(2) for j in range(2)]


_RHS_TERMS = ((0, 1, 3), (0, 0, 0), (1, -1, 3), (2, -1, 0), (3, 0, 3), (0, 1, 1), (2, 1, 3))


def _rhs_term(get, p):
    a, sign, b = _RHS_TERMS[p]
    return get(a) if sign == 0 else get(a) + get(b) if sign > 0 else get(a) - get(b)


def _lhs49(get):
    return [v for q in _strassen_lhs(*_grid(get)) for v in _strassen_lhs(*q.blocks)]


_LHS_TERMS = ((0, 1, 3), (2, 1, 3), (0, 0, 0), (3, 0, 3), (0, 1, 1), (2, -1, 0), (1, -1, 3))


def _lhs7(get, p):
    a, sign, b = _LHS_TERMS[p]
    quad = lambda n: _Quad(get(2 * (n // 2) + k // 2, 2 * (n % 2) + k % 2) for k in range(4))
    q = quad(a) if sign == 0 else quad(a) + quad(b) if sign > 0 else quad(a) - quad(b)
    return _strassen_lhs(*q.blocks)


def _rhs7(word, p, z):
    words = [[word(2 * (n // 2) + k // 2, 2 * (n % 2) + k % 2) for k in range(4)]
             if n in (_RHS_TERMS[p][0], _RHS_TERMS[p][2]) else None for n in range(4)]
    shift, high = z | _U32(16), z | _U32(0xFFFF0000)
    halves = []
    for half in (lambda w: w << shift, lambda w: w & high):
        q = _rhs_term(lambda n: _Quad(pltpu.bitcast(half(w), _F32) for w in words[n]), p)
        halves.append([_rhs_term(lambda n: q.blocks[n], k) for k in range(7)])
    return [pltpu.pack_elementwise([e, o], packed_dtype=_BF16) for e, o in zip(*halves)]


def _any(words):
    while len(words) > 1:
        words = [functools.reduce(jnp.bitwise_or, words[k:k + 2]) for k in range(0, len(words), 2)]
    return words[0]


def _fill_jobs(b_v, word, log=None):
    def job(p, k, z):
        for j, w in enumerate(_rhs7(lambda r, c: word(r, c, k), p, z)):
            b_v[7 * p + j, pl.ds(k, 8), :] = w
            if log is not None:
                log.append(w)
    return [functools.partial(job, p, k) for p in (0, 1, 3, 5, 6, 2, 4)
            for k in range(0, b_v.shape[1], 8)]


def _strassen49(prod, done):
    seen = []

    def outer(p):
        out = [None] * 4
        seen.extend(_strassen(lambda k: prod(7 * p + k), out.__setitem__))
        return _Quad(out)

    def finish(n, q):
        for k, v in enumerate(q.blocks):
            done(2 * (n // 2) + k // 2, 2 * (n % 2) + k % 2, v)

    _strassen(outer, finish)
    return seen


def _memory(out_hbm, x_v, wa_v, a_v, xn_v, ffn_v, b0_v, b1_v, mem0_hbm, seg,
            pre_v, post_v, a2_v, acc_v, att_v, fin_v, mem0_v, sem_out):
    S, D = x_v.shape
    dh, dq = D // 2, D // 4
    H, E = wa_v.shape[0] // 4, wa_v.shape[2]
    n_wo = D // 128
    n_mem = mem0_hbm.shape[0]
    mem0_copy = pltpu.make_async_copy(mem0_hbm, mem0_v, sem_out.at[1])
    mem0_copy.start()
    zero = _zero_bits(x_v)
    n_seg = S // seg
    early = seg - _LATE
    ql = n_seg * _LATE // 4

    def mark(v):
        return pltpu.bitcast(v[:8, :128], _U32) & zero

    def spread(jobs, marks):
        for k, job in enumerate(jobs):
            job(marks[k * len(marks) // len(jobs)])

    def fill(b_v, n, marks):
        spread(_fill_jobs(b_v, lambda r, c, k: wa_v[n + c, pl.ds(r * dq // 2 + k, 8), :]), marks)

    def mixer_out(i, r):
        rows = _ds((i // 2) * (_TM // 4) + (r % 2) * seg, seg, seg)
        cols = [None] * 4
        for b in range(2):
            c = _strassen_out([ffn_v[p, 2 * (r // 2) + b, rows, :] for p in range(7)])
            for k in range(2):
                cols[2 * k + b] = jnp.where(i % 2 == 0, c[k], c[2 + k])
        return jnp.concatenate(cols, axis=1)

    def project(n0, lhs, done):
        for j in range(4):
            b_v, marks = (b0_v, b1_v)[j % 2], []
            for r0 in range(0, ql, _PM):
                marks += [mark(v) for v in _strassen49(
                    lambda p: _dot(lhs(j, p, r0), _unpack(b_v[p])),
                    lambda r, c, v: done(j, r, c, r0, v))]
            fill((b1_v, b0_v)[j % 2], n0 + 4 * j + 4 if isinstance(n0, int) else jnp.minimum(n0 + 4 * j + 4, 4 * H - 4), marks[_PF[0]:_PF[1] if j < 3 else _PF[2]])

    if _ONLYA != 1: fill(b0_v, 0, [zero])

    def pre(i, _):
        even = {}

        def done(j, r, c, r0, v):
            if r % 2 == 0:
                even[c] = v
            else:
                pre_v[16 * i + 4 * j + c, r // 2, pl.ds(r0, _PM), :] = pltpu.pack_elementwise(
                    [even[c], v], packed_dtype=_BF16)

        project(16 * i, lambda j, p, r0: _unpack(a_v[p, pl.ds(r0 // 2, _PM // 2), :]), done)
        return 0

    with _scope("pre"):
        if _ONLYA != 1:
            pre(0, 0)
            lax.fori_loop(1, 3 * H // 16, pre, 0)

    L = n_mem + seg
    row = lax.broadcasted_iota(jnp.int32, (L, L), 0)
    col = lax.broadcasted_iota(jnp.int32, (L, L), 1)
    mask = (row < n_mem) | (row >= col)
    scale = float(E) ** -0.5

    def step(i, r, mem):
        rows = _ds((4 * i + r) * seg, early, seg)
        hh = jnp.concatenate([mem, _get(xn_v, rows)], axis=0)
        hb = hh.astype(_BF16)
        ng = H // _HG
        qkv, sc = {}, {}

        def proj(g):
            tiles = range(3 * _HG * g, 3 * _HG * (g + 1))
            w = jnp.concatenate([_unpack(wa_v[n]) for n in tiles], axis=1)
            if g == 0:
                y = _dot(hb[:, :dh], w[:dh])
                y = _dot(hb[:, dh:], w[dh:]) + y
            else:
                y = _dot(hb, w)
            w = jnp.concatenate([pre_v[n, r // 2, _ds(i * _LATE, _LATE, _LATE), :] for n in tiles], axis=1)
            qkv[g] = jnp.concatenate(
                [y, pltpu.bitcast(w & _U32(0xFFFF0000) if r % 2 else w << 16, _F32)], axis=0)

        def scores(g):
            y = qkv[g]
            sc[g] = [_dot_nt(y[:, (3 * n) * E:(3 * n + 1) * E],
                             y[:, (3 * n + 1) * E:(3 * n + 2) * E].astype(_BF16))
                     for n in range(_HG)]

        def attend(g):
            y = qkv[g]
            for n in range(_HG):
                z = jnp.where(mask, sc[g][n] * (scale * _LOG2E), -1e9 * _LOG2E)
                e = jnp.exp2(z - jnp.max(z, axis=-1, keepdims=True))
                tot = jnp.sum(e, axis=-1, keepdims=True)
                if _RC:
                    inv = pl.reciprocal(tot, approx=True)
                    inv = inv * (2.0 - tot * inv)
                else:
                    inv = 1.0 / tot
                o = _dot(e * inv, y[:, (3 * n + 2) * E:(3 * n + 3) * E].astype(_BF16))
                cols = pl.ds((g * _HG + n) * E, E)
                att_v[:, cols] = _pack(o[:L - _LATE])
                post_v[r, :, cols] = o[L - _LATE:]

        def outproj(g0, g1):
            k0, kn, w = g0 * _HG * E, (g1 - g0) * _HG * E, _HG * E
            wo = jnp.concatenate([jnp.concatenate(
                [_unpack(wa_v[_wo_tile(H, k // D, j), pl.ds(k % D // 2, w // 2), :])
                 for k in range(k0, k0 + kn, w)], axis=0) for j in range(n_wo)], axis=1)
            return _dot(_unpack(att_v[:, pl.ds(k0, kn)]), wo)

        o = None
        cuts = (0,) + _WO + (ng,)
        for t in range(ng + len(cuts) - 1):
            if t < ng:
                proj(t)
            else:
                d = outproj(cuts[t - ng], cuts[t - ng + 1])
                o = d if o is None else d + o
            if _SP and 0 <= t - _AL[1] < ng:
                attend(t - _AL[1])
            if 0 <= t - _AL[0] < ng:
                scores(t - _AL[0])
            if not _SP and 0 <= t - _AL[1] < ng:
                attend(t - _AL[1])
        rest = x_v[_ds((4 * i + r) * seg, seg, seg), :].astype(_F32) + mixer_out(i, r)
        x_v[rows, :] = (rest[:early] + o[n_mem:]).astype(_BF16)
        _put(acc_v.at[r], _ds(i * _LATE, _LATE, _LATE), 0, rest[early:])
        return o[:n_mem]

    with _scope("A"):
        def steps(i, mem):
            for r in range(4):
                mem = step(i, r, mem)
            for m in range(H * E // D):
                for c in range(0, dq, 128):
                    ops = _lhs49(lambda a, b: post_v[a, :, pl.ds(m * D + b * dq + c, 128)])
                    for p, v in enumerate(ops):
                        a2_v[p, _ds(i * _LATE, _LATE, _LATE), pl.ds(m * dq + c, 128)] = v
            for r in range(4):
                rows = _ds((4 * i + r) * seg, early, seg)
                pltpu.make_async_copy(x_v.at[rows], out_hbm.at[rows], sem_out.at[0]).start()
            return mem

        mem0_copy.wait()
        if _ONLYA != 2: lax.fori_loop(0, n_seg // 4, steps, mem0_v[...].astype(_F32))

    def post(i, _):
        def done(m, r, c, r0, v):
            v = v + acc_v[r, 4 * i + c, pl.ds(r0, _PM), :] if m == 0 else v + part.pop((r, c, r0))
            if m < 3:
                part[r, c, r0] = v
                return
            for k in range(0, _PM, _LATE):
                fin_v[r, pl.ds(r0 + k, _LATE), _ds((4 * i + c) * 128, 128, 128)] = (
                    v[k:k + _LATE].astype(_BF16))

        part = {}
        project(3 * H + 16 * i, lambda m, p, r0: a2_v[p, pl.ds(r0, _PM), pl.ds(m * dq, dq)], done)
        for r in range(n_seg):
            cols = _ds(i * dh, dh, dh)
            pltpu.make_async_copy(fin_v.at[r % 4, pl.ds(r // 4 * _LATE, _LATE), cols],
                                  out_hbm.at[pl.ds(r * seg + early, _LATE), cols], sem_out.at[0]).start()
        return 0

    with _scope("post"):
        if _ONLYA != 1: lax.fori_loop(0, 2, post, 0)
    pltpu.make_async_copy(x_v, out_hbm, sem_out.at[0]).wait()


@functools.partial(jax.jit, static_argnames=("A_seg_len",))
def pallas_parallel_sum__memory_aug_recurrent_mem_tr__mixer_s_mlp__prompt_kernel(
    A_x: jax.Array,
    A_mem0: jax.Array,
    A_Wq: jax.Array,
    A_Wk: jax.Array,
    A_Wv: jax.Array,
    A_Wo: jax.Array,
    A_seg_len: int,
    B_x: jax.Array,
    B_w1: jax.Array,
    B_w2: jax.Array,
    B_w3: jax.Array,
    B_w4: jax.Array,
):
    del B_x
    B, S, D = A_x.shape
    _, H, E = A_Wq.shape
    M = A_mem0.shape[1]
    F = B_w3.shape[1]
    seg = int(A_seg_len)
    nblk = S // _TM
    assert B == 1 and S % _TM == 0 and S % seg == 0 and F % _FC == 0 and H % _HG == 0
    assert nblk == D // 128

    hbm = pl.BlockSpec(memory_space=pltpu.HBM)
    out = pl.pallas_call(
        functools.partial(_kernel, seg=seg),
        out_shape=jax.ShapeDtypeStruct((S, D), A_x.dtype),
        in_specs=[hbm] * 10,
        out_specs=hbm,
        scratch_shapes=[
            pltpu.VMEM((S, D), _BF16),
            pltpu.VMEM((4 * H, D // 2, E), _U32),
            pltpu.VMEM((49, S // seg * _LATE // 8, D // 4), _U32),
            pltpu.VMEM((D // 128, S + _PAD, 128), _F32),
            pltpu.VMEM((7, 4, S // 4, D // 4), _F32),
            pltpu.VMEM((49, D // 8, 128), _U32),
            pltpu.VMEM((49, D // 8, 128), _U32),
        ],
        compiler_params=pltpu.CompilerParams(vmem_limit_bytes=126 * 1024 * 1024, flags=_FLAGS),
    )(A_x.reshape(S, D), A_mem0.reshape(M, D),
      A_Wq.reshape(D * H, E), A_Wk.reshape(D * H, E), A_Wv.reshape(D * H, E),
      A_Wo.reshape(H * E, D), B_w1, B_w2, B_w3, B_w4)
    return out.reshape(B, S, D)
```

```python
import functools

import jax
import jax.numpy as jnp
import numpy as np
from jax import lax
import jax.experimental.pallas as pl
import jax.experimental.pallas.tpu as pltpu

_F32 = jnp.float32
_BF16 = jnp.bfloat16
_U32 = jnp.uint32

_EPS = 1e-5
_LOG2E = float(np.log2(np.e))
_TM = 256
_SM = 64
_FC = 512
_RD = 160
_HG = 4
_LATE = 8
_PAD = 8


def _dot(a, b):
    return lax.dot_general(a, b, (((1,), (0,)), ((), ())), preferred_element_type=_F32)


def _dot_nt(a, b):
    return lax.dot_general(a, b, (((1,), (1,)), ((), ())), preferred_element_type=_F32)


def _ds(start, size, align):
    return pl.ds(start if isinstance(start, int) else pl.multiple_of(start, align), size)


def _pack(x):
    return pltpu.bitcast(x.astype(_BF16), _U32)


def _unpack(w):
    return pltpu.bitcast(w, _BF16)


def _pair(even, odd):
    return pltpu.pack_elementwise([even, odd], packed_dtype=_BF16)


def _split(w):
    return pltpu.bitcast(w << 16, _F32), pltpu.bitcast(w & _U32(0xFFFF0000), _F32)


def _get(ref, rows):
    return jnp.concatenate([ref[k, rows, :] for k in range(ref.shape[0])], axis=1)


def _put(ref, rows, c0, x):
    for c in range(0, x.shape[1], 128):
        ref[(c0 + c) // 128, rows, :] = x[:, c:c + 128]


def _wo_slab(heads, m, j):
    return 3 * heads + 16 * (j // 4) + 4 * m + j % 4


def _gelu(hx):
    c0 = 2.0 * float(np.sqrt(2.0 / np.pi))
    c1 = 4.0 * 0.044715 * c0
    return hx + hx * jnp.tanh(hx * (c0 + c1 * (hx * hx)))


def _layernorm_twice(load):
    m = jnp.mean(load(0), axis=-1, keepdims=True)
    c = load(1) - m
    mu = jnp.mean(c, axis=-1, keepdims=True)
    v = jnp.mean(c * c, axis=-1, keepdims=True)
    r = lax.rsqrt(v + _EPS)
    r2 = (0.5 * r) * lax.rsqrt((r * r) * jnp.maximum(v - mu * mu, 0.0) + _EPS)
    c = load(2) - m
    return c * r, (c - mu) * r2


def _zero_bits(ref):
    return jnp.where(jnp.abs(ref[:16, :128].astype(_F32)[:8]) < 0.0, 1, 0).astype(_U32)


def _after(x, z):
    w = pltpu.bitcast(x, _U32)
    z = jnp.tile(z, (w.shape[0] // z.shape[0], w.shape[1] // z.shape[1]))
    return pltpu.bitcast(w | z, x.dtype)


def _any(words):
    while len(words) > 1:
        words = [functools.reduce(jnp.bitwise_or, words[k:k + 2]) for k in range(0, len(words), 2)]
    return words[0]


def _spread(jobs, marks, lo=0.0, hi=1.0, prev=None):
    marks = marks[int(lo * len(marks)):int(hi * len(marks))]
    for k, job in enumerate(jobs):
        z = marks[k * len(marks) // len(jobs)]
        prev = job(z if prev is None else z | prev)
    return prev


_LHS_TERMS = ((0, 1, 3), (2, 1, 3), (0, 0, 0), (3, 0, 3), (0, 1, 1), (2, -1, 0), (1, -1, 3))
_RHS_TERMS = ((0, 1, 3), (0, 0, 0), (1, -1, 3), (2, -1, 0), (3, 0, 3), (0, 1, 1), (2, 1, 3))
_ORDER = (0, 1, 3, 5, 6, 2, 4)


class _Quad:
    def __init__(self, blocks):
        self.blocks = list(blocks)

    def __add__(self, other):
        return _Quad(a + b for a, b in zip(self.blocks, other.blocks))

    def __sub__(self, other):
        return _Quad(a - b for a, b in zip(self.blocks, other.blocks))


def _term(terms, get, p):
    a, sign, b = terms[p]
    return get(a) if sign == 0 else get(a) + get(b) if sign > 0 else get(a) - get(b)


def _operands(terms, quadrants):
    return [_term(terms, quadrants.__getitem__, p) for p in range(7)]


def _block(n, k):
    return 2 * (n // 2) + k // 2, 2 * (n % 2) + k % 2


def _operands7(terms, get, p):
    outer = _term(terms, lambda n: _Quad(get(*_block(n, k)) for k in range(4)), p)
    return _operands(terms, outer.blocks)


def _combine(m):
    m1, m2, m3, m4, m5, m6, m7 = m
    return (m1 + m4) + (m7 - m5), m3 + m5, m2 + m4, (m1 - m2) + (m3 + m6)


def _strassen(prod, done):
    m1, m2 = prod(0), prod(1)
    c22 = m1 - m2
    m4 = prod(3)
    done(2, m2 + m4)
    c11 = m1 + m4
    c22 = prod(5) + c22
    c11 = prod(6) + c11
    m3 = prod(2)
    done(3, c22 + m3)
    m5 = prod(4)
    done(0, c11 - m5)
    done(1, m3 + m5)
    return m1, m2, m4, c22, c11, m3, m5


def _strassen49(prod, done):
    seen = []

    def outer(p):
        out = [None] * 4
        m = _strassen(lambda k: prod(7 * p + k), out.__setitem__)
        seen.extend(m[k] for k in (0, 1, 3, 4))
        return _Quad(out)

    def finish(n, quad):
        for k, v in enumerate(quad.blocks):
            done(*_block(n, k), v)

    _strassen(outer, finish)
    return seen


def _halves(z):
    shift, high = z | _U32(16), z | _U32(0xFFFF0000)
    return (lambda w: pltpu.bitcast(w << shift, _F32)), (lambda w: pltpu.bitcast(w & high, _F32))


def _fill_jobs(b_v, word):
    def job(p, k, z):
        even, odd = (_operands7(_RHS_TERMS, lambda r, c: half(word(r, c, k)), p)
                     for half in _halves(z))
        for j in range(7):
            b_v[7 * p + j, pl.ds(k, 8), :] = _pair(even[j], odd[j])

    return [functools.partial(job, p, k) for p in _ORDER for k in range(0, b_v.shape[1], 8)]


def _mixer(x_hbm, wq_hbm, wk_hbm, wv_hbm, wo_hbm, w1_hbm, w2_hbm, w3_hbm, w4_hbm,
           x_v, wa_v, a_v, xn_v, ffn_v, b0_v, b1_v, seg,
           w1_v, w2_v, w3_v, w4_v, f_v, stage_v, h_v, y_v, g_v, t0_v, t1_v, t2_v, nil_s,
           sem_x, sem_w, sem_f, sem_s, sem_o):
    S, D = x_v.shape
    H, E = wa_v.shape[0] // 4, wa_v.shape[2]
    dh, dq, th, tq = D // 2, D // 4, _TM // 2, _TM // 4
    nblk = S // _TM
    nfc = w3_hbm.shape[1] // _FC
    corners = [(r, c) for r in (0, th) for c in (0, dh)]
    tiles = [(r, c) for r in range(0, th, _SM) for c in range(0, dh, 128)]

    def x_copy(i):
        rows = pl.ds(i * _TM, _TM)
        return pltpu.make_async_copy(x_hbm.at[rows], x_v.at[rows], sem_x.at[i])

    def w3_copy(c):
        src = w3_hbm.bitcast(_U32).at[:, _ds(c * _FC, _FC, _FC)]
        return pltpu.make_async_copy(src, w3_v.at[c % 2], sem_f.at[c % 2, 0])

    def w4_copy(c):
        src = w4_hbm.bitcast(_U32).at[_ds(c * _FC // 2, _FC // 2, _FC // 2)]
        return pltpu.make_async_copy(src, w4_v.at[c % 2], sem_f.at[c % 2, 1])

    def retile_row(c):
        return min(c * _RD, D - _RD) if isinstance(c, int) else jnp.minimum(c * _RD, D - _RD)

    def stage_copy(t, c):
        src = (wq_hbm, wk_hbm, wv_hbm)[t].bitcast(_U32)
        rows = _ds(retile_row(c) * H // 2, _RD * H // 2, 8 * H)
        return pltpu.make_async_copy(src.at[rows], stage_v.at[c % 2, t], sem_s.at[c % 2, t])

    wo_copies = [pltpu.make_async_copy(
        wo_hbm.bitcast(_U32).at[pl.ds(m * dh, dh), pl.ds(j * 128, 128)],
        wa_v.at[_wo_slab(H, m, j)], sem_o.at[j, m])
        for j in range(D // 128) for m in range(H * E // D)]
    w1_copies = [pltpu.make_async_copy(w1_hbm.bitcast(_U32).at[:, pl.ds(k * dh, dh)], w3_v.at[k],
                                       sem_w.at[k]) for k in range(2)]
    w2_copies = [pltpu.make_async_copy(w2_hbm.bitcast(_U32).at[pl.ds(k * dq, dq)], w4_v.at[k],
                                       sem_w.at[2 + k]) for k in range(2)]

    nil_s[0] = 0
    x_copy(0).start()
    x_copy(1).start()
    w1_copies[0].start()
    for r in (0, _PAD + S):
        _put(h_v, pl.ds(r, _PAD), 0, jnp.zeros((_PAD, D), _F32))
    x_copy(0).wait()
    zero = _zero_bits(x_v)

    def mark(v, r=0):
        return pltpu.bitcast(v[r:r + 8, :128], _U32) & zero

    def norm(rows, z):
        nil = nil_s[0]

        def load(k):
            w = [_pack(x_v[_ds(r + 16 * k * nil, 16, 16), :]) for r in rows]
            return jnp.concatenate([h for v in w for h in _split(v if k else _after(v, z))], axis=0)

        xn, y = _layernorm_twice(load)
        for k, r in enumerate(rows):
            for odd in range(2):
                _put(xn_v, pl.ds(r + odd, 8, stride=2), 0, xn[16 * k + 8 * odd:16 * k + 8 * odd + 8])
        return y

    def norm_jobs(i):
        def job(r, z):
            y = norm((i * _TM + r, i * _TM + th + r), z)
            even, odd = (_operands(_LHS_TERMS, [y[k + a:k + a + 8, c:c + dh]
                                                for a in (0, 16) for c in (0, dh)]) for k in (0, 8))
            for p in range(7):
                y_v[i % 2, p, pl.ds(r // 2, 8), :] = _pair(even[p], odd[p])
            return functools.reduce(jnp.bitwise_or, [mark(y, k) for k in range(0, 32, 8)])

        return [functools.partial(job, r) for r in range(0, th, 16)]

    def shift_jobs(i, combine):
        def job(r0, c0, z):
            def load(r, c, odd):
                shift = (-1, 1, -2, 2)[(c + c0) // dq]
                rows = pl.ds(i * _TM + _PAD + r + r0 + shift + odd, _SM // 2, stride=2)
                return _after(h_v[(c + c0) // 128, rows, :], z)

            even, odd = (combine([load(r, c, k) for r, c in corners]) for k in range(2))
            for p in range(len(even)):
                g_v[p, pl.ds(r0 // 2, _SM // 2), pl.ds(c0, 128)] = _pair(even[p], odd[p])

        return [functools.partial(job, r0, c0) for r0, c0 in tiles]

    def weight_jobs(w_v, word):
        def job(k, c, z):
            quads = [word(r, q, k, c) for r in range(2) for q in range(2)]
            high = z | _U32(0xFFFF0000)
            even = _operands(_RHS_TERMS, [pltpu.bitcast(w << 16, _F32) for w in quads])
            odd = _operands(_RHS_TERMS, [pltpu.bitcast(w & high, _F32) for w in quads])
            for p in (0, 2, 3, 5, 6):
                w_v[p, pl.ds(k, 8), pl.ds(c, 128)] = _pair(even[p], odd[p])
            w_v[1, pl.ds(k, 8), pl.ds(c, 128)] = quads[0]
            w_v[4, pl.ds(k, 8), pl.ds(c, 128)] = quads[3]

        return [functools.partial(job, k, c) for c in range(0, dh, 128) for k in range(0, dq, 8)]

    def plain(lhs, rhs, put, c0, c1):
        marks = []
        for c in range(c0, c1, 128):
            for r0 in range(0, th, _SM):
                for q in (2, 0):
                    y = jnp.concatenate([_unpack(lhs[q + n, pl.ds(r0 // 2, _SM // 2), :])
                                         for n in range(2)], axis=1)
                    v = _dot(y, _unpack(rhs(c)))
                    put(q // 2 * th + r0, c, v)
                    marks.append(mark(v))
        return marks

    def fast(lhs, w_v, put):
        marks = []
        for r0, c0 in tiles:
            marks += [mark(v) for v in _strassen(
                lambda p: _dot(_unpack(lhs[p, pl.ds(r0 // 2, _SM // 2), :]),
                               _unpack(w_v[p, :, pl.ds(c0, 128)])),
                lambda q, v: put(corners[q][0] + r0, corners[q][1] + c0, v))]
        return marks

    def put_h(i):
        return lambda r, c, v: _put(h_v, pl.ds(_PAD + i * _TM + r, _SM), c, _gelu(v))

    def put_x1(i):
        held = {}

        def put(r, c, v):
            v = v + xn_v[c // 128, pl.ds(i * _TM + r, _SM), :]
            (t0_v, t1_v)[i % 2][c // 128, pl.ds(r, _SM), :] = v
            quadrant, key = 2 * (r // th) + c // dh, (r % th, c % dh)
            held[key, quadrant] = v
            seeds = {0: [(6, v)], 1: [(2, v)], 2: [(1, v)], 3: []}[quadrant]
            if quadrant and all((key, n) in held for n in (1, 2, 3)):
                seeds.append((5, held[key, 3] + (held[key, 2] - held[key, 1])))
            for p, w in seeds:
                ffn_v[p, 2 * (r % th // tq) + c % dh // dq, pl.ds(i * tq + r % tq, _SM),
                      pl.ds(c % dq, 128)] = w

        return put

    def ffn_norm_jobs(i):
        t_v, nil = (t0_v, t1_v)[i % 2], nil_s[0]

        def mean(parts):
            return jnp.sum(functools.reduce(jnp.add, parts), axis=-1, keepdims=True) * (1.0 / D)

        def normalise(r, z):
            def load(k):
                return [t_v[c + k * nil, pl.ds(r, 32), :] for c in range(D // 128)]

            x1 = load(1)
            m = mean([_after(x1[0], z)] + x1[1:])
            inv = 0.5 * lax.rsqrt(mean([(e - m) * (e - m) for e in load(2)]) + _EPS)
            for c, e in enumerate(load(3)):
                e = (e - m) * inv
                t2_v[c, pl.ds(r, 32), :] = e
            return _any([mark(e, k) for k in range(0, 32, 8)])

        def sums(r, c, p, z):
            r0 = r // 32 * 32 + r % 32 // 16
            lo, hi = (_operands7(_LHS_TERMS, lambda a, b: _after(
                t2_v[(b * dq + c) // 128, pl.ds(a * tq + r0 + k, 8, stride=4), :], z), p)
                for k in (0, 2))
            for k in range(7):
                lo[k] = _pair(lo[k], hi[k])
                f_v[7 * p + k, pl.ds((i * tq + r) // 2, 8), pl.ds(c, 128)] = lo[k]
            return _any(lo) & zero

        return ([functools.partial(normalise, a * tq + r) for r in range(0, tq, 32) for a in range(4)],
                [functools.partial(sums, r, c, p)
                 for r in range(0, tq, 16) for c in range(0, dq, 128) for p in range(7)])

    def w3_jobs(c):
        return _fill_jobs(b0_v, lambda r, k, j: w3_v[
            c % 2, pl.ds(r * dq // 2 + j, 8), pl.ds(k * 128, 128)])

    def w4_jobs(c):
        return _fill_jobs(b1_v, lambda r, k, j: w4_v[
            c % 2, pl.ds(r * 64 + j % 64, 8), pl.ds(k * dq + j // 64 * 128, 128)])

    def fast_lhs(quadrants):
        return _operands(_LHS_TERMS, quadrants)

    y0 = norm(range(0, _TM, 16), zero)
    for r in range(0, _TM, 16):
        for k in range(2):
            y_v[0, 2 * (r // th) + k, pl.ds(r % th // 2, 8), :] = _pair(
                y0[r:r + 8, k * dh:(k + 1) * dh], y0[r + 8:r + 16, k * dh:(k + 1) * dh])

    x_copy(1).wait()
    w1_copies[1].start()
    w1_copies[0].wait()
    x_copy(2).start()
    marks = plain(y_v.at[0], lambda c: w3_v[0, :, pl.ds(c, 128)], put_h(0), 0, dh)
    jobs = norm_jobs(1)
    _spread(jobs[:5], marks, 0, 0.75)
    w1_copies[1].wait()
    for cp in w2_copies:
        cp.start()
    x_copy(3).start()
    marks = plain(y_v.at[0], lambda c: w3_v[1, :, pl.ds(c - dh, 128)], put_h(0), dh, D)
    _spread(weight_jobs(w1_v, lambda r, q, k, c: w3_v[q, pl.ds(r * dq + k, 8), pl.ds(c, 128)]), marks)
    _spread(jobs[5:], marks, 0, 0.75)

    x_copy(2).wait()
    for k in range(4, nblk):
        x_copy(k).start()
    w3_copy(0).start()
    marks = fast(y_v.at[1], w1_v, put_h(1))
    _spread(shift_jobs(0, list), marks, 0.1, 0.9)
    _spread(norm_jobs(2), marks, 0, 0.8)
    for cp in w2_copies:
        cp.wait()
    x_copy(3).wait()
    marks = plain(g_v, lambda c: jnp.concatenate(
        [w4_v[n, :, pl.ds(c, 128)] for n in range(2)], axis=0), put_x1(0), 0, D)
    _spread(weight_jobs(w2_v, lambda r, q, k, c: w4_v[r, pl.ds(k, 8), pl.ds(q * dh + c, 128)]), marks)

    for k in range(4, nblk):
        x_copy(k).wait()
    w3_copy(0).wait()
    w3_copy(1).start()
    w4_copy(0).start()
    for t in range(3):
        stage_copy(t, 0).start()
    for cp in wo_copies:
        cp.start()
    prev = None
    for i in range(2, nblk + 1):
        marks = []
        if i < nblk:
            marks += fast(y_v.at[i % 2], w1_v, put_h(i))
            _spread(shift_jobs(i - 1, fast_lhs), marks, 0.1, 0.9)
        else:
            _spread(shift_jobs(i - 1, fast_lhs), [zero])
        marks += fast(g_v, w2_v, put_x1(i - 1))
        if i + 1 == nblk:
            _spread(w3_jobs(0), marks, 0.02, 0.8)
        normalise, sums = ffn_norm_jobs(i - 2)
        if i + 1 < nblk:
            jobs = [job for pair in zip(normalise, norm_jobs(i + 1)) for job in pair]
            _spread(jobs, marks, 0.02, 0.8, prev)
        else:
            _spread(normalise, marks, 0, 0.55, prev)
        prev = _spread(sums, marks, 0.6, 0.99)
    for jobs in ffn_norm_jobs(nblk - 1):
        for job in jobs:
            job(zero)

    def late_jobs(i):
        def job(c, p, z):
            lo, hi = (_operands7(_LHS_TERMS, lambda a, b: _after(xn_v[
                (b * dq + c) // 128, _ds(i * _TM + (4 * k + a + 1) * seg - _LATE, _LATE, _LATE), :],
                z), p) for k in range(2))
            for k in range(7):
                a_v[7 * p + k, _ds(i * _LATE, _LATE, _LATE), pl.ds(c, 128)] = _pack(
                    jnp.concatenate([lo[k], hi[k]], axis=0))

        return [functools.partial(job, c, p) for c in range(0, dq, 128) for p in range(7)]

    def hidden_rows(k, r, n):
        return pl.ds(k * S // 8 + r // 2, n // 2)

    def ffn(c, _):
        @pl.when(c + 1 < nfc)
        def _():
            for t in range(3):
                stage_copy(t, c + 1).start()
            w4_copy(c + 1).start()
            w3_copy(c + 1).wait()

        @pl.when(c + 2 < nfc)
        def _():
            w3_copy(c + 2).start()

        w4_copy(c).wait()
        for t in range(3):
            stage_copy(t, c).wait()

        def retile(t, r, jh, odd, z):
            v = stage_v[c % 2, t, pl.ds(r * H, 8 * H), :].reshape(8, H, E)
            a, b = v[:, 8 * jh:8 * jh + 8], v[:, H // 2 + 8 * jh:H // 2 + 8 * jh + 8]
            low = (z | _U32(0xFFFF))[None]
            w = ((a >> 16) | (b & ~low)) if odd else ((a & low) | (b << 16))
            w = jnp.swapaxes(w, 0, 1)
            rows = _ds(retile_row(c) // 2 + r, 8, 8)
            for j in range(8):
                wa_v[6 * (8 * jh + j) + 3 * odd + t, rows, :] = w[j]

        def activate(r0, hid, marks):
            def act(a, b, z):
                hid[a, b] = _gelu(_after(hid[a, b], z))

            _spread([functools.partial(act, a, b) for a in range(2) for b in range(4)],
                    marks, 0.03, 0.9)
            for p in _ORDER:
                for r in range(0, tq, 16):
                    r1 = r // 32 * 32 + r % 32 // 2
                    even, odd = (_operands7(_LHS_TERMS, lambda a, b: hid[a, b][k:k + 8], p)
                                 for k in (r1, r1 + 16))
                    for k in range(7):
                        h_v[p, hidden_rows(k, r0 + r, 16), :] = pltpu.bitcast(
                            _pair(even[k], odd[k]), _F32)

        marks, pending, fills = [], None, w4_jobs(c)
        for r0 in range(0, S // 4, tq):
            hid = {}
            seen = [mark(v) for v in _strassen49(
                lambda p: _dot(_unpack(f_v[p, pl.ds(r0 // 2, tq // 2), :]), _unpack(b0_v[p])),
                lambda a, b, v: hid.__setitem__((a, b), v if a < 2 else _gelu(v)))]
            if pending:
                activate(*pending, seen)
            n = len(fills) // 7
            _spread(fills[r0 // tq * n:][:n], seen)
            pending = (r0, hid)
            marks += seen
        retiles = [functools.partial(retile, t, r, jh, odd) for t in range(3)
                   for r in range(0, _RD // 2, 8) for jh in range(H // 16) for odd in range(2)]
        _spread(retiles[:18], marks, 0.004, 0.98)

        marks = []
        for r0 in range(0, S // 4, tq):
            for j in range(2):
                for p in range(7):
                    def done(q, v):
                        idx = (p, q, pl.ds(r0, tq), pl.ds(j * 128, 128))
                        old = ffn_v[idx]
                        ffn_v[idx] = v + (jnp.where(c > 0, old, 0.0) if p in (0, 3, 4) else old)

                    marks += [mark(v) for v in _strassen(
                        lambda k: _dot(_unpack(h_v[p, hidden_rows(k, r0, tq), :]),
                                       _unpack(b1_v[7 * p + k, pl.ds(j * 64, 64), :])), done)]
            if pending:
                activate(*pending, marks)
                pending = None
        _spread(w3_jobs(jnp.minimum(c + 1, nfc - 1)), marks, 0.2, 0.98)
        _spread(retiles[18:], marks, 0.25, 0.97)
        _spread(late_jobs(c) + late_jobs(c + 1), marks, 0.3, 0.95)
        return 0

    lax.fori_loop(0, nfc, ffn, 0)
    for cp in wo_copies:
        cp.wait()


def _memory(out_hbm, mem0_hbm, x_v, wa_v, a_v, xn_v, ffn_v, b0_v, b1_v, seg,
            pre_v, post_v, a2_v, acc_v, att_v, fin_v, mem0_v, sem):
    S, D = x_v.shape
    H, E = wa_v.shape[0] // 4, wa_v.shape[2]
    dh, dq = D // 2, D // 4
    n_mem, n_seg, early = mem0_hbm.shape[0], S // seg, seg - _LATE
    L = n_mem + seg
    mem0_copy = pltpu.make_async_copy(mem0_hbm, mem0_v, sem.at[1])
    mem0_copy.start()
    zero = _zero_bits(x_v)

    def fill_jobs(b_v, n):
        return _fill_jobs(b_v, lambda r, c, k: wa_v[n + c, pl.ds(r * dq // 2 + k, 8), :])

    def project(n0, lhs, done):
        for j in range(4):
            b_v, marks = (b0_v, b1_v)[j % 2], []
            for r0 in range(0, n_seg * _LATE // 4, _SM):
                marks += [pltpu.bitcast(v[:8], _U32) & zero for v in _strassen49(
                    lambda p: _dot(lhs(j, p, r0), _unpack(b_v[p])),
                    lambda r, c, v: done(j, r, c, r0, v))]
            n = n0 + 4 * j + 4
            n = n if isinstance(n, int) else jnp.minimum(n, 4 * H - 4)
            _spread(fill_jobs((b1_v, b0_v)[j % 2], n), marks[:-3])

    def pre(i, _):
        even = {}

        def done(j, r, c, r0, v):
            if r % 2 == 0:
                even[c] = v
            else:
                pre_v[16 * i + 4 * j + c, r // 2, pl.ds(r0, _SM), :] = _pair(even[c], v)

        project(16 * i, lambda j, p, r0: _unpack(a_v[p, pl.ds(r0 // 2, _SM // 2), :]), done)
        return 0

    _spread(fill_jobs(b0_v, 0), [zero])
    pre(0, 0)
    lax.fori_loop(1, 3 * H // 16, pre, 0)

    row = lax.broadcasted_iota(jnp.int32, (L, L), 0)
    col = lax.broadcasted_iota(jnp.int32, (L, L), 1)
    mask = (row < n_mem) | (row >= col)
    scale = float(E) ** -0.5

    def mixer_out(i, r):
        rows = _ds((i // 2) * (_TM // 4) + (r % 2) * seg, seg, seg)
        cols = [None] * 4
        for b in range(2):
            c = _combine([ffn_v[p, 2 * (r // 2) + b, rows, :] for p in range(7)])
            for k in range(2):
                cols[2 * k + b] = jnp.where(i % 2 == 0, c[k], c[2 + k])
        return jnp.concatenate(cols, axis=1)

    def step(i, r, mem):
        rows = _ds((4 * i + r) * seg, early, seg)
        late = _ds(i * _LATE, _LATE, _LATE)
        h = jnp.concatenate([mem, _get(xn_v, rows)], axis=0).astype(_BF16)
        groups = H // _HG
        qkv, sc = {}, {}

        def project_rows(g):
            slabs = range(3 * _HG * g, 3 * _HG * (g + 1))
            w = jnp.concatenate([_unpack(wa_v[n]) for n in slabs], axis=1)
            if g == 0:
                y = _dot(h[:, :dh], w[:dh])
                y = _dot(h[:, dh:], w[dh:]) + y
            else:
                y = _dot(h, w)
            w = jnp.concatenate([pre_v[n, r // 2, late, :] for n in slabs], axis=1)
            qkv[g] = jnp.concatenate([y, _split(w)[r % 2]], axis=0)

        def part(g, n, t):
            return qkv[g][:, (3 * n + t) * E:(3 * n + t + 1) * E]

        def scores(g):
            sc[g] = [_dot_nt(part(g, n, 0), part(g, n, 1).astype(_BF16)) for n in range(_HG)]

        def attend(g):
            for n in range(_HG):
                z = jnp.where(mask, sc[g][n] * (scale * _LOG2E), -1e9 * _LOG2E)
                e = jnp.exp2(z - jnp.max(z, axis=-1, keepdims=True))
                total = jnp.sum(e, axis=-1, keepdims=True)
                inv = pl.reciprocal(total, approx=True)
                inv = inv * (2.0 - total * inv)
                o = _dot(e * inv, part(g, n, 2).astype(_BF16))
                cols = pl.ds((g * _HG + n) * E, E)
                att_v[:, cols] = _pack(o[:L - _LATE])
                post_v[r, :, cols] = o[L - _LATE:]

        def project_out(g0, g1):
            w = _HG * E
            wo = jnp.concatenate([jnp.concatenate(
                [_unpack(wa_v[_wo_slab(H, k // D, j), pl.ds(k % D // 2, w // 2), :])
                 for k in range(g0 * w, g1 * w, w)], axis=0) for j in range(D // 128)], axis=1)
            return _dot(_unpack(att_v[:, pl.ds(g0 * w, (g1 - g0) * w)]), wo)

        o, cuts = None, (0, groups // 4, groups // 2, groups)
        for t in range(groups + 3):
            if t < groups:
                project_rows(t)
            else:
                d = project_out(cuts[t - groups], cuts[t - groups + 1])
                o = d if o is None else d + o
            if 0 <= t - 2 < groups:
                attend(t - 2)
            if 0 <= t - 1 < groups:
                scores(t - 1)
        rest = x_v[_ds((4 * i + r) * seg, seg, seg), :].astype(_F32) + mixer_out(i, r)
        x_v[rows, :] = (rest[:early] + o[n_mem:]).astype(_BF16)
        _put(acc_v.at[r], late, 0, rest[early:])
        return o[:n_mem]

    def steps(i, mem):
        for r in range(4):
            mem = step(i, r, mem)
        for m in range(H * E // D):
            for c in range(0, dq, 128):
                for p in range(7):
                    for k, v in enumerate(_operands7(_LHS_TERMS, lambda a, b: post_v[
                            a, :, pl.ds(m * D + b * dq + c, 128)], p)):
                        a2_v[7 * p + k, _ds(i * _LATE, _LATE, _LATE), pl.ds(m * dq + c, 128)] = v
        for r in range(4):
            rows = _ds((4 * i + r) * seg, early, seg)
            pltpu.make_async_copy(x_v.at[rows], out_hbm.at[rows], sem.at[0]).start()
        return mem

    mem0_copy.wait()
    lax.fori_loop(0, n_seg // 4, steps, mem0_v[...].astype(_F32))

    def post(i, _):
        partial = {}

        def done(m, r, c, r0, v):
            v = v + (partial.pop((r, c, r0)) if m else acc_v[r, 4 * i + c, pl.ds(r0, _SM), :])
            if m < 3:
                partial[r, c, r0] = v
                return
            for k in range(0, _SM, _LATE):
                fin_v[r, pl.ds(r0 + k, _LATE), _ds((4 * i + c) * 128, 128, 128)] = (
                    v[k:k + _LATE].astype(_BF16))

        project(3 * H + 16 * i, lambda m, p, r0: a2_v[p, pl.ds(r0, _SM), pl.ds(m * dq, dq)], done)
        cols = _ds(i * dh, dh, dh)
        for s in range(n_seg):
            pltpu.make_async_copy(fin_v.at[s % 4, pl.ds(s // 4 * _LATE, _LATE), cols],
                                  out_hbm.at[pl.ds(s * seg + early, _LATE), cols], sem.at[0]).start()
        return 0

    lax.fori_loop(0, 2, post, 0)
    pltpu.make_async_copy(x_v, out_hbm, sem.at[0]).wait()


def _kernel(x_hbm, mem0_hbm, wq_hbm, wk_hbm, wv_hbm, wo_hbm, w1_hbm, w2_hbm, w3_hbm, w4_hbm,
            out_hbm, *shared, seg):
    S, D = x_hbm.shape
    HE = wo_hbm.shape[0]
    n_mem, n_late = mem0_hbm.shape[0], S // seg * _LATE
    pl.run_scoped(
        functools.partial(_mixer, x_hbm, wq_hbm, wk_hbm, wv_hbm, wo_hbm, w1_hbm, w2_hbm, w3_hbm,
                          w4_hbm, *shared, seg),
        pltpu.VMEM((7, D // 4, D // 2), _U32),
        pltpu.VMEM((7, D // 4, D // 2), _U32),
        pltpu.VMEM((2, D // 2, _FC), _U32),
        pltpu.VMEM((2, _FC // 2, D), _U32),
        pltpu.VMEM((49, S // 8, D // 4), _U32),
        pltpu.VMEM((2, 3, _RD * HE // 256, 128), _U32),
        pltpu.VMEM((D // 128, S + 2 * _PAD, 128), _F32),
        pltpu.VMEM((2, 7, _TM // 4, D // 2), _U32),
        pltpu.VMEM((7, _TM // 4, D // 2), _U32),
        pltpu.VMEM((D // 128, _TM, 128), _F32),
        pltpu.VMEM((D // 128, _TM, 128), _F32),
        pltpu.VMEM((D // 128, _TM + _PAD, 128), _F32),
        pltpu.SMEM((1,), jnp.int32),
        pltpu.SemaphoreType.DMA((S // _TM,)),
        pltpu.SemaphoreType.DMA((4,)),
        pltpu.SemaphoreType.DMA((2, 2)),
        pltpu.SemaphoreType.DMA((2, 3)),
        pltpu.SemaphoreType.DMA((D // 128, HE // D)))
    pl.run_scoped(
        functools.partial(_memory, out_hbm, mem0_hbm, *shared, seg),
        pltpu.VMEM((3 * HE // 128, 2, n_late // 4, 128), _U32),
        pltpu.VMEM((4, _LATE, HE), _F32),
        pltpu.VMEM((49, n_late // 4, HE // 4), _F32),
        pltpu.VMEM((4, D // 128, n_late // 4, 128), _F32),
        pltpu.VMEM(((n_mem + seg - _LATE) // 2, HE), _U32),
        pltpu.VMEM((4, n_late // 4, D), _BF16),
        pltpu.VMEM((n_mem, D), _BF16),
        pltpu.SemaphoreType.DMA((2,)))


@functools.partial(jax.jit, static_argnames=("A_seg_len",))
def pallas_parallel_sum__memory_aug_recurrent_mem_tr__mixer_s_mlp__prompt_kernel(
    A_x: jax.Array,
    A_mem0: jax.Array,
    A_Wq: jax.Array,
    A_Wk: jax.Array,
    A_Wv: jax.Array,
    A_Wo: jax.Array,
    A_seg_len: int,
    B_x: jax.Array,
    B_w1: jax.Array,
    B_w2: jax.Array,
    B_w3: jax.Array,
    B_w4: jax.Array,
):
    del B_x
    B, S, D = A_x.shape
    _, H, E = A_Wq.shape
    M = A_mem0.shape[1]
    seg = int(A_seg_len)
    assert (B, S, D, H, E, M, seg, B_w3.shape[1]) == (1, 2048, 1024, 32, 128, 8, 32, 3584)

    hbm = pl.BlockSpec(memory_space=pltpu.HBM)
    out = pl.pallas_call(
        functools.partial(_kernel, seg=seg),
        out_shape=jax.ShapeDtypeStruct((S, D), A_x.dtype),
        in_specs=[hbm] * 10,
        out_specs=hbm,
        scratch_shapes=[
            pltpu.VMEM((S, D), _BF16),
            pltpu.VMEM((4 * H, D // 2, E), _U32),
            pltpu.VMEM((49, S // seg * _LATE // 8, D // 4), _U32),
            pltpu.VMEM((D // 128, S + _PAD, 128), _F32),
            pltpu.VMEM((7, 4, S // 4, D // 4), _F32),
            pltpu.VMEM((49, D // 8, 128), _U32),
            pltpu.VMEM((49, D // 8, 128), _U32),
        ],
        compiler_params=pltpu.CompilerParams(vmem_limit_bytes=126 * 1024 * 1024),
    )(A_x.reshape(S, D), A_mem0.reshape(M, D),
      A_Wq.reshape(D * H, E), A_Wk.reshape(D * H, E), A_Wv.reshape(D * H, E),
      A_Wo.reshape(H * E, D), B_w1, B_w2, B_w3, B_w4)
    return out.reshape(B, S, D)
```

```python
import functools

import jax
import jax.numpy as jnp
import numpy as np
from jax import lax
import jax.experimental.pallas as pl
import jax.experimental.pallas.tpu as pltpu

_F32 = jnp.float32
_BF16 = jnp.bfloat16
_U32 = jnp.uint32

_EPS = 1e-5
_LOG2E = float(np.log2(np.e))
_TM = 256
_SM = 64
_FC = 512
_RD = 160
_HG = 4
_LATE = 8
_PAD = 8


def _dot(a, b):
    return lax.dot_general(a, b, (((1,), (0,)), ((), ())), preferred_element_type=_F32)


def _dot_nt(a, b):
    return lax.dot_general(a, b, (((1,), (1,)), ((), ())), preferred_element_type=_F32)


def _ds(start, size, align):
    return pl.ds(start if isinstance(start, int) else pl.multiple_of(start, align), size)


def _pack(x):
    return pltpu.bitcast(x.astype(_BF16), _U32)


def _unpack(w):
    return pltpu.bitcast(w, _BF16)


def _pair(even, odd):
    return pltpu.pack_elementwise([even, odd], packed_dtype=_BF16)


def _split(w):
    return pltpu.bitcast(w << 16, _F32), pltpu.bitcast(w & _U32(0xFFFF0000), _F32)


def _get(ref, rows):
    return jnp.concatenate([ref[k, rows, :] for k in range(ref.shape[0])], axis=1)


def _put(ref, rows, c0, x):
    for c in range(0, x.shape[1], 128):
        ref[(c0 + c) // 128, rows, :] = x[:, c:c + 128]


def _wo_slab(heads, m, j):
    return 3 * heads + 16 * (j % 4 // 2) + 4 * m + 2 * (j % 2) + j // 4


def _gelu(hx):
    c0 = 2.0 * float(np.sqrt(2.0 / np.pi))
    c1 = 4.0 * 0.044715 * c0
    return hx + hx * jnp.tanh(hx * (c0 + c1 * (hx * hx)))


def _layernorm_twice(load):
    m = jnp.mean(load(0), axis=-1, keepdims=True)
    c = load(1) - m
    mu = jnp.mean(c, axis=-1, keepdims=True)
    v = jnp.mean(c * c, axis=-1, keepdims=True)
    r = lax.rsqrt(v + _EPS)
    r2 = (0.5 * r) * lax.rsqrt((r * r) * jnp.maximum(v - mu * mu, 0.0) + _EPS)
    c = load(2) - m
    return c * r, (c - mu) * r2


def _zero_bits(ref):
    return jnp.where(jnp.abs(ref[:16, :128].astype(_F32)[:8]) < 0.0, 1, 0).astype(_U32)


def _after(x, z):
    w = pltpu.bitcast(x, _U32)
    z = jnp.tile(z, (w.shape[0] // z.shape[0], w.shape[1] // z.shape[1]))
    return pltpu.bitcast(w | z, x.dtype)


def _any(words):
    while len(words) > 1:
        words = [functools.reduce(jnp.bitwise_or, words[k:k + 2]) for k in range(0, len(words), 2)]
    return words[0]


def _spread(jobs, marks, lo=0.0, hi=1.0, prev=None):
    marks = marks[int(lo * len(marks)):int(hi * len(marks))]
    for k, job in enumerate(jobs):
        z = marks[k * len(marks) // len(jobs)]
        prev = job(z if prev is None else z | prev)
    return prev


_LHS_TERMS = ((0, 1, 3), (2, 1, 3), (0, 0, 0), (3, 0, 3), (0, 1, 1), (2, -1, 0), (1, -1, 3))
_RHS_TERMS = ((0, 1, 3), (0, 0, 0), (1, -1, 3), (2, -1, 0), (3, 0, 3), (0, 1, 1), (2, 1, 3))
_ORDER = (0, 1, 3, 5, 6, 2, 4)


_MIXING = (0, 5, 6)


class _Quad:
    def __init__(self, blocks):
        self.blocks = list(blocks)

    def __add__(self, other):
        return _Quad(a + b for a, b in zip(self.blocks, other.blocks))

    def __sub__(self, other):
        return _Quad(a - b for a, b in zip(self.blocks, other.blocks))


def _term(terms, get, p):
    a, sign, b = terms[p]
    return get(a) if sign == 0 else get(a) + get(b) if sign > 0 else get(a) - get(b)


def _operands(terms, quadrants):
    return [_term(terms, quadrants.__getitem__, p) for p in range(7)]


def _block(n, k):
    return 2 * (n // 2) + k // 2, 2 * (n % 2) + k % 2


def _operands7(terms, get, p):
    outer = _term(terms, lambda n: _Quad(get(*_block(n, k)) for k in range(4)), p)
    return _operands(terms, outer.blocks)


def _combine(m):
    m1, m2, m3, m4, m5, m6, m7 = m
    return (m1 + m4) + (m7 - m5), m3 + m5, m2 + m4, (m1 - m2) + (m3 + m6)


def _strassen(prod, done):
    m1, m2 = prod(0), prod(1)
    c22 = m1 - m2
    m4 = prod(3)
    done(2, m2 + m4)
    c11 = m1 + m4
    c22 = prod(5) + c22
    c11 = prod(6) + c11
    m3 = prod(2)
    done(3, c22 + m3)
    m5 = prod(4)
    done(0, c11 - m5)
    done(1, m3 + m5)
    return m1, m2, m4, c22, c11, m3, m5


def _strassen49(prod, done):
    seen = []

    def outer(p):
        out = [None] * 4
        m = _strassen(lambda k: prod(7 * p + k), out.__setitem__)
        seen.extend(m[k] for k in (0, 1, 3, 4))
        return _Quad(out)

    def finish(n, quad):
        for k, v in enumerate(quad.blocks):
            done(*_block(n, k), v)

    _strassen(outer, finish)
    return seen


def _halves(z):
    shift, high = z | _U32(16), z | _U32(0xFFFF0000)
    return (lambda w: pltpu.bitcast(w << shift, _F32)), (lambda w: pltpu.bitcast(w & high, _F32))


def _fill_jobs(b_v, word, slots=tuple(zip(_ORDER, _ORDER))):
    def job(n, p, k, z):
        even, odd = (_operands7(_RHS_TERMS, lambda r, c: half(word(r, c, k)), p)
                     for half in _halves(z))
        for j in range(7):
            b_v[7 * n + j, pl.ds(k, 8), :] = _pair(even[j], odd[j])

    return [functools.partial(job, n, p, k) for n, p in slots for k in range(0, b_v.shape[1], 8)]


def _mixer(x_hbm, wq_hbm, wk_hbm, wv_hbm, w1_hbm, w2_hbm, w3_hbm, w4_hbm,
           x_v, wa_v, a_v, xn_v, ffn_v, b0_v, b1_v, seg,
           w1_v, w2_v, w3_v, w4_v, f_v, stage_v, h_v, y_v, g_v, t0_v, t1_v, t2_v, nil_s,
           sem_x, sem_w, sem_f, sem_s):
    S, D = x_v.shape
    H, E = wa_v.shape[0] // 4, wa_v.shape[2]
    dh, dq, th, tq = D // 2, D // 4, _TM // 2, _TM // 4
    nblk = S // _TM
    nfc = w3_hbm.shape[1] // _FC
    corners = [(r, c) for r in (0, th) for c in (0, dh)]
    tiles = [(r, c) for r in range(0, th, _SM) for c in range(0, dh, 128)]

    def x_copy(i):
        rows = pl.ds(i * _TM, _TM)
        return pltpu.make_async_copy(x_hbm.at[rows], x_v.at[rows], sem_x.at[i])

    def w3_copy(c):
        src = w3_hbm.bitcast(_U32).at[:, _ds(c * _FC, _FC, _FC)]
        return pltpu.make_async_copy(src, w3_v.at[c % 2], sem_f.at[c % 2, 0])

    def w4_copy(c):
        src = w4_hbm.bitcast(_U32).at[_ds(c * _FC // 2, _FC // 2, _FC // 2)]
        return pltpu.make_async_copy(src, w4_v.at[c % 2], sem_f.at[c % 2, 1])

    def retile_row(c):
        return min(c * _RD, D - _RD) if isinstance(c, int) else jnp.minimum(c * _RD, D - _RD)

    def stage_copy(t, c):
        src = (wq_hbm, wk_hbm, wv_hbm)[t].bitcast(_U32)
        rows = _ds(retile_row(c) * H // 2, _RD * H // 2, 8 * H)
        return pltpu.make_async_copy(src.at[rows], stage_v.at[c % 2, t], sem_s.at[c % 2, t])

    w1_copies = [pltpu.make_async_copy(w1_hbm.bitcast(_U32).at[:, pl.ds(k * dh, dh)], w3_v.at[k],
                                       sem_w.at[k]) for k in range(2)]
    w2_copies = [pltpu.make_async_copy(w2_hbm.bitcast(_U32).at[pl.ds(k * dq, dq)], w4_v.at[k],
                                       sem_w.at[2 + k]) for k in range(2)]

    nil_s[0] = 0
    x_copy(0).start()
    x_copy(1).start()
    w1_copies[0].start()
    for r in (0, _PAD + S):
        _put(h_v, pl.ds(r, _PAD), 0, jnp.zeros((_PAD, D), _F32))
    x_copy(0).wait()
    zero = _zero_bits(x_v)

    def mark(v, r=0):
        return pltpu.bitcast(v[r:r + 8, :128], _U32) & zero

    def norm(rows, z):
        nil = nil_s[0]

        def load(k):
            w = [_pack(x_v[_ds(r + 16 * k * nil, 16, 16), :]) for r in rows]
            return jnp.concatenate([h for v in w for h in _split(v if k else _after(v, z))], axis=0)

        xn, y = _layernorm_twice(load)
        for k, r in enumerate(rows):
            for odd in range(2):
                _put(xn_v, pl.ds(r + odd, 8, stride=2), 0, xn[16 * k + 8 * odd:16 * k + 8 * odd + 8])
        return y

    def norm_jobs(i):
        def job(r, z):
            y = norm((i * _TM + r, i * _TM + th + r), z)
            even, odd = (_operands(_LHS_TERMS, [y[k + a:k + a + 8, c:c + dh]
                                                for a in (0, 16) for c in (0, dh)]) for k in (0, 8))
            for p in range(7):
                y_v[i % 2, p, pl.ds(r // 2, 8), :] = _pair(even[p], odd[p])
            return functools.reduce(jnp.bitwise_or, [mark(y, k) for k in range(0, 32, 8)])

        return [functools.partial(job, r) for r in range(0, th, 16)]

    def shift_jobs(i, combine):
        def job(r0, c0, z):
            def load(r, c, odd):
                shift = (-1, 1, -2, 2)[(c + c0) // dq]
                rows = pl.ds(i * _TM + _PAD + r + r0 + shift + odd, _SM // 2, stride=2)
                return _after(h_v[(c + c0) // 128, rows, :], z)

            even, odd = (combine([load(r, c, k) for r, c in corners]) for k in range(2))
            for p in range(len(even)):
                g_v[p, pl.ds(r0 // 2, _SM // 2), pl.ds(c0, 128)] = _pair(even[p], odd[p])

        return [functools.partial(job, r0, c0) for r0, c0 in tiles]

    def weight_jobs(w_v, word):
        def job(k, c, z):
            quads = [word(r, q, k, c) for r in range(2) for q in range(2)]
            high = z | _U32(0xFFFF0000)
            even = _operands(_RHS_TERMS, [pltpu.bitcast(w << 16, _F32) for w in quads])
            odd = _operands(_RHS_TERMS, [pltpu.bitcast(w & high, _F32) for w in quads])
            for p in (0, 2, 3, 5, 6):
                w_v[p, pl.ds(k, 8), pl.ds(c, 128)] = _pair(even[p], odd[p])
            w_v[1, pl.ds(k, 8), pl.ds(c, 128)] = quads[0]
            w_v[4, pl.ds(k, 8), pl.ds(c, 128)] = quads[3]

        return [functools.partial(job, k, c) for c in range(0, dh, 128) for k in range(0, dq, 8)]

    def plain(lhs, rhs, put, c0, c1):
        marks = []
        for c in range(c0, c1, 128):
            for r0 in range(0, th, _SM):
                for q in (2, 0):
                    y = jnp.concatenate([_unpack(lhs[q + n, pl.ds(r0 // 2, _SM // 2), :])
                                         for n in range(2)], axis=1)
                    v = _dot(y, _unpack(rhs(c)))
                    put(q // 2 * th + r0, c, v)
                    marks.append(mark(v))
        return marks

    def fast(lhs, w_v, put):
        marks = []
        for r0, c0 in tiles:
            marks += [mark(v) for v in _strassen(
                lambda p: _dot(_unpack(lhs[p, pl.ds(r0 // 2, _SM // 2), :]),
                               _unpack(w_v[p, :, pl.ds(c0, 128)])),
                lambda q, v: put(corners[q][0] + r0, corners[q][1] + c0, v))]
        return marks

    def put_h(i):
        return lambda r, c, v: _put(h_v, pl.ds(_PAD + i * _TM + r, _SM), c, _gelu(v))

    def put_x1(i):
        held = {}

        def put(r, c, v):
            v = v + xn_v[c // 128, pl.ds(i * _TM + r, _SM), :]
            (t0_v, t1_v)[i % 2][c // 128, pl.ds(r, _SM), :] = v
            quadrant, key = 2 * (r // th) + c // dh, (r % th, c % dh)
            held[key, quadrant] = v
            seeds = {0: [(6, v)], 1: [(2, v)], 2: [(1, v)], 3: []}[quadrant]
            if quadrant and all((key, n) in held for n in (1, 2, 3)):
                seeds.append((5, held[key, 3] + (held[key, 2] - held[key, 1])))
            for p, w in seeds:
                ffn_v[p, 2 * (r % th // tq) + c % dh // dq, pl.ds(i * tq + r % tq, _SM),
                      pl.ds(c % dq, 128)] = w

        return put

    def ffn_norm_jobs(i):
        t_v, nil = (t0_v, t1_v)[i % 2], nil_s[0]

        def mean(parts):
            return jnp.sum(functools.reduce(jnp.add, parts), axis=-1, keepdims=True) * (1.0 / D)

        def normalise(r, z):
            def load(k):
                return [t_v[c + k * nil, pl.ds(r, 32), :] for c in range(D // 128)]

            x1 = load(1)
            m = mean([_after(x1[0], z)] + x1[1:])
            inv = 0.5 * lax.rsqrt(mean([(e - m) * (e - m) for e in load(2)]) + _EPS)
            for c, e in enumerate(load(3)):
                e = (e - m) * inv
                t2_v[c, pl.ds(r, 32), :] = e
            return _any([mark(e, k) for k in range(0, 32, 8)])

        def sums(r, c, p, z):
            r0 = r // 32 * 32 + r % 32 // 16
            lo, hi = (_operands7(_LHS_TERMS, lambda a, b: _after(
                t2_v[(b * dq + c) // 128, pl.ds(a * tq + r0 + k, 8, stride=4), :], z), p)
                for k in (0, 2))
            for k in range(7):
                lo[k] = _pair(lo[k], hi[k])
                f_v[7 * p + k, pl.ds((i * tq + r) // 2, 8), pl.ds(c, 128)] = lo[k]
            return _any(lo) & zero

        return ([functools.partial(normalise, a * tq + r) for r in range(0, tq, 32) for a in range(4)],
                [functools.partial(sums, r, c, p)
                 for r in range(0, tq, 16) for c in range(0, dq, 128) for p in range(7)])

    def w3_jobs(c):
        return _fill_jobs(b0_v, lambda r, k, j: w3_v[
            c % 2, pl.ds(r * dq // 2 + j, 8), pl.ds(k * 128, 128)])

    def w4_jobs(c):
        return _fill_jobs(b1_v, lambda r, k, j: w4_v[
            c % 2, pl.ds(r * 64 + j % 64, 8), pl.ds(k * dq + j // 64 * 128, 128)])

    def fast_lhs(quadrants):
        return _operands(_LHS_TERMS, quadrants)

    y0 = norm(range(0, _TM, 16), zero)
    for r in range(0, _TM, 16):
        for k in range(2):
            y_v[0, 2 * (r // th) + k, pl.ds(r % th // 2, 8), :] = _pair(
                y0[r:r + 8, k * dh:(k + 1) * dh], y0[r + 8:r + 16, k * dh:(k + 1) * dh])

    x_copy(1).wait()
    w1_copies[1].start()
    w1_copies[0].wait()
    x_copy(2).start()
    marks = plain(y_v.at[0], lambda c: w3_v[0, :, pl.ds(c, 128)], put_h(0), 0, dh)
    jobs = norm_jobs(1)
    _spread(jobs[:5], marks, 0, 0.75)
    w1_copies[1].wait()
    for cp in w2_copies:
        cp.start()
    x_copy(3).start()
    marks = plain(y_v.at[0], lambda c: w3_v[1, :, pl.ds(c - dh, 128)], put_h(0), dh, D)
    _spread(weight_jobs(w1_v, lambda r, q, k, c: w3_v[q, pl.ds(r * dq + k, 8), pl.ds(c, 128)]), marks)
    _spread(jobs[5:], marks, 0, 0.75)

    x_copy(2).wait()
    for k in range(4, nblk):
        x_copy(k).start()
    w3_copy(0).start()
    marks = fast(y_v.at[1], w1_v, put_h(1))
    _spread(shift_jobs(0, list), marks, 0.1, 0.9)
    _spread(norm_jobs(2), marks, 0, 0.8)
    for cp in w2_copies:
        cp.wait()
    x_copy(3).wait()
    marks = plain(g_v, lambda c: jnp.concatenate(
        [w4_v[n, :, pl.ds(c, 128)] for n in range(2)], axis=0), put_x1(0), 0, D)
    _spread(weight_jobs(w2_v, lambda r, q, k, c: w4_v[r, pl.ds(k, 8), pl.ds(q * dh + c, 128)]), marks)

    for k in range(4, nblk):
        x_copy(k).wait()
    w3_copy(0).wait()
    w3_copy(1).start()
    w4_copy(0).start()
    for t in range(3):
        stage_copy(t, 0).start()
    prev = None
    for i in range(2, nblk + 1):
        marks = []
        if i < nblk:
            marks += fast(y_v.at[i % 2], w1_v, put_h(i))
            _spread(shift_jobs(i - 1, fast_lhs), marks, 0.1, 0.9)
        else:
            _spread(shift_jobs(i - 1, fast_lhs), [zero])
        marks += fast(g_v, w2_v, put_x1(i - 1))
        if i + 1 == nblk:
            _spread(w3_jobs(0), marks, 0.02, 0.8)
        normalise, sums = ffn_norm_jobs(i - 2)
        if i + 1 < nblk:
            jobs = [job for pair in zip(normalise, norm_jobs(i + 1)) for job in pair]
            _spread(jobs, marks, 0.02, 0.8, prev)
        else:
            _spread(normalise, marks, 0, 0.55, prev)
        prev = _spread(sums, marks, 0.6, 0.99)
    for jobs in ffn_norm_jobs(nblk - 1):
        for job in jobs:
            job(zero)

    def late_jobs(i):
        def job(r, c, n, z):
            def rows(a, k):
                return _ds(i * _TM + (4 * r + 2 * k + a % 2 + 1) * seg + (a // 2 - 2) * _LATE,
                           _LATE, _LATE)

            lo, hi = (_operands7(_LHS_TERMS, lambda a, b: _after(
                xn_v[(b * dq + c) // 128, rows(a, k), :], z), _MIXING[n]) for k in range(2))
            for k in range(7):
                a_v[7 * n + k, _ds((2 * i + r) * _LATE, _LATE, _LATE), pl.ds(c, 128)] = _pack(
                    jnp.concatenate([lo[k], hi[k]], axis=0))

        return [functools.partial(job, r, c, n)
                for r in range(2) for c in range(0, dq, 128) for n in range(3)]

    def hidden_rows(k, r, n):
        return pl.ds(k * S // 8 + r // 2, n // 2)

    def ffn(c, _):
        @pl.when(c + 1 < nfc)
        def _():
            for t in range(3):
                stage_copy(t, c + 1).start()
            w4_copy(c + 1).start()
            w3_copy(c + 1).wait()

        @pl.when(c + 2 < nfc)
        def _():
            w3_copy(c + 2).start()

        w4_copy(c).wait()
        for t in range(3):
            stage_copy(t, c).wait()

        def retile(t, r, jh, odd, z):
            v = stage_v[c % 2, t, pl.ds(r * H, 8 * H), :].reshape(8, H, E)
            a, b = v[:, 8 * jh:8 * jh + 8], v[:, H // 2 + 8 * jh:H // 2 + 8 * jh + 8]
            low = (z | _U32(0xFFFF))[None]
            w = ((a >> 16) | (b & ~low)) if odd else ((a & low) | (b << 16))
            w = jnp.swapaxes(w, 0, 1)
            rows = _ds(retile_row(c) // 2 + r, 8, 8)
            for j in range(8):
                wa_v[6 * (8 * jh + j) + 3 * odd + t, rows, :] = w[j]

        def activate(r0, hid, marks):
            def act(a, b, z):
                hid[a, b] = _gelu(_after(hid[a, b], z))

            _spread([functools.partial(act, a, b) for a in range(2) for b in range(4)],
                    marks, 0.03, 0.9)
            for p in _ORDER:
                for r in range(0, tq, 16):
                    r1 = r // 32 * 32 + r % 32 // 2
                    even, odd = (_operands7(_LHS_TERMS, lambda a, b: hid[a, b][k:k + 8], p)
                                 for k in (r1, r1 + 16))
                    for k in range(7):
                        h_v[p, hidden_rows(k, r0 + r, 16), :] = pltpu.bitcast(
                            _pair(even[k], odd[k]), _F32)

        marks, pending, fills = [], None, w4_jobs(c)
        for r0 in range(0, S // 4, tq):
            hid = {}
            seen = [mark(v) for v in _strassen49(
                lambda p: _dot(_unpack(f_v[p, pl.ds(r0 // 2, tq // 2), :]), _unpack(b0_v[p])),
                lambda a, b, v: hid.__setitem__((a, b), v if a < 2 else _gelu(v)))]
            if pending:
                activate(*pending, seen)
            n = len(fills) // 7
            _spread(fills[r0 // tq * n:][:n], seen)
            pending = (r0, hid)
            marks += seen
        retiles = [functools.partial(retile, t, r, jh, odd) for t in range(3)
                   for r in range(0, _RD // 2, 8) for jh in range(H // 16) for odd in range(2)]
        _spread(retiles[:18], marks, 0.004, 0.98)

        marks = []
        for r0 in range(0, S // 4, tq):
            for j in range(2):
                for p in range(7):
                    def done(q, v):
                        idx = (p, q, pl.ds(r0, tq), pl.ds(j * 128, 128))
                        old = ffn_v[idx]
                        ffn_v[idx] = v + (jnp.where(c > 0, old, 0.0) if p in (0, 3, 4) else old)

                    marks += [mark(v) for v in _strassen(
                        lambda k: _dot(_unpack(h_v[p, hidden_rows(k, r0, tq), :]),
                                       _unpack(b1_v[7 * p + k, pl.ds(j * 64, 64), :])), done)]
            if pending:
                activate(*pending, marks)
                pending = None
        _spread(w3_jobs(jnp.minimum(c + 1, nfc - 1)), marks, 0.2, 0.98)
        _spread(retiles[18:], marks, 0.25, 0.97)
        _spread(late_jobs(c) + late_jobs(c + 1), marks, 0.3, 0.95)
        return 0

    lax.fori_loop(0, nfc, ffn, 0)


def _memory(out_hbm, mem0_hbm, wo_hbm, x_v, wa_v, a_v, xn_v, ffn_v, b0_v, b1_v, seg,
            wo_v, pre_v, post_v, a2_v, acc_v, att_v, fin_v, mem0_v, sem, sem_o):
    S, D = x_v.shape
    H, E = wa_v.shape[0] // 4, wa_v.shape[2]
    dh, dq = D // 2, D // 4
    n_mem, n_seg, early = mem0_hbm.shape[0], S // seg, seg - 2 * _LATE
    L = n_mem + seg
    mem0_copy = pltpu.make_async_copy(mem0_hbm, mem0_v, sem.at[1])
    mem0_copy.start()

    def wo_copies(q, raw=0):
        copies = []
        for k in range(8):
            m, j = 2 * (q % 2) + k // 4, 4 * (k % 2) + 2 * (q // 2) + k % 4 // 2
            src = wo_hbm.bitcast(_U32).at[_ds(m * dh, dh, dh), _ds(j * 128, 128, 128)]
            dst = wo_v.at[8 * q + k] if raw else wa_v.at[3 * H + 8 * q + k]
            copies.append(pltpu.make_async_copy(src, dst, sem_o.at[4 * raw + q, k]))
        return copies

    zero = _zero_bits(x_v)

    def fill_jobs(b_v, w_v, n):
        return _fill_jobs(b_v, lambda r, c, k: w_v[
            n + 2 * (c % 2) + c // 2, pl.ds(r * dq // 2 + k, 8), :], tuple(enumerate(_MIXING)))

    def loop_form_jobs(slabs):
        def job(n, k, z):
            quads = [wa_v[n + c, pl.ds(r * dq + k, 16), :] for r in range(2) for c in range(2)]
            even, odd = ([half(w) for w in quads] for half in _halves(jnp.tile(z, (2, 1))))
            wa_v[n + 1, pl.ds(k, 16), :] = _pair(even[1] - even[3], odd[1] - odd[3])
            wa_v[n, pl.ds(dq + k, 16), :] = _pair(even[2] - even[0], odd[2] - odd[0])

        return [functools.partial(job, n, k) for n in slabs for k in range(0, dq, 16)]

    def project(lhs, done, jobs):
        for j in range(4):
            b_v, marks = (b0_v, b1_v)[j % 2], []
            for r0 in range(0, n_seg * _LATE // 2, _SM):
                m = []
                for n in range(3):
                    m.append([None] * 4)
                    seen = _strassen(lambda k: _dot(lhs(j, 7 * n + k, r0), _unpack(b_v[7 * n + k])),
                                     m[n].__setitem__)
                    marks += [pltpu.bitcast(seen[k][:8], _U32) & zero for k in (0, 1, 3, 4)]
                for k in range(4):
                    done(j, k, r0, m[0][k] + m[2][k], m[0][k] + m[1][k])
            for some in jobs(j, (b1_v, b0_v)[j % 2]):
                _spread(some, marks[:-3])

    def pre(i):
        def done(j, k, r0, c11, c22):
            pre_v[8 * i + 2 * j + k % 2, k // 2, pl.ds(r0, _SM), :] = _pair(c11, c22)

        def jobs(j, b_v):
            n = 16 * i + 4 * j
            if not isinstance(i, int):
                return [fill_jobs(b_v, wa_v, n + 4),
                        loop_form_jobs((n, n + 2, 3 * H + 8 * (i - 1) + 2 * j))]
            return [fill_jobs(b_v, wa_v, n + 4) if n + 4 < 3 * H else fill_jobs(b_v, wo_v, 0),
                    loop_form_jobs((n, n + 2))]

        project(lambda j, p, r0: _unpack(a_v[p, pl.ds(r0 // 2, _SM // 2), :]), done, jobs)

    for cp in wo_copies(0):
        cp.start()
    _spread(fill_jobs(b0_v, wa_v, 0), [zero])
    pre(0)

    for cp in wo_copies(0, raw=1):
        cp.start()

    @pl.loop(1, 5)
    def _(i):
        @pl.when(i < 4)
        def _():
            for cp in wo_copies(i):
                cp.start()

        for cp in wo_copies(i - 1):
            cp.wait()
        pre(i)

    for cp in wo_copies(0, raw=1):
        cp.wait()
    pre(5)
    rest_of_wo = [cp for q in range(1, 4) for cp in wo_copies(q, raw=1)]
    for cp in rest_of_wo:
        cp.start()

    row = lax.broadcasted_iota(jnp.int32, (L, L), 0)
    col = lax.broadcasted_iota(jnp.int32, (L, L), 1)
    mask = (row < n_mem) | (row >= col)
    scale = float(E) ** -0.5

    def mixer_out(i, r):
        rows = _ds((i // 2) * (_TM // 4) + (r % 2) * seg, seg, seg)
        cols = [None] * 4
        for b in range(2):
            c = _combine([ffn_v[p, 2 * (r // 2) + b, rows, :] for p in range(7)])
            for k in range(2):
                cols[2 * k + b] = jnp.where(i % 2 == 0, c[k], c[2 + k])
        return jnp.concatenate(cols, axis=1)

    def forms(v):
        n = L - 2 * _LATE
        first = jnp.concatenate([v[:n], v[n + _LATE:]], axis=0)
        second = v[:n + _LATE]
        return ((first[:, :dh] + first[:, dh:], first[:, dh:]),
                (second[:, :dh], second[:, :dh] + second[:, dh:]))

    def assemble(p1, q1, p2, q2, c11, c22):
        n = L - 2 * _LATE
        y1, y2 = p1 + q1, p2 + q2
        return (jnp.concatenate([y1[:n], (q1[n:] - q2[n:]) + c11, y1[n:]], axis=0),
                jnp.concatenate([y2, (p2[n:] - p1[n:]) + c22], axis=0))

    def step(i, r, mem):
        rows = _ds((4 * i + r) * seg, seg, seg)
        late = _ds((2 * i + r // 2) * _LATE, _LATE, _LATE)
        h = [[v.astype(_BF16) for v in f]
             for f in forms(jnp.concatenate([mem, _get(xn_v, rows)], axis=0))]
        groups = H // _HG
        qkv, sc, out = {}, {}, {}

        def project_rows(g):
            slabs = range(3 * _HG * g, 3 * _HG * (g + 1))
            y = {}
            for c, k in ((1, 0), (0, 1), (0, 0), (1, 1)):
                y[c, k] = _dot(h[c][k], jnp.concatenate(
                    [_unpack(wa_v[n, pl.ds(k * dq, dq), :]) for n in slabs[c::2]], axis=1))
            c11, c22 = _split(jnp.concatenate(
                [pre_v[n // 2, r % 2, late, :] for n in slabs[::2]], axis=1))
            qkv[g] = assemble(y[0, 0], y[0, 1], y[1, 0], y[1, 1], c11, c22)

        def part(g, n, t):
            k, c = divmod(3 * n + t, 2)
            return qkv[g][c][:, k * E:(k + 1) * E]

        def scores(g):
            sc[g] = [_dot_nt(part(g, n, 0), part(g, n, 1).astype(_BF16)) for n in range(_HG)]

        def attend(g):
            for n in range(_HG):
                z = jnp.where(mask, sc[g][n] * (scale * _LOG2E), -1e9 * _LOG2E)
                e = jnp.exp2(z - jnp.max(z, axis=-1, keepdims=True))
                total = jnp.sum(e, axis=-1, keepdims=True)
                inv = pl.reciprocal(total, approx=True)
                inv = inv * (2.0 - total * inv)
                out[g, n] = _dot(e * inv, part(g, n, 2).astype(_BF16))
                post_v[r, :, pl.ds((g * _HG + n) * E, E)] = out[g, n][L - 2 * _LATE:]
            if g % 2:
                f = forms(jnp.concatenate([out[k, n] for k in (g - 1, g) for n in range(_HG)], axis=1))
                for c in range(2):
                    for k in range(2):
                        att_v[c, k, :, pl.ds(g // 2 * dh, dh)] = _pack(f[c][k])

        def project_out(m):
            for c in range(2):
                for j in range(4):
                    for k in range(2):
                        d = _dot(_unpack(att_v[c, k, :, pl.ds(m * dh, dh)]),
                                 _unpack(wa_v[_wo_slab(H, m, 4 * c + j), pl.ds(k * dq, dq), :]))
                        o[c, k, j] = d + o[c, k, j] if m else d

        o = {}
        for t in range(groups + 4):
            if t < groups:
                project_rows(t)
            else:
                project_out(t - groups)
            if 0 <= t - 2 < groups:
                attend(t - 2)
            if 0 <= t - 1 < groups:
                scores(t - 1)
        o = jnp.concatenate(assemble(*[jnp.concatenate([o[c, k, j] for j in range(4)], axis=1)
                                       for c in range(2) for k in range(2)], 0.0, 0.0), axis=1)
        y = (x_v[rows, :].astype(_F32) + mixer_out(i, r)) + o[n_mem:]
        x_v[rows, :] = y.astype(_BF16)
        _put(acc_v.at[r % 2], late, 0, y[early:early + _LATE, :dh])
        _put(acc_v.at[r % 2], late, dh, y[early + _LATE:, dh:])
        return o[:n_mem]

    def steps(i, mem):
        for r in range(4):
            mem = step(i, r, mem)
        for r in range(2):
            rows = _ds((2 * i + r) * _LATE, _LATE, _LATE)
            for m in range(H * E // D):
                for c in range(0, dq, 128):
                    for n, p in enumerate(_MIXING):
                        for k, v in enumerate(_operands7(_LHS_TERMS, lambda a, b: post_v[
                                2 * r + a % 2, pl.ds(a // 2 * _LATE, _LATE),
                                pl.ds(m * D + b * dq + c, 128)], p)):
                            a2_v[7 * n + k, rows, pl.ds(m * dq + c, 128)] = v
        for r in range(4):
            for r0, n, c0, w in ((0, early, 0, D), (early, _LATE, dh, dh), (early + _LATE, _LATE, 0, dh)):
                at = (_ds((4 * i + r) * seg + r0, n, _LATE), pl.ds(c0, w))
                pltpu.make_async_copy(x_v.at[at], out_hbm.at[at], sem.at[0]).start()
        return mem

    mem0_copy.wait()
    lax.fori_loop(0, n_seg // 4, steps, mem0_v[...].astype(_F32))

    for cp in rest_of_wo:
        cp.wait()

    @pl.loop(0, 2)
    def _(i):
        partial = {}

        def done(m, k, r0, *blocks):
            for c, v in enumerate(blocks):
                j = 4 * c + 2 * i + k % 2
                v = v + (partial.pop((c, k, r0)) if m else acc_v[k // 2, j, pl.ds(r0, _SM), :])
                if m < 3:
                    partial[c, k, r0] = v
                    continue
                for t in range(0, _SM, _LATE):
                    fin_v[k // 2, pl.ds(r0 + t, _LATE), _ds(j * 128, 128, 128)] = (
                        v[t:t + _LATE].astype(_BF16))

        project(lambda m, p, r0: a2_v[p, pl.ds(r0, _SM), pl.ds(m * dq, dq)], done,
                lambda j, b_v: [fill_jobs(b_v, wo_v, jnp.minimum(16 * i + 4 * j + 4, H - 4))])
        for s in range(n_seg):
            for c in range(2):
                cols = _ds(c * dh + i * dq, dq, dq)
                pltpu.make_async_copy(
                    fin_v.at[s % 2, pl.ds(s // 2 * _LATE, _LATE), cols],
                    out_hbm.at[pl.ds(s * seg + early + c * _LATE, _LATE), cols], sem.at[0]).start()

    pltpu.make_async_copy(x_v, out_hbm, sem.at[0]).wait()


def _kernel(x_hbm, mem0_hbm, wq_hbm, wk_hbm, wv_hbm, wo_hbm, w1_hbm, w2_hbm, w3_hbm, w4_hbm,
            out_hbm, *shared, seg):
    S, D = x_hbm.shape
    HE = wo_hbm.shape[0]
    n_mem, n_late = mem0_hbm.shape[0], S // seg * _LATE
    pl.run_scoped(
        functools.partial(_mixer, x_hbm, wq_hbm, wk_hbm, wv_hbm, w1_hbm, w2_hbm, w3_hbm,
                          w4_hbm, *shared, seg),
        pltpu.VMEM((7, D // 4, D // 2), _U32),
        pltpu.VMEM((7, D // 4, D // 2), _U32),
        pltpu.VMEM((2, D // 2, _FC), _U32),
        pltpu.VMEM((2, _FC // 2, D), _U32),
        pltpu.VMEM((49, S // 8, D // 4), _U32),
        pltpu.VMEM((2, 3, _RD * HE // 256, 128), _U32),
        pltpu.VMEM((D // 128, S + 2 * _PAD, 128), _F32),
        pltpu.VMEM((2, 7, _TM // 4, D // 2), _U32),
        pltpu.VMEM((7, _TM // 4, D // 2), _U32),
        pltpu.VMEM((D // 128, _TM, 128), _F32),
        pltpu.VMEM((D // 128, _TM, 128), _F32),
        pltpu.VMEM((D // 128, _TM + _PAD, 128), _F32),
        pltpu.SMEM((1,), jnp.int32),
        pltpu.SemaphoreType.DMA((S // _TM,)),
        pltpu.SemaphoreType.DMA((4,)),
        pltpu.SemaphoreType.DMA((2, 2)),
        pltpu.SemaphoreType.DMA((2, 3)))
    pl.run_scoped(
        functools.partial(_memory, out_hbm, mem0_hbm, wo_hbm, *shared, seg),
        pltpu.VMEM((HE // 128, D // 2, 128), _U32),
        pltpu.VMEM((3 * HE // 256, 2, n_late // 2, 128), _U32),
        pltpu.VMEM((4, 2 * _LATE, HE), _F32),
        pltpu.VMEM((21, n_late // 2, HE // 4), _F32),
        pltpu.VMEM((2, D // 128, n_late // 2, 128), _F32),
        pltpu.VMEM((2, 2, (n_mem + seg - _LATE) // 2, HE // 2), _U32),
        pltpu.VMEM((2, n_late // 2, D), _BF16),
        pltpu.VMEM((n_mem, D), _BF16),
        pltpu.SemaphoreType.DMA((2,)),
        pltpu.SemaphoreType.DMA((8, 8)))


@functools.partial(jax.jit, static_argnames=("A_seg_len",))
def pallas_parallel_sum__memory_aug_recurrent_mem_tr__mixer_s_mlp__prompt_kernel(
    A_x: jax.Array,
    A_mem0: jax.Array,
    A_Wq: jax.Array,
    A_Wk: jax.Array,
    A_Wv: jax.Array,
    A_Wo: jax.Array,
    A_seg_len: int,
    B_x: jax.Array,
    B_w1: jax.Array,
    B_w2: jax.Array,
    B_w3: jax.Array,
    B_w4: jax.Array,
):
    del B_x
    B, S, D = A_x.shape
    _, H, E = A_Wq.shape
    M = A_mem0.shape[1]
    seg = int(A_seg_len)
    assert (B, S, D, H, E, M, seg, B_w3.shape[1]) == (1, 2048, 1024, 32, 128, 8, 32, 3584)

    hbm = pl.BlockSpec(memory_space=pltpu.HBM)
    out = pl.pallas_call(
        functools.partial(_kernel, seg=seg),
        out_shape=jax.ShapeDtypeStruct((S, D), A_x.dtype),
        in_specs=[hbm] * 10,
        out_specs=hbm,
        scratch_shapes=[
            pltpu.VMEM((S, D), _BF16),
            pltpu.VMEM((4 * H, D // 2, E), _U32),
            pltpu.VMEM((21, S // seg * _LATE // 4, D // 4), _U32),
            pltpu.VMEM((D // 128, S + _PAD, 128), _F32),
            pltpu.VMEM((7, 4, S // 4, D // 4), _F32),
            pltpu.VMEM((49, D // 8, 128), _U32),
            pltpu.VMEM((49, D // 8, 128), _U32),
        ],
        compiler_params=pltpu.CompilerParams(vmem_limit_bytes=126 * 1024 * 1024),
    )(A_x.reshape(S, D), A_mem0.reshape(M, D),
      A_Wq.reshape(D * H, E), A_Wk.reshape(D * H, E), A_Wv.reshape(D * H, E),
      A_Wo.reshape(H * E, D), B_w1, B_w2, B_w3, B_w4)
    return out.reshape(B, S, D)
```

```python
import functools

import jax
import jax.numpy as jnp
import numpy as np
from jax import lax
import jax.experimental.pallas as pl
import jax.experimental.pallas.tpu as pltpu

_F32 = jnp.float32
_BF16 = jnp.bfloat16
_U32 = jnp.uint32

_EPS = 1e-5
_LOG2E = float(np.log2(np.e))
_TM = 256
_SM = 64
_FC = 512
_RD = 160
_HG = 4
_LATE = 8
_PAD = 8


def _dot(a, b):
    return lax.dot_general(a, b, (((1,), (0,)), ((), ())), preferred_element_type=_F32)


def _dot_nt(a, b):
    return lax.dot_general(a, b, (((1,), (1,)), ((), ())), preferred_element_type=_F32)


def _ds(start, size, align):
    return pl.ds(start if isinstance(start, int) else pl.multiple_of(start, align), size)


def _pack(x):
    return pltpu.bitcast(x.astype(_BF16), _U32)


def _unpack(w):
    return pltpu.bitcast(w, _BF16)


def _pair(even, odd):
    return pltpu.pack_elementwise([even, odd], packed_dtype=_BF16)


def _split(w):
    return (pltpu.bitcast(lax.shift_left(w, np.uint32(16)), _F32),
            pltpu.bitcast(lax.bitwise_and(w, np.uint32(0xFFFF0000)), _F32))


def _get(ref, rows):
    return jnp.concatenate([ref[k, rows, :] for k in range(ref.shape[0])], axis=1)


def _put(ref, rows, c0, x):
    for c in range(0, x.shape[1], 128):
        ref[(c0 + c) // 128, rows, :] = lax.slice_in_dim(x, c, c + 128, axis=1)


def _wo_slab(heads, m, j):
    return 3 * heads + 16 * (j % 4 // 2) + 4 * m + 2 * (j % 2) + j // 4


def _gelu(hx):
    c0 = 2.0 * float(np.sqrt(2.0 / np.pi))
    c1 = 4.0 * 0.044715 * c0
    inner = lax.mul(hx, lax.add(np.float32(c0), lax.mul(np.float32(c1), lax.mul(hx, hx))))
    return lax.add(hx, lax.mul(hx, lax.tanh(inner)))


def _layernorm_twice(load):
    m = jnp.mean(load(0), axis=-1, keepdims=True)
    c = load(1) - m
    mu = jnp.mean(c, axis=-1, keepdims=True)
    v = jnp.mean(c * c, axis=-1, keepdims=True)
    r = lax.rsqrt(v + _EPS)
    r2 = (0.5 * r) * lax.rsqrt((r * r) * jnp.maximum(v - mu * mu, 0.0) + _EPS)
    c = load(2) - m
    return c * r, (c - mu) * r2


def _zero_bits(ref):
    return jnp.where(jnp.abs(ref[:16, :128].astype(_F32)[:8]) < 0.0, 1, 0).astype(_U32)


def _after(x, z):
    w = pltpu.bitcast(x, _U32)
    for axis in range(2):
        if w.shape[axis] > z.shape[axis]:
            z = lax.concatenate([z] * (w.shape[axis] // z.shape[axis]), axis)
    return pltpu.bitcast(lax.bitwise_or(w, z), x.dtype)


def _mark(v, zero, r=0):
    return lax.bitwise_and(pltpu.bitcast(lax.slice(v, (r, 0), (r + 8, 128)), _U32), zero)


def _any(words):
    while len(words) > 1:
        words = [functools.reduce(lax.bitwise_or, words[k:k + 2]) for k in range(0, len(words), 2)]
    return words[0]


def _spread(jobs, marks, lo=0.0, hi=1.0, prev=None):
    marks = marks[int(lo * len(marks)):int(hi * len(marks))]
    for k, job in enumerate(jobs):
        z = marks[k * len(marks) // len(jobs)]
        prev = job(z if prev is None else lax.bitwise_or(z, prev))
    return prev


_LHS_TERMS = ((0, 1, 3), (2, 1, 3), (0, 0, 0), (3, 0, 3), (0, 1, 1), (2, -1, 0), (1, -1, 3))
_RHS_TERMS = ((0, 1, 3), (0, 0, 0), (1, -1, 3), (2, -1, 0), (3, 0, 3), (0, 1, 1), (2, 1, 3))
_ORDER = (0, 1, 3, 5, 6, 2, 4)


_MIXING = (0, 5, 6)


class _Quad:
    def __init__(self, blocks):
        self.blocks = list(blocks)


def _add(a, b):
    return _Quad(map(lax.add, a.blocks, b.blocks)) if isinstance(a, _Quad) else lax.add(a, b)


def _sub(a, b):
    return _Quad(map(lax.sub, a.blocks, b.blocks)) if isinstance(a, _Quad) else lax.sub(a, b)


def _term(terms, get, p):
    a, sign, b = terms[p]
    return get(a) if sign == 0 else (_add if sign > 0 else _sub)(get(a), get(b))


def _operands(terms, quadrants):
    return [_term(terms, quadrants.__getitem__, p) for p in range(7)]


def _block(n, k):
    return 2 * (n // 2) + k // 2, 2 * (n % 2) + k % 2


def _operands7(terms, get, p):
    outer = _term(terms, lambda n: _Quad(get(*_block(n, k)) for k in range(4)), p)
    return _operands(terms, outer.blocks)


def _combine(m):
    m1, m2, m3, m4, m5, m6, m7 = m
    return (m1 + m4) + (m7 - m5), m3 + m5, m2 + m4, (m1 - m2) + (m3 + m6)


def _strassen(prod, done):
    m1, m2 = prod(0), prod(1)
    c22 = _sub(m1, m2)
    m4 = prod(3)
    done(2, _add(m2, m4))
    c11 = _add(m1, m4)
    c22 = _add(prod(5), c22)
    c11 = _add(prod(6), c11)
    m3 = prod(2)
    done(3, _add(c22, m3))
    m5 = prod(4)
    done(0, _sub(c11, m5))
    done(1, _add(m3, m5))
    return m1, m2, m4, c22, c11, m3, m5


def _strassen49(prod, done):
    seen = []

    def outer(p):
        out = [None] * 4
        m = _strassen(lambda k: prod(7 * p + k), out.__setitem__)
        seen.extend(m[k] for k in (0, 1, 3, 4))
        return _Quad(out)

    def finish(n, quad):
        for k, v in enumerate(quad.blocks):
            done(*_block(n, k), v)

    _strassen(outer, finish)
    return seen


def _halves(z):
    shift, high = lax.bitwise_or(z, np.uint32(16)), lax.bitwise_or(z, np.uint32(0xFFFF0000))
    return (lambda w: pltpu.bitcast(lax.shift_left(w, shift), _F32),
            lambda w: pltpu.bitcast(lax.bitwise_and(w, high), _F32))


def _fill_jobs(b_v, word, slots=tuple(zip(_ORDER, _ORDER))):
    def job(n, p, k, z):
        load = functools.cache(lambda r, c: word(r, c, k))
        even, odd = (_operands7(_RHS_TERMS, lambda r, c: half(load(r, c)), p) for half in _halves(z))
        for j in range(7):
            b_v[7 * n + j, pl.ds(k, 8), :] = _pair(even[j], odd[j])

    return [functools.partial(job, n, p, k) for n, p in slots for k in range(0, b_v.shape[1], 8)]


def _mixer(x_hbm, wq_hbm, wk_hbm, wv_hbm, w1_hbm, w2_hbm, w3_hbm, w4_hbm,
           x_v, wa_v, a_v, xn_v, ffn_v, b0_v, b1_v, seg,
           w1_v, w2_v, w3_v, w4_v, f_v, stage_v, h_v, y_v, g_v, t0_v, t1_v, t2_v, nil_s,
           sem_x, sem_w, sem_f, sem_s):
    S, D = x_v.shape
    H, E = wa_v.shape[0] // 4, wa_v.shape[2]
    dh, dq, th, tq = D // 2, D // 4, _TM // 2, _TM // 4
    nblk = S // _TM
    nfc = w3_hbm.shape[1] // _FC
    corners = [(r, c) for r in (0, th) for c in (0, dh)]
    tiles = [(r, c) for r in range(0, th, _SM) for c in range(0, dh, 128)]

    def x_copy(i):
        rows = pl.ds(i * _TM, _TM)
        return pltpu.make_async_copy(x_hbm.at[rows], x_v.at[rows], sem_x.at[i])

    def w3_copy(c):
        src = w3_hbm.bitcast(_U32).at[:, _ds(c * _FC, _FC, _FC)]
        return pltpu.make_async_copy(src, w3_v.at[c % 2], sem_f.at[c % 2, 0])

    def w4_copy(c):
        src = w4_hbm.bitcast(_U32).at[_ds(c * _FC // 2, _FC // 2, _FC // 2)]
        return pltpu.make_async_copy(src, w4_v.at[c % 2], sem_f.at[c % 2, 1])

    def retile_row(c):
        return min(c * _RD, D - _RD) if isinstance(c, int) else jnp.minimum(c * _RD, D - _RD)

    def stage_copy(t, c):
        src = (wq_hbm, wk_hbm, wv_hbm)[t].bitcast(_U32)
        rows = _ds(retile_row(c) * H // 2, _RD * H // 2, 8 * H)
        return pltpu.make_async_copy(src.at[rows], stage_v.at[c % 2, t], sem_s.at[c % 2, t])

    w1_copies = [pltpu.make_async_copy(w1_hbm.bitcast(_U32).at[:, pl.ds(k * dh, dh)], w3_v.at[k],
                                       sem_w.at[k]) for k in range(2)]
    w2_copies = [pltpu.make_async_copy(w2_hbm.bitcast(_U32).at[pl.ds(k * dq, dq)], w4_v.at[k],
                                       sem_w.at[2 + k]) for k in range(2)]

    nil_s[0] = 0
    x_copy(0).start()
    x_copy(1).start()
    w1_copies[0].start()
    for r in (0, _PAD + S):
        _put(h_v, pl.ds(r, _PAD), 0, jnp.zeros((_PAD, D), _F32))
    x_copy(0).wait()
    zero = _zero_bits(x_v)

    def mark(v, r=0):
        return _mark(v, zero, r)

    def norm(rows, z):
        nil = nil_s[0]

        def load(k):
            w = [_pack(x_v[_ds(r + 16 * k * nil, 16, 16), :]) for r in rows]
            return jnp.concatenate([h for v in w for h in _split(v if k else _after(v, z))], axis=0)

        xn, y = _layernorm_twice(load)
        for k, r in enumerate(rows):
            for odd in range(2):
                _put(xn_v, pl.ds(r + odd, 8, stride=2), 0, xn[16 * k + 8 * odd:16 * k + 8 * odd + 8])
        return y

    def norm_jobs(i):
        def job(r, z):
            y = norm((i * _TM + r, i * _TM + th + r), z)
            even, odd = (_operands(_LHS_TERMS, [y[k + a:k + a + 8, c:c + dh]
                                                for a in (0, 16) for c in (0, dh)]) for k in (0, 8))
            for p in range(7):
                y_v[i % 2, p, pl.ds(r // 2, 8), :] = _pair(even[p], odd[p])
            return functools.reduce(jnp.bitwise_or, [mark(y, k) for k in range(0, 32, 8)])

        return [functools.partial(job, r) for r in range(0, th, 16)]

    def shift_jobs(i, combine):
        def job(r0, c0, z):
            def load(r, c, odd):
                shift = (-1, 1, -2, 2)[(c + c0) // dq]
                rows = pl.ds(i * _TM + _PAD + r + r0 + shift + odd, _SM // 2, stride=2)
                return _after(h_v[(c + c0) // 128, rows, :], z)

            even, odd = (combine([load(r, c, k) for r, c in corners]) for k in range(2))
            for p in range(len(even)):
                g_v[p, pl.ds(r0 // 2, _SM // 2), pl.ds(c0, 128)] = _pair(even[p], odd[p])

        return [functools.partial(job, r0, c0) for r0, c0 in tiles]

    def weight_jobs(w_v, word):
        def job(k, c, z):
            quads = [word(r, q, k, c) for r in range(2) for q in range(2)]
            even, odd = (_operands(_RHS_TERMS, [half(w) for w in quads]) for half in _halves(z))
            for p in (0, 2, 3, 5, 6):
                w_v[p, pl.ds(k, 8), pl.ds(c, 128)] = _pair(even[p], odd[p])
            w_v[1, pl.ds(k, 8), pl.ds(c, 128)] = quads[0]
            w_v[4, pl.ds(k, 8), pl.ds(c, 128)] = quads[3]

        return [functools.partial(job, k, c) for c in range(0, dh, 128) for k in range(0, dq, 8)]

    def plain(lhs, rhs, put, c0, c1):
        marks = []
        for c in range(c0, c1, 128):
            for r0 in range(0, th, _SM):
                for q in (2, 0):
                    y = jnp.concatenate([_unpack(lhs[q + n, pl.ds(r0 // 2, _SM // 2), :])
                                         for n in range(2)], axis=1)
                    v = _dot(y, _unpack(rhs(c)))
                    put(q // 2 * th + r0, c, v)
                    marks.append(mark(v))
        return marks

    def fast(lhs, w_v, put):
        marks = []
        for r0, c0 in tiles:
            marks += [mark(v) for v in _strassen(
                lambda p: _dot(_unpack(lhs[p, pl.ds(r0 // 2, _SM // 2), :]),
                               _unpack(w_v[p, :, pl.ds(c0, 128)])),
                lambda q, v: put(corners[q][0] + r0, corners[q][1] + c0, v))]
        return marks

    def put_h(i):
        return lambda r, c, v: _put(h_v, pl.ds(_PAD + i * _TM + r, _SM), c, _gelu(v))

    def put_x1(i):
        held = {}

        def put(r, c, v):
            v = v + xn_v[c // 128, pl.ds(i * _TM + r, _SM), :]
            (t0_v, t1_v)[i % 2][c // 128, pl.ds(r, _SM), :] = v
            quadrant, key = 2 * (r // th) + c // dh, (r % th, c % dh)
            held[key, quadrant] = v
            seeds = {0: [(6, v)], 1: [(2, v)], 2: [(1, v)], 3: []}[quadrant]
            if quadrant and all((key, n) in held for n in (1, 2, 3)):
                seeds.append((5, held[key, 3] + (held[key, 2] - held[key, 1])))
            for p, w in seeds:
                ffn_v[p, 2 * (r % th // tq) + c % dh // dq, pl.ds(i * tq + r % tq, _SM),
                      pl.ds(c % dq, 128)] = w

        return put

    def ffn_norm_jobs(i):
        t_v, nil = (t0_v, t1_v)[i % 2], nil_s[0]

        def mean(parts):
            return jnp.sum(functools.reduce(jnp.add, parts), axis=-1, keepdims=True) * (1.0 / D)

        def normalise(r, z):
            def load(k):
                return [t_v[c + k * nil, pl.ds(r, 32), :] for c in range(D // 128)]

            x1 = load(1)
            m = mean([_after(x1[0], z)] + x1[1:])
            inv = 0.5 * lax.rsqrt(mean([(e - m) * (e - m) for e in load(2)]) + _EPS)
            for c, e in enumerate(load(3)):
                e = (e - m) * inv
                t2_v[c, pl.ds(r, 32), :] = e
            return _any([mark(e, k) for k in range(0, 32, 8)])

        def sums(r, c, p, z):
            r0 = r // 32 * 32 + r % 32 // 16
            lo, hi = (_operands7(_LHS_TERMS, lambda a, b: _after(
                t2_v[(b * dq + c) // 128, pl.ds(a * tq + r0 + k, 8, stride=4), :], z), p)
                for k in (0, 2))
            for k in range(7):
                lo[k] = _pair(lo[k], hi[k])
                f_v[7 * p + k, pl.ds((i * tq + r) // 2, 8), pl.ds(c, 128)] = lo[k]
            return lax.bitwise_and(_any(lo), zero)

        return ([functools.partial(normalise, a * tq + r) for r in range(0, tq, 32) for a in range(4)],
                [functools.partial(sums, r, c, p)
                 for r in range(0, tq, 16) for c in range(0, dq, 128) for p in range(7)])

    def w3_jobs(c):
        return _fill_jobs(b0_v, lambda r, k, j: w3_v[
            c % 2, pl.ds(r * dq // 2 + j, 8), pl.ds(k * 128, 128)])

    def w4_jobs(c):
        return _fill_jobs(b1_v, lambda r, k, j: w4_v[
            c % 2, pl.ds(r * 64 + j % 64, 8), pl.ds(k * dq + j // 64 * 128, 128)])

    def fast_lhs(quadrants):
        return _operands(_LHS_TERMS, quadrants)

    y0 = norm(range(0, _TM, 16), zero)
    for r in range(0, _TM, 16):
        for k in range(2):
            y_v[0, 2 * (r // th) + k, pl.ds(r % th // 2, 8), :] = _pair(
                y0[r:r + 8, k * dh:(k + 1) * dh], y0[r + 8:r + 16, k * dh:(k + 1) * dh])

    x_copy(1).wait()
    w1_copies[1].start()
    w1_copies[0].wait()
    x_copy(2).start()
    marks = plain(y_v.at[0], lambda c: w3_v[0, :, pl.ds(c, 128)], put_h(0), 0, dh)
    jobs = norm_jobs(1)
    _spread(jobs[:5], marks, 0, 0.75)
    w1_copies[1].wait()
    for cp in w2_copies:
        cp.start()
    x_copy(3).start()
    marks = plain(y_v.at[0], lambda c: w3_v[1, :, pl.ds(c - dh, 128)], put_h(0), dh, D)
    _spread(weight_jobs(w1_v, lambda r, q, k, c: w3_v[q, pl.ds(r * dq + k, 8), pl.ds(c, 128)]), marks)
    _spread(jobs[5:], marks, 0, 0.75)

    x_copy(2).wait()
    for k in range(4, nblk):
        x_copy(k).start()
    w3_copy(0).start()
    marks = fast(y_v.at[1], w1_v, put_h(1))
    _spread(shift_jobs(0, list), marks, 0.1, 0.9)
    _spread(norm_jobs(2), marks, 0, 0.8)
    for cp in w2_copies:
        cp.wait()
    x_copy(3).wait()
    marks = plain(g_v, lambda c: jnp.concatenate(
        [w4_v[n, :, pl.ds(c, 128)] for n in range(2)], axis=0), put_x1(0), 0, D)
    _spread(weight_jobs(w2_v, lambda r, q, k, c: w4_v[r, pl.ds(k, 8), pl.ds(q * dh + c, 128)]), marks)

    for k in range(4, nblk):
        x_copy(k).wait()
    w3_copy(0).wait()
    w3_copy(1).start()
    w4_copy(0).start()
    for t in range(3):
        stage_copy(t, 0).start()
    prev = None
    for i in range(2, nblk + 1):
        marks = []
        if i < nblk:
            marks += fast(y_v.at[i % 2], w1_v, put_h(i))
            _spread(shift_jobs(i - 1, fast_lhs), marks, 0.1, 0.9)
        else:
            _spread(shift_jobs(i - 1, fast_lhs), [zero])
        marks += fast(g_v, w2_v, put_x1(i - 1))
        if i + 1 == nblk:
            _spread(w3_jobs(0), marks, 0.02, 0.8)
        normalise, sums = ffn_norm_jobs(i - 2)
        if i + 1 < nblk:
            jobs = [job for pair in zip(normalise, norm_jobs(i + 1)) for job in pair]
            _spread(jobs, marks, 0.02, 0.8, prev)
        else:
            _spread(normalise, marks, 0, 0.55, prev)
        prev = _spread(sums, marks, 0.6, 0.99)
    for jobs in ffn_norm_jobs(nblk - 1):
        for job in jobs:
            job(zero)

    def late_jobs(i):
        def job(r, c, n, z):
            def rows(a, k):
                return _ds(i * _TM + (4 * r + 2 * k + a % 2 + 1) * seg + (a // 2 - 2) * _LATE,
                           _LATE, _LATE)

            lo, hi = (_operands7(_LHS_TERMS, lambda a, b: _after(
                xn_v[(b * dq + c) // 128, rows(a, k), :], z), _MIXING[n]) for k in range(2))
            for k in range(7):
                a_v[7 * n + k, _ds((2 * i + r) * _LATE, _LATE, _LATE), pl.ds(c, 128)] = _pack(
                    jnp.concatenate([lo[k], hi[k]], axis=0))

        return [functools.partial(job, r, c, n)
                for r in range(2) for c in range(0, dq, 128) for n in range(3)]

    def hidden_rows(k, r, n):
        return pl.ds(k * S // 8 + r // 2, n // 2)

    def ffn(c, _):
        @pl.when(c + 1 < nfc)
        def _():
            for t in range(3):
                stage_copy(t, c + 1).start()
            w4_copy(c + 1).start()
            w3_copy(c + 1).wait()

        @pl.when(c + 2 < nfc)
        def _():
            w3_copy(c + 2).start()

        w4_copy(c).wait()
        for t in range(3):
            stage_copy(t, c).wait()

        def retile(t, r, jh, odd, z):
            v = stage_v[c % 2, t, pl.ds(r * H, 8 * H), :].reshape(8, H, E)
            a, b = v[:, 8 * jh:8 * jh + 8], v[:, H // 2 + 8 * jh:H // 2 + 8 * jh + 8]
            low = (z | _U32(0xFFFF))[None]
            w = ((a >> 16) | (b & ~low)) if odd else ((a & low) | (b << 16))
            w = jnp.swapaxes(w, 0, 1)
            rows = _ds(retile_row(c) // 2 + r, 8, 8)
            for j in range(8):
                wa_v[6 * (8 * jh + j) + 3 * odd + t, rows, :] = w[j]

        def activate(r0, hid, marks):
            def act(a, b, z):
                hid[a, b] = _gelu(_after(hid[a, b], z))

            _spread([functools.partial(act, a, b) for a in range(2) for b in range(4)],
                    marks, 0.03, 0.9)
            for p in _ORDER:
                for r in range(0, tq, 16):
                    r1 = r // 32 * 32 + r % 32 // 2
                    even, odd = (_operands7(_LHS_TERMS, lambda a, b: lax.slice_in_dim(
                        hid[a, b], k, k + 8), p)
                                 for k in (r1, r1 + 16))
                    for k in range(7):
                        h_v[p, hidden_rows(k, r0 + r, 16), :] = pltpu.bitcast(
                            _pair(even[k], odd[k]), _F32)

        marks, pending, fills = [], None, w4_jobs(c)
        for r0 in range(0, S // 4, tq):
            hid = {}
            seen = [mark(v) for v in _strassen49(
                lambda p: _dot(_unpack(f_v[p, pl.ds(r0 // 2, tq // 2), :]), _unpack(b0_v[p])),
                lambda a, b, v: hid.__setitem__((a, b), v if a < 2 else _gelu(v)))]
            if pending:
                activate(*pending, seen)
            n = len(fills) // 7
            _spread(fills[r0 // tq * n:][:n], seen)
            pending = (r0, hid)
            marks += seen
        retiles = [functools.partial(retile, t, r, jh, odd) for t in range(3)
                   for r in range(0, _RD // 2, 8) for jh in range(H // 16) for odd in range(2)]
        _spread(retiles[:18], marks, 0.004, 0.98)

        marks = []
        for r0 in range(0, S // 4, tq):
            for j in range(2):
                for p in range(7):
                    def done(q, v):
                        idx = (p, q, pl.ds(r0, tq), pl.ds(j * 128, 128))
                        old = ffn_v[idx]
                        ffn_v[idx] = lax.add(v, jnp.where(c > 0, old, 0.0) if p in (0, 3, 4) else old)

                    marks += [mark(v) for v in _strassen(
                        lambda k: _dot(_unpack(h_v[p, hidden_rows(k, r0, tq), :]),
                                       _unpack(b1_v[7 * p + k, pl.ds(j * 64, 64), :])), done)]
            if pending:
                activate(*pending, marks)
                pending = None
        _spread(w3_jobs(jnp.minimum(c + 1, nfc - 1)), marks, 0.2, 0.98)
        _spread(retiles[18:], marks, 0.25, 0.97)
        _spread(late_jobs(c) + late_jobs(c + 1), marks, 0.3, 0.95)
        return 0

    lax.fori_loop(0, nfc, ffn, 0)


def _memory(out_hbm, mem0_hbm, wo_hbm, x_v, wa_v, a_v, xn_v, ffn_v, b0_v, b1_v, seg,
            wo_v, pre_v, post_v, a2_v, acc_v, att_v, fin_v, mem0_v, sem, sem_o):
    S, D = x_v.shape
    H, E = wa_v.shape[0] // 4, wa_v.shape[2]
    dh, dq = D // 2, D // 4
    n_mem, n_seg, early = mem0_hbm.shape[0], S // seg, seg - 2 * _LATE
    L = n_mem + seg
    mem0_copy = pltpu.make_async_copy(mem0_hbm, mem0_v, sem.at[1])
    mem0_copy.start()

    def wo_copies(q, raw=0):
        copies = []
        for k in range(8):
            m, j = 2 * (q % 2) + k // 4, 4 * (k % 2) + 2 * (q // 2) + k % 4 // 2
            src = wo_hbm.bitcast(_U32).at[_ds(m * dh, dh, dh), _ds(j * 128, 128, 128)]
            dst = wo_v.at[8 * q + k] if raw else wa_v.at[3 * H + 8 * q + k]
            copies.append(pltpu.make_async_copy(src, dst, sem_o.at[4 * raw + q, k]))
        return copies

    zero = _zero_bits(x_v)

    def fill_jobs(b_v, w_v, n):
        return _fill_jobs(b_v, lambda r, c, k: w_v[
            n + 2 * (c % 2) + c // 2, pl.ds(r * dq // 2 + k, 8), :], tuple(enumerate(_MIXING)))

    def loop_form_jobs(slabs):
        def job(n, k, z):
            quads = [wa_v[n + c, pl.ds(r * dq + k, 16), :] for r in range(2) for c in range(2)]
            even, odd = ([half(w) for w in quads] for half in _halves(jnp.tile(z, (2, 1))))
            wa_v[n + 1, pl.ds(k, 16), :] = _pair(even[1] - even[3], odd[1] - odd[3])
            wa_v[n, pl.ds(dq + k, 16), :] = _pair(even[2] - even[0], odd[2] - odd[0])

        return [functools.partial(job, n, k) for n in slabs for k in range(0, dq, 16)]

    def project(lhs, done, jobs):
        for j in range(4):
            b_v, marks = (b0_v, b1_v)[j % 2], []
            for r0 in range(0, n_seg * _LATE // 2, _SM):
                m = []
                for n in range(3):
                    m.append([None] * 4)
                    seen = _strassen(lambda k: _dot(lhs(j, 7 * n + k, r0), _unpack(b_v[7 * n + k])),
                                     m[n].__setitem__)
                    marks += [_mark(seen[k], zero) for k in (0, 1, 3, 4)]
                for k in range(4):
                    done(j, k, r0, lax.add(m[0][k], m[2][k]), lax.add(m[0][k], m[1][k]))
            for some in jobs(j, (b1_v, b0_v)[j % 2]):
                _spread(some, marks[:-3])

    def pre(i):
        def done(j, k, r0, c11, c22):
            pre_v[8 * i + 2 * j + k % 2, k // 2, pl.ds(r0, _SM), :] = _pair(c11, c22)

        def jobs(j, b_v):
            n = 16 * i + 4 * j
            if not isinstance(i, int):
                return [fill_jobs(b_v, wa_v, n + 4),
                        loop_form_jobs((n, n + 2, 3 * H + 8 * (i - 1) + 2 * j))]
            return [fill_jobs(b_v, wa_v, n + 4) if n + 4 < 3 * H else fill_jobs(b_v, wo_v, 0),
                    loop_form_jobs((n, n + 2))]

        project(lambda j, p, r0: _unpack(a_v[p, pl.ds(r0 // 2, _SM // 2), :]), done, jobs)

    for cp in wo_copies(0):
        cp.start()
    _spread(fill_jobs(b0_v, wa_v, 0), [zero])
    pre(0)

    for cp in wo_copies(0, raw=1):
        cp.start()

    @pl.loop(1, 5)
    def _(i):
        @pl.when(i < 4)
        def _():
            for cp in wo_copies(i):
                cp.start()

        for cp in wo_copies(i - 1):
            cp.wait()
        pre(i)

    for cp in wo_copies(0, raw=1):
        cp.wait()
    pre(5)
    rest_of_wo = [cp for q in range(1, 4) for cp in wo_copies(q, raw=1)]
    for cp in rest_of_wo:
        cp.start()

    row = lax.broadcasted_iota(jnp.int32, (L, L), 0)
    col = lax.broadcasted_iota(jnp.int32, (L, L), 1)
    mask = (row < n_mem) | (row >= col)
    scale = float(E) ** -0.5

    def mixer_out(i, r):
        rows = _ds((i // 2) * (_TM // 4) + (r % 2) * seg, seg, seg)
        cols = [None] * 4
        for b in range(2):
            c = _combine([ffn_v[p, 2 * (r // 2) + b, rows, :] for p in range(7)])
            for k in range(2):
                cols[2 * k + b] = jnp.where(i % 2 == 0, c[k], c[2 + k])
        return jnp.concatenate(cols, axis=1)

    def forms(v):
        n = L - 2 * _LATE
        first = jnp.concatenate([v[:n], v[n + _LATE:]], axis=0)
        second = v[:n + _LATE]
        return ((first[:, :dh] + first[:, dh:], first[:, dh:]),
                (second[:, :dh], second[:, :dh] + second[:, dh:]))

    def assemble(p1, q1, p2, q2, c11, c22):
        n = L - 2 * _LATE
        y1, y2 = p1 + q1, p2 + q2
        return (jnp.concatenate([y1[:n], (q1[n:] - q2[n:]) + c11, y1[n:]], axis=0),
                jnp.concatenate([y2, (p2[n:] - p1[n:]) + c22], axis=0))

    def step(i, r, mem):
        rows = _ds((4 * i + r) * seg, seg, seg)
        late = _ds((2 * i + r // 2) * _LATE, _LATE, _LATE)
        h = [[v.astype(_BF16) for v in f]
             for f in forms(jnp.concatenate([mem, _get(xn_v, rows)], axis=0))]
        groups = H // _HG
        qkv, sc, out = {}, {}, {}

        def project_rows(g):
            slabs = range(3 * _HG * g, 3 * _HG * (g + 1))
            y = {}
            for c, k in ((1, 0), (0, 1), (0, 0), (1, 1)):
                y[c, k] = _dot(h[c][k], jnp.concatenate(
                    [_unpack(wa_v[n, pl.ds(k * dq, dq), :]) for n in slabs[c::2]], axis=1))
            c11, c22 = _split(jnp.concatenate(
                [pre_v[n // 2, r % 2, late, :] for n in slabs[::2]], axis=1))
            qkv[g] = assemble(y[0, 0], y[0, 1], y[1, 0], y[1, 1], c11, c22)

        def part(g, n, t):
            k, c = divmod(3 * n + t, 2)
            return qkv[g][c][:, k * E:(k + 1) * E]

        def scores(g):
            sc[g] = [_dot_nt(part(g, n, 0), part(g, n, 1).astype(_BF16)) for n in range(_HG)]

        def attend(g):
            for n in range(_HG):
                z = jnp.where(mask, sc[g][n] * (scale * _LOG2E), -1e9 * _LOG2E)
                e = jnp.exp2(z - jnp.max(z, axis=-1, keepdims=True))
                total = jnp.sum(e, axis=-1, keepdims=True)
                inv = pl.reciprocal(total, approx=True)
                inv = inv * (2.0 - total * inv)
                out[g, n] = _dot(e * inv, part(g, n, 2).astype(_BF16))
                post_v[r, :, pl.ds((g * _HG + n) * E, E)] = out[g, n][L - 2 * _LATE:]
            if g % 2:
                f = forms(jnp.concatenate([out[k, n] for k in (g - 1, g) for n in range(_HG)], axis=1))
                for c in range(2):
                    for k in range(2):
                        att_v[c, k, :, pl.ds(g // 2 * dh, dh)] = _pack(f[c][k])

        def project_out(m):
            for c in range(2):
                for j in range(4):
                    for k in range(2):
                        d = _dot(_unpack(att_v[c, k, :, pl.ds(m * dh, dh)]),
                                 _unpack(wa_v[_wo_slab(H, m, 4 * c + j), pl.ds(k * dq, dq), :]))
                        o[c, k, j] = d + o[c, k, j] if m else d

        o = {}
        for t in range(groups + 4):
            if t < groups:
                project_rows(t)
            else:
                project_out(t - groups)
            if 0 <= t - 2 < groups:
                attend(t - 2)
            if 0 <= t - 1 < groups:
                scores(t - 1)
        o = jnp.concatenate(assemble(*[jnp.concatenate([o[c, k, j] for j in range(4)], axis=1)
                                       for c in range(2) for k in range(2)], 0.0, 0.0), axis=1)
        y = (x_v[rows, :].astype(_F32) + mixer_out(i, r)) + o[n_mem:]
        x_v[rows, :] = y.astype(_BF16)
        _put(acc_v.at[r % 2], late, 0, y[early:early + _LATE, :dh])
        _put(acc_v.at[r % 2], late, dh, y[early + _LATE:, dh:])
        return o[:n_mem]

    def steps(i, mem):
        for r in range(4):
            mem = step(i, r, mem)
        for r in range(2):
            rows = _ds((2 * i + r) * _LATE, _LATE, _LATE)
            for m in range(H * E // D):
                for c in range(0, dq, 128):
                    for n, p in enumerate(_MIXING):
                        for k, v in enumerate(_operands7(_LHS_TERMS, lambda a, b: post_v[
                                2 * r + a % 2, pl.ds(a // 2 * _LATE, _LATE),
                                pl.ds(m * D + b * dq + c, 128)], p)):
                            a2_v[7 * n + k, rows, pl.ds(m * dq + c, 128)] = v
        for r in range(4):
            for r0, n, c0, w in ((0, early, 0, D), (early, _LATE, dh, dh), (early + _LATE, _LATE, 0, dh)):
                at = (_ds((4 * i + r) * seg + r0, n, _LATE), pl.ds(c0, w))
                pltpu.make_async_copy(x_v.at[at], out_hbm.at[at], sem.at[0]).start()
        return mem

    mem0_copy.wait()
    lax.fori_loop(0, n_seg // 4, steps, mem0_v[...].astype(_F32))

    for cp in rest_of_wo:
        cp.wait()

    @pl.loop(0, 2)
    def _(i):
        partial = {}

        def done(m, k, r0, *blocks):
            for c, v in enumerate(blocks):
                j = 4 * c + 2 * i + k % 2
                v = v + (partial.pop((c, k, r0)) if m else acc_v[k // 2, j, pl.ds(r0, _SM), :])
                if m < 3:
                    partial[c, k, r0] = v
                    continue
                for t in range(0, _SM, _LATE):
                    fin_v[k // 2, pl.ds(r0 + t, _LATE), _ds(j * 128, 128, 128)] = (
                        v[t:t + _LATE].astype(_BF16))

        project(lambda m, p, r0: a2_v[p, pl.ds(r0, _SM), pl.ds(m * dq, dq)], done,
                lambda j, b_v: [fill_jobs(b_v, wo_v, jnp.minimum(16 * i + 4 * j + 4, H - 4))])
        for s in range(n_seg):
            for c in range(2):
                cols = _ds(c * dh + i * dq, dq, dq)
                pltpu.make_async_copy(
                    fin_v.at[s % 2, pl.ds(s // 2 * _LATE, _LATE), cols],
                    out_hbm.at[pl.ds(s * seg + early + c * _LATE, _LATE), cols], sem.at[0]).start()

    pltpu.make_async_copy(x_v, out_hbm, sem.at[0]).wait()


def _kernel(x_hbm, mem0_hbm, wq_hbm, wk_hbm, wv_hbm, wo_hbm, w1_hbm, w2_hbm, w3_hbm, w4_hbm,
            out_hbm, *shared, seg):
    S, D = x_hbm.shape
    HE = wo_hbm.shape[0]
    n_mem, n_late = mem0_hbm.shape[0], S // seg * _LATE
    pl.run_scoped(
        functools.partial(_mixer, x_hbm, wq_hbm, wk_hbm, wv_hbm, w1_hbm, w2_hbm, w3_hbm,
                          w4_hbm, *shared, seg),
        pltpu.VMEM((7, D // 4, D // 2), _U32),
        pltpu.VMEM((7, D // 4, D // 2), _U32),
        pltpu.VMEM((2, D // 2, _FC), _U32),
        pltpu.VMEM((2, _FC // 2, D), _U32),
        pltpu.VMEM((49, S // 8, D // 4), _U32),
        pltpu.VMEM((2, 3, _RD * HE // 256, 128), _U32),
        pltpu.VMEM((D // 128, S + 2 * _PAD, 128), _F32),
        pltpu.VMEM((2, 7, _TM // 4, D // 2), _U32),
        pltpu.VMEM((7, _TM // 4, D // 2), _U32),
        pltpu.VMEM((D // 128, _TM, 128), _F32),
        pltpu.VMEM((D // 128, _TM, 128), _F32),
        pltpu.VMEM((D // 128, _TM + _PAD, 128), _F32),
        pltpu.SMEM((1,), jnp.int32),
        pltpu.SemaphoreType.DMA((S // _TM,)),
        pltpu.SemaphoreType.DMA((4,)),
        pltpu.SemaphoreType.DMA((2, 2)),
        pltpu.SemaphoreType.DMA((2, 3)))
    pl.run_scoped(
        functools.partial(_memory, out_hbm, mem0_hbm, wo_hbm, *shared, seg),
        pltpu.VMEM((HE // 128, D // 2, 128), _U32),
        pltpu.VMEM((3 * HE // 256, 2, n_late // 2, 128), _U32),
        pltpu.VMEM((4, 2 * _LATE, HE), _F32),
        pltpu.VMEM((21, n_late // 2, HE // 4), _F32),
        pltpu.VMEM((2, D // 128, n_late // 2, 128), _F32),
        pltpu.VMEM((2, 2, (n_mem + seg - _LATE) // 2, HE // 2), _U32),
        pltpu.VMEM((2, n_late // 2, D), _BF16),
        pltpu.VMEM((n_mem, D), _BF16),
        pltpu.SemaphoreType.DMA((2,)),
        pltpu.SemaphoreType.DMA((8, 8)))


@functools.partial(jax.jit, static_argnames=("A_seg_len",))
def pallas_parallel_sum__memory_aug_recurrent_mem_tr__mixer_s_mlp__prompt_kernel(
    A_x: jax.Array,
    A_mem0: jax.Array,
    A_Wq: jax.Array,
    A_Wk: jax.Array,
    A_Wv: jax.Array,
    A_Wo: jax.Array,
    A_seg_len: int,
    B_x: jax.Array,
    B_w1: jax.Array,
    B_w2: jax.Array,
    B_w3: jax.Array,
    B_w4: jax.Array,
):
    del B_x
    B, S, D = A_x.shape
    _, H, E = A_Wq.shape
    M = A_mem0.shape[1]
    seg = int(A_seg_len)
    assert (B, S, D, H, E, M, seg, B_w3.shape[1]) == (1, 2048, 1024, 32, 128, 8, 32, 3584)

    hbm = pl.BlockSpec(memory_space=pltpu.HBM)
    out = pl.pallas_call(
        functools.partial(_kernel, seg=seg),
        out_shape=jax.ShapeDtypeStruct((S, D), A_x.dtype),
        in_specs=[hbm] * 10,
        out_specs=hbm,
        scratch_shapes=[
            pltpu.VMEM((S, D), _BF16),
            pltpu.VMEM((4 * H, D // 2, E), _U32),
            pltpu.VMEM((21, S // seg * _LATE // 4, D // 4), _U32),
            pltpu.VMEM((D // 128, S + _PAD, 128), _F32),
            pltpu.VMEM((7, 4, S // 4, D // 4), _F32),
            pltpu.VMEM((49, D // 8, 128), _U32),
            pltpu.VMEM((49, D // 8, 128), _U32),
        ],
        compiler_params=pltpu.CompilerParams(vmem_limit_bytes=126 * 1024 * 1024),
    )(A_x.reshape(S, D), A_mem0.reshape(M, D),
      A_Wq.reshape(D * H, E), A_Wk.reshape(D * H, E), A_Wv.reshape(D * H, E),
      A_Wo.reshape(H * E, D), B_w1, B_w2, B_w3, B_w4)
    return out.reshape(B, S, D)
```

```python
import functools

import jax
import jax.numpy as jnp
import numpy as np
from jax import lax
import jax.experimental.pallas as pl
import jax.experimental.pallas.tpu as pltpu

_F32 = jnp.float32
_BF16 = jnp.bfloat16
_U32 = jnp.uint32

_EPS = 1e-5
_LOG2E = float(np.log2(np.e))
_TM = 256
_SM = 64
_FC = 512
_RD = 160
_HG = 4
_LATE = 8
_PAD = 8


def _dot(a, b):
    return lax.dot_general(a, b, (((1,), (0,)), ((), ())), preferred_element_type=_F32)


def _dot_nt(a, b):
    return lax.dot_general(a, b, (((1,), (1,)), ((), ())), preferred_element_type=_F32)


def _ds(start, size, align):
    return pl.ds(start if isinstance(start, int) else pl.multiple_of(start, align), size)


def _pack(x):
    return pltpu.bitcast(x.astype(_BF16), _U32)


def _unpack(w):
    return pltpu.bitcast(w, _BF16)


def _pair(even, odd):
    return pltpu.pack_elementwise([even, odd], packed_dtype=_BF16)


def _split(w):
    return (pltpu.bitcast(lax.shift_left(w, np.uint32(16)), _F32),
            pltpu.bitcast(lax.bitwise_and(w, np.uint32(0xFFFF0000)), _F32))


def _get(ref, rows):
    return jnp.concatenate([ref[k, rows, :] for k in range(ref.shape[0])], axis=1)


def _put(ref, rows, c0, x):
    for c in range(0, x.shape[1], 128):
        ref[(c0 + c) // 128, rows, :] = lax.slice_in_dim(x, c, c + 128, axis=1)


def _wo_slab(heads, m, j):
    return 3 * heads + 16 * (j % 4 // 2) + 4 * m + 2 * (j % 2) + j // 4


def _gelu(hx):
    c0 = 2.0 * float(np.sqrt(2.0 / np.pi))
    c1 = 4.0 * 0.044715 * c0
    inner = lax.mul(hx, lax.add(np.float32(c0), lax.mul(np.float32(c1), lax.mul(hx, hx))))
    return lax.add(hx, lax.mul(hx, lax.tanh(inner)))


def _layernorm_twice(load):
    m = jnp.mean(load(0), axis=-1, keepdims=True)
    c = load(1) - m
    mu = jnp.mean(c, axis=-1, keepdims=True)
    v = jnp.mean(c * c, axis=-1, keepdims=True)
    r = lax.rsqrt(v + _EPS)
    r2 = (0.5 * r) * lax.rsqrt((r * r) * jnp.maximum(v - mu * mu, 0.0) + _EPS)
    c = load(2) - m
    return c * r, (c - mu) * r2


def _zero_bits(ref):
    return jnp.where(jnp.abs(ref[:16, :128].astype(_F32)[:8]) < 0.0, 1, 0).astype(_U32)


def _after(x, z):
    w = pltpu.bitcast(x, _U32)
    for axis in range(2):
        if w.shape[axis] > z.shape[axis]:
            z = lax.concatenate([z] * (w.shape[axis] // z.shape[axis]), axis)
    return pltpu.bitcast(lax.bitwise_or(w, z), x.dtype)


def _mark(v, zero, r=0):
    return lax.bitwise_and(pltpu.bitcast(lax.slice(v, (r, 0), (r + 8, 128)), _U32), zero)


def _any(words):
    while len(words) > 1:
        words = [functools.reduce(lax.bitwise_or, words[k:k + 2]) for k in range(0, len(words), 2)]
    return words[0]


def _spread(jobs, marks, lo=0.0, hi=1.0, prev=None):
    marks = marks[int(lo * len(marks)):int(hi * len(marks))]
    for k, job in enumerate(jobs):
        z = marks[k * len(marks) // len(jobs)]
        prev = job(z if prev is None else lax.bitwise_or(z, prev))
    return prev


_LHS_TERMS = ((0, 1, 3), (2, 1, 3), (0, 0, 0), (3, 0, 3), (0, 1, 1), (2, -1, 0), (1, -1, 3))
_RHS_TERMS = ((0, 1, 3), (0, 0, 0), (1, -1, 3), (2, -1, 0), (3, 0, 3), (0, 1, 1), (2, 1, 3))
_ORDER = (0, 1, 3, 5, 6, 2, 4)


_MIXING = (0, 5, 6)


class _Quad:
    def __init__(self, blocks):
        self.blocks = list(blocks)


def _add(a, b):
    return _Quad(map(lax.add, a.blocks, b.blocks)) if isinstance(a, _Quad) else lax.add(a, b)


def _sub(a, b):
    return _Quad(map(lax.sub, a.blocks, b.blocks)) if isinstance(a, _Quad) else lax.sub(a, b)


def _term(terms, get, p):
    a, sign, b = terms[p]
    return get(a) if sign == 0 else (_add if sign > 0 else _sub)(get(a), get(b))


def _operands(terms, quadrants):
    return [_term(terms, quadrants.__getitem__, p) for p in range(7)]


def _block(n, k):
    return 2 * (n // 2) + k // 2, 2 * (n % 2) + k % 2


def _operands7(terms, get, p):
    outer = _term(terms, lambda n: _Quad(get(*_block(n, k)) for k in range(4)), p)
    return _operands(terms, outer.blocks)


def _combine(m):
    m1, m2, m3, m4, m5, m6, m7 = m
    return (m1 + m4) + (m7 - m5), m3 + m5, m2 + m4, (m1 - m2) + (m3 + m6)


def _strassen(prod, done):
    m1, m2 = prod(0), prod(1)
    c22 = _sub(m1, m2)
    m4 = prod(3)
    done(2, _add(m2, m4))
    c11 = _add(m1, m4)
    c22 = _add(prod(5), c22)
    c11 = _add(prod(6), c11)
    m3 = prod(2)
    done(3, _add(c22, m3))
    m5 = prod(4)
    done(0, _sub(c11, m5))
    done(1, _add(m3, m5))
    return m1, m2, m4, c22, c11, m3, m5


def _strassen49(prod, done):
    seen = []

    def outer(p):
        out = [None] * 4
        m = _strassen(lambda k: prod(7 * p + k), out.__setitem__)
        seen.extend(m[k] for k in (0, 1, 3, 4))
        return _Quad(out)

    def finish(n, quad):
        for k, v in enumerate(quad.blocks):
            done(*_block(n, k), v)

    _strassen(outer, finish)
    return seen


def _halves(z):
    shift, high = lax.bitwise_or(z, np.uint32(16)), lax.bitwise_or(z, np.uint32(0xFFFF0000))
    return (lambda w: pltpu.bitcast(lax.shift_left(w, shift), _F32),
            lambda w: pltpu.bitcast(lax.bitwise_and(w, high), _F32))


def _fill_jobs(b_v, word, slots=tuple(zip(_ORDER, _ORDER))):
    def job(n, p, k, z):
        load = functools.cache(lambda r, c: word(r, c, k))
        even, odd = (_operands7(_RHS_TERMS, lambda r, c: half(load(r, c)), p) for half in _halves(z))
        for j in range(7):
            b_v[7 * n + j, pl.ds(k, 8), :] = _pair(even[j], odd[j])

    return [functools.partial(job, n, p, k) for n, p in slots for k in range(0, b_v.shape[1], 8)]


def _mixer(x_hbm, wq_hbm, wk_hbm, wv_hbm, w1_hbm, w2_hbm, w3_hbm, w4_hbm,
           x_v, wa_v, a_v, xn_v, ffn_v, b0_v, b1_v, seg,
           w1_v, w2_v, w3_v, w4_v, f_v, stage_v, h_v, y_v, g_v, t0_v, t1_v, t2_v, nil_s,
           sem_x, sem_w, sem_f, sem_s):
    S, D = x_v.shape
    H, E = wa_v.shape[0] // 4, wa_v.shape[2]
    dh, dq, th, tq = D // 2, D // 4, _TM // 2, _TM // 4
    nblk = S // _TM
    nfc = w3_hbm.shape[1] // _FC
    corners = [(r, c) for r in (0, th) for c in (0, dh)]
    tiles = [(r, c) for r in range(0, th, _SM) for c in range(0, dh, 128)]

    def x_copy(i):
        rows = pl.ds(i * _TM, _TM)
        return pltpu.make_async_copy(x_hbm.at[rows], x_v.at[rows], sem_x.at[i])

    def w3_copy(c):
        src = w3_hbm.bitcast(_U32).at[:, _ds(c * _FC, _FC, _FC)]
        return pltpu.make_async_copy(src, w3_v.at[c % 2], sem_f.at[c % 2, 0])

    def w4_copy(c):
        src = w4_hbm.bitcast(_U32).at[_ds(c * _FC // 2, _FC // 2, _FC // 2)]
        return pltpu.make_async_copy(src, w4_v.at[c % 2], sem_f.at[c % 2, 1])

    def retile_row(c):
        return min(c * _RD, D - _RD) if isinstance(c, int) else jnp.minimum(c * _RD, D - _RD)

    def stage_copy(t, c):
        src = (wq_hbm, wk_hbm, wv_hbm)[t].bitcast(_U32)
        rows = _ds(retile_row(c) * H // 2, _RD * H // 2, 8 * H)
        return pltpu.make_async_copy(src.at[rows], stage_v.at[c % 2, t], sem_s.at[c % 2, t])

    w1_copies = [pltpu.make_async_copy(w1_hbm.bitcast(_U32).at[:, pl.ds(k * dh, dh)], w3_v.at[k],
                                       sem_w.at[k]) for k in range(2)]
    w2_copies = [pltpu.make_async_copy(w2_hbm.bitcast(_U32).at[pl.ds(k * dq, dq)], w4_v.at[k],
                                       sem_w.at[2 + k]) for k in range(2)]

    nil_s[0] = 0
    x_copy(0).start()
    x_copy(1).start()
    w1_copies[0].start()
    for r in (0, _PAD + S):
        _put(h_v, pl.ds(r, _PAD), 0, jnp.zeros((_PAD, D), _F32))
    x_copy(0).wait()
    zero = _zero_bits(x_v)

    def mark(v, r=0):
        return _mark(v, zero, r)

    def norm(rows, z):
        nil = nil_s[0]

        def load(k):
            w = [_pack(x_v[_ds(r + 16 * k * nil, 16, 16), :]) for r in rows]
            return jnp.concatenate([h for v in w for h in _split(v if k else _after(v, z))], axis=0)

        xn, y = _layernorm_twice(load)
        for k, r in enumerate(rows):
            for odd in range(2):
                _put(xn_v, pl.ds(r + odd, 8, stride=2), 0, xn[16 * k + 8 * odd:16 * k + 8 * odd + 8])
        return y

    def norm_jobs(i):
        def job(r, z):
            y = norm((i * _TM + r, i * _TM + th + r), z)
            even, odd = (_operands(_LHS_TERMS, [y[k + a:k + a + 8, c:c + dh]
                                                for a in (0, 16) for c in (0, dh)]) for k in (0, 8))
            for p in range(7):
                y_v[i % 2, p, pl.ds(r // 2, 8), :] = _pair(even[p], odd[p])
            return functools.reduce(jnp.bitwise_or, [mark(y, k) for k in range(0, 32, 8)])

        return [functools.partial(job, r) for r in range(0, th, 16)]

    def shift_jobs(i, combine):
        def job(r0, c0, z):
            def load(r, c, odd):
                shift = (-1, 1, -2, 2)[(c + c0) // dq]
                rows = pl.ds(i * _TM + _PAD + r + r0 + shift + odd, _SM // 2, stride=2)
                return _after(h_v[(c + c0) // 128, rows, :], z)

            even, odd = (combine([load(r, c, k) for r, c in corners]) for k in range(2))
            for p in range(len(even)):
                g_v[p, pl.ds(r0 // 2, _SM // 2), pl.ds(c0, 128)] = _pair(even[p], odd[p])

        return [functools.partial(job, r0, c0) for r0, c0 in tiles]

    def weight_jobs(w_v, word):
        def job(k, c, z):
            quads = [word(r, q, k, c) for r in range(2) for q in range(2)]
            even, odd = (_operands(_RHS_TERMS, [half(w) for w in quads]) for half in _halves(z))
            for p in (0, 2, 3, 5, 6):
                w_v[p, pl.ds(k, 8), pl.ds(c, 128)] = _pair(even[p], odd[p])
            w_v[1, pl.ds(k, 8), pl.ds(c, 128)] = quads[0]
            w_v[4, pl.ds(k, 8), pl.ds(c, 128)] = quads[3]

        return [functools.partial(job, k, c) for c in range(0, dh, 128) for k in range(0, dq, 8)]

    def plain(lhs, rhs, put, c0, c1):
        marks = []
        for c in range(c0, c1, 128):
            for r0 in range(0, th, _SM):
                for q in (2, 0):
                    y = jnp.concatenate([_unpack(lhs[q + n, pl.ds(r0 // 2, _SM // 2), :])
                                         for n in range(2)], axis=1)
                    v = _dot(y, _unpack(rhs(c)))
                    put(q // 2 * th + r0, c, v)
                    marks.append(mark(v))
        return marks

    def fast(lhs, w_v, put):
        marks = []
        for r0, c0 in tiles:
            marks += [mark(v) for v in _strassen(
                lambda p: _dot(_unpack(lhs[p, pl.ds(r0 // 2, _SM // 2), :]),
                               _unpack(w_v[p, :, pl.ds(c0, 128)])),
                lambda q, v: put(corners[q][0] + r0, corners[q][1] + c0, v))]
        return marks

    def put_h(i):
        return lambda r, c, v: _put(h_v, pl.ds(_PAD + i * _TM + r, _SM), c, _gelu(v))

    def put_x1(i):
        held = {}

        def put(r, c, v):
            v = v + xn_v[c // 128, pl.ds(i * _TM + r, _SM), :]
            (t0_v, t1_v)[i % 2][c // 128, pl.ds(r, _SM), :] = v
            quadrant, key = 2 * (r // th) + c // dh, (r % th, c % dh)
            held[key, quadrant] = v
            seeds = {0: [(6, v)], 1: [(2, v)], 2: [(1, v)], 3: []}[quadrant]
            if quadrant and all((key, n) in held for n in (1, 2, 3)):
                seeds.append((5, held[key, 3] + (held[key, 2] - held[key, 1])))
            for p, w in seeds:
                ffn_v[p, 2 * (r % th // tq) + c % dh // dq, pl.ds(i * tq + r % tq, _SM),
                      pl.ds(c % dq, 128)] = w

        return put

    def ffn_norm_jobs(i):
        t_v, nil = (t0_v, t1_v)[i % 2], nil_s[0]

        def mean(parts):
            return jnp.sum(functools.reduce(jnp.add, parts), axis=-1, keepdims=True) * (1.0 / D)

        def normalise(r, z):
            def load(k):
                return [t_v[c + k * nil, pl.ds(r, 32), :] for c in range(D // 128)]

            x1 = load(1)
            m = mean([_after(x1[0], z)] + x1[1:])
            inv = 0.5 * lax.rsqrt(mean([(e - m) * (e - m) for e in load(2)]) + _EPS)
            for c, e in enumerate(load(3)):
                e = (e - m) * inv
                t2_v[c, pl.ds(r, 32), :] = e
            return _any([mark(e, k) for k in range(0, 32, 8)])

        def sums(r, c, p, z):
            r0 = r // 32 * 32 + r % 32 // 16
            lo, hi = (_operands7(_LHS_TERMS, lambda a, b: _after(
                t2_v[(b * dq + c) // 128, pl.ds(a * tq + r0 + k, 8, stride=4), :], z), p)
                for k in (0, 2))
            for k in range(7):
                lo[k] = _pair(lo[k], hi[k])
                f_v[7 * p + k, pl.ds((i * tq + r) // 2, 8), pl.ds(c, 128)] = lo[k]
            return lax.bitwise_and(_any(lo), zero)

        return ([functools.partial(normalise, a * tq + r) for r in range(0, tq, 32) for a in range(4)],
                [functools.partial(sums, r, c, p)
                 for r in range(0, tq, 16) for c in range(0, dq, 128) for p in range(7)])

    def w3_jobs(c):
        return _fill_jobs(b0_v, lambda r, k, j: w3_v[
            c % 2, pl.ds(r * dq // 2 + j, 8), pl.ds(k * 128, 128)])

    def w4_jobs(c):
        return _fill_jobs(b1_v, lambda r, k, j: w4_v[
            c % 2, pl.ds(r * 64 + j % 64, 8), pl.ds(k * dq + j // 64 * 128, 128)])

    def fast_lhs(quadrants):
        return _operands(_LHS_TERMS, quadrants)

    y0 = norm(range(0, _TM, 16), zero)
    for r in range(0, _TM, 16):
        for k in range(2):
            y_v[0, 2 * (r // th) + k, pl.ds(r % th // 2, 8), :] = _pair(
                y0[r:r + 8, k * dh:(k + 1) * dh], y0[r + 8:r + 16, k * dh:(k + 1) * dh])

    x_copy(1).wait()
    w1_copies[0].wait()
    w1_copies[1].start()
    marks = plain(y_v.at[0], lambda c: w3_v[0, :, pl.ds(c, 128)], put_h(0), 0, dh)
    jobs = norm_jobs(1)
    _spread(jobs[:5], marks, 0, 0.75)
    w1_copies[1].wait()
    x_copy(2).start()
    for cp in w2_copies:
        cp.start()
    x_copy(3).start()
    marks = plain(y_v.at[0], lambda c: w3_v[1, :, pl.ds(c - dh, 128)], put_h(0), dh, D)
    _spread(weight_jobs(w1_v, lambda r, q, k, c: w3_v[q, pl.ds(r * dq + k, 8), pl.ds(c, 128)]), marks)
    _spread(jobs[5:], marks, 0, 0.75)

    x_copy(2).wait()
    for k in range(4, nblk):
        x_copy(k).start()
    marks = fast(y_v.at[1], w1_v, put_h(1))
    _spread(shift_jobs(0, list), marks, 0.1, 0.9)
    _spread(norm_jobs(2), marks, 0, 0.8)
    for cp in w2_copies:
        cp.wait()
    x_copy(3).wait()
    marks = plain(g_v, lambda c: jnp.concatenate(
        [w4_v[n, :, pl.ds(c, 128)] for n in range(2)], axis=0), put_x1(0), 0, D)
    _spread(weight_jobs(w2_v, lambda r, q, k, c: w4_v[r, pl.ds(k, 8), pl.ds(q * dh + c, 128)]), marks)

    for k in range(4, nblk):
        x_copy(k).wait()
    w3_copy(0).start()
    w3_copy(1).start()
    w4_copy(0).start()
    for t in range(3):
        stage_copy(t, 0).start()
    prev = None
    for i in range(2, nblk + 1):
        if i == nblk - 1:
            w3_copy(0).wait()
        marks = []
        if i < nblk:
            marks += fast(y_v.at[i % 2], w1_v, put_h(i))
            _spread(shift_jobs(i - 1, fast_lhs), marks, 0.1, 0.9)
        else:
            _spread(shift_jobs(i - 1, fast_lhs), [zero])
        marks += fast(g_v, w2_v, put_x1(i - 1))
        if i + 1 == nblk:
            _spread(w3_jobs(0), marks, 0.02, 0.8)
        normalise, sums = ffn_norm_jobs(i - 2)
        if i + 1 < nblk:
            jobs = [job for pair in zip(normalise, norm_jobs(i + 1)) for job in pair]
            _spread(jobs, marks, 0.02, 0.8, prev)
        else:
            _spread(normalise, marks, 0, 0.55, prev)
        prev = _spread(sums, marks, 0.6, 0.99)
    for jobs in ffn_norm_jobs(nblk - 1):
        for job in jobs:
            job(zero)

    def late_jobs(i):
        def job(r, c, n, z):
            def rows(a, k):
                return _ds(i * _TM + (4 * r + 2 * k + a % 2 + 1) * seg + (a // 2 - 2) * _LATE,
                           _LATE, _LATE)

            lo, hi = (_operands7(_LHS_TERMS, lambda a, b: _after(
                xn_v[(b * dq + c) // 128, rows(a, k), :], z), _MIXING[n]) for k in range(2))
            for k in range(7):
                a_v[7 * n + k, _ds((2 * i + r) * _LATE, _LATE, _LATE), pl.ds(c, 128)] = _pack(
                    jnp.concatenate([lo[k], hi[k]], axis=0))

        return [functools.partial(job, r, c, n)
                for r in range(2) for c in range(0, dq, 128) for n in range(3)]

    def hidden_rows(k, r, n):
        return pl.ds(k * S // 8 + r // 2, n // 2)

    def ffn(c, _):
        @pl.when(c + 1 < nfc)
        def _():
            for t in range(3):
                stage_copy(t, c + 1).start()
            w4_copy(c + 1).start()
            w3_copy(c + 1).wait()

        @pl.when(c + 2 < nfc)
        def _():
            w3_copy(c + 2).start()

        w4_copy(c).wait()
        for t in range(3):
            stage_copy(t, c).wait()

        sublane = lax.broadcasted_iota(jnp.int32, (8, E), 0)

        def retile(t, r, jh, odd, z):
            low = lax.bitwise_or(z, np.uint32(0xFFFF))
            w = []
            for k in range(8):
                a, b = (stage_v[c % 2, t, pl.ds((r + k) * H + half + 8 * jh, 8), :]
                        for half in (0, H // 2))
                w.append(((a >> 16) | (b & ~low)) if odd else ((a & low) | (b << 16)))
            for d in (4, 2, 1):
                keep = (sublane & d) == 0
                for k in (k for k in range(8) if not k & d):
                    w[k], w[k + d] = (jnp.where(keep, w[k], pltpu.roll(w[k + d], d, 0)),
                                      jnp.where(keep, pltpu.roll(w[k], 8 - d, 0), w[k + d]))
            rows = _ds(retile_row(c) // 2 + r, 8, 8)
            for j in range(8):
                wa_v[6 * (8 * jh + j) + 3 * odd + t, rows, :] = w[j]

        def activate(r0, hid, marks):
            def act(a, b, z):
                hid[a, b] = _gelu(_after(hid[a, b], z))

            _spread([functools.partial(act, a, b) for a in range(2) for b in range(4)],
                    marks, 0.03, 0.9)
            for p in _ORDER:
                for r in range(0, tq, 16):
                    r1 = r // 32 * 32 + r % 32 // 2
                    even, odd = (_operands7(_LHS_TERMS, lambda a, b: lax.slice_in_dim(
                        hid[a, b], k, k + 8), p)
                                 for k in (r1, r1 + 16))
                    for k in range(7):
                        h_v[p, hidden_rows(k, r0 + r, 16), :] = pltpu.bitcast(
                            _pair(even[k], odd[k]), _F32)

        marks, pending, fills = [], None, w4_jobs(c)
        for r0 in range(0, S // 4, tq):
            hid = {}
            seen = [mark(v) for v in _strassen49(
                lambda p: _dot(_unpack(f_v[p, pl.ds(r0 // 2, tq // 2), :]), _unpack(b0_v[p])),
                lambda a, b, v: hid.__setitem__((a, b), v if a < 2 else _gelu(v)))]
            if pending:
                activate(*pending, seen)
            n = len(fills) // 7
            _spread(fills[r0 // tq * n:][:n], seen)
            pending = (r0, hid)
            marks += seen
        retiles = [functools.partial(retile, t, r, jh, odd) for t in range(3)
                   for r in range(0, _RD // 2, 8) for jh in range(H // 16) for odd in range(2)]
        _spread(retiles[:18], marks, 0.004, 0.98)

        marks = []
        for r0 in range(0, S // 4, tq):
            for j in range(2):
                for p in range(7):
                    def done(q, v):
                        idx = (p, q, pl.ds(r0, tq), pl.ds(j * 128, 128))
                        old = ffn_v[idx]
                        ffn_v[idx] = lax.add(v, jnp.where(c > 0, old, 0.0) if p in (0, 3, 4) else old)

                    marks += [mark(v) for v in _strassen(
                        lambda k: _dot(_unpack(h_v[p, hidden_rows(k, r0, tq), :]),
                                       _unpack(b1_v[7 * p + k, pl.ds(j * 64, 64), :])), done)]
            if pending:
                activate(*pending, marks)
                pending = None
        _spread(w3_jobs(jnp.minimum(c + 1, nfc - 1)), marks, 0.2, 0.98)
        _spread(retiles[18:], marks, 0.25, 0.97)
        _spread(late_jobs(c) + late_jobs(c + 1), marks, 0.3, 0.95)
        return 0

    lax.fori_loop(0, nfc, ffn, 0)


def _memory(out_hbm, mem0_hbm, wo_hbm, x_v, wa_v, a_v, xn_v, ffn_v, b0_v, b1_v, seg,
            wo_v, pre_v, post_v, a2_v, acc_v, att_v, fin_v, mem0_v, sem, sem_o):
    S, D = x_v.shape
    H, E = wa_v.shape[0] // 4, wa_v.shape[2]
    dh, dq = D // 2, D // 4
    n_mem, n_seg, early = mem0_hbm.shape[0], S // seg, seg - 2 * _LATE
    L = n_mem + seg
    mem0_copy = pltpu.make_async_copy(mem0_hbm, mem0_v, sem.at[1])
    mem0_copy.start()

    def wo_copies(q, raw=0):
        copies = []
        for k in range(8):
            m, j = 2 * (q % 2) + k // 4, 4 * (k % 2) + 2 * (q // 2) + k % 4 // 2
            src = wo_hbm.bitcast(_U32).at[_ds(m * dh, dh, dh), _ds(j * 128, 128, 128)]
            dst = wo_v.at[8 * q + k] if raw else wa_v.at[3 * H + 8 * q + k]
            copies.append(pltpu.make_async_copy(src, dst, sem_o.at[4 * raw + q, k]))
        return copies

    zero = _zero_bits(x_v)

    def fill_jobs(b_v, w_v, n):
        return _fill_jobs(b_v, lambda r, c, k: w_v[
            n + 2 * (c % 2) + c // 2, pl.ds(r * dq // 2 + k, 8), :], tuple(enumerate(_MIXING)))

    def loop_form_jobs(slabs):
        def job(n, k, z):
            quads = [wa_v[n + c, pl.ds(r * dq + k, 16), :] for r in range(2) for c in range(2)]
            even, odd = ([half(w) for w in quads] for half in _halves(jnp.tile(z, (2, 1))))
            wa_v[n + 1, pl.ds(k, 16), :] = _pair(even[1] - even[3], odd[1] - odd[3])
            wa_v[n, pl.ds(dq + k, 16), :] = _pair(even[2] - even[0], odd[2] - odd[0])

        return [functools.partial(job, n, k) for n in slabs for k in range(0, dq, 16)]

    def project(lhs, done, jobs):
        for j in range(4):
            b_v, marks = (b0_v, b1_v)[j % 2], []
            for r0 in range(0, n_seg * _LATE // 2, _SM):
                m = []
                for n in range(3):
                    m.append([None] * 4)
                    seen = _strassen(lambda k: _dot(lhs(j, 7 * n + k, r0), _unpack(b_v[7 * n + k])),
                                     m[n].__setitem__)
                    marks += [_mark(seen[k], zero) for k in (0, 1, 3, 4)]
                for k in range(4):
                    done(j, k, r0, lax.add(m[0][k], m[2][k]), lax.add(m[0][k], m[1][k]))
            for some in jobs(j, (b1_v, b0_v)[j % 2]):
                _spread(some, marks[:-3])

    def pre(i):
        def done(j, k, r0, c11, c22):
            pre_v[8 * i + 2 * j + k % 2, k // 2, pl.ds(r0, _SM), :] = _pair(c11, c22)

        def jobs(j, b_v):
            n = 16 * i + 4 * j
            if not isinstance(i, int):
                return [fill_jobs(b_v, wa_v, n + 4),
                        loop_form_jobs((n, n + 2, 3 * H + 8 * (i - 1) + 2 * j))]
            return [fill_jobs(b_v, wa_v, n + 4) if n + 4 < 3 * H else fill_jobs(b_v, wo_v, 0),
                    loop_form_jobs((n, n + 2))]

        project(lambda j, p, r0: _unpack(a_v[p, pl.ds(r0 // 2, _SM // 2), :]), done, jobs)

    for cp in wo_copies(0):
        cp.start()
    _spread(fill_jobs(b0_v, wa_v, 0), [zero])
    pre(0)

    for cp in wo_copies(0, raw=1):
        cp.start()

    @pl.loop(1, 5)
    def _(i):
        @pl.when(i < 4)
        def _():
            for cp in wo_copies(i):
                cp.start()

        for cp in wo_copies(i - 1):
            cp.wait()
        pre(i)

    for cp in wo_copies(0, raw=1):
        cp.wait()
    pre(5)
    rest_of_wo = [cp for q in range(1, 4) for cp in wo_copies(q, raw=1)]
    for cp in rest_of_wo:
        cp.start()

    row = lax.broadcasted_iota(jnp.int32, (L, L), 0)
    col = lax.broadcasted_iota(jnp.int32, (L, L), 1)
    mask = (row < n_mem) | (row >= col)
    scale = float(E) ** -0.5

    def mixer_out(i, r):
        rows = _ds((i // 2) * (_TM // 4) + (r % 2) * seg, seg, seg)
        cols = [None] * 4
        for b in range(2):
            c = _combine([ffn_v[p, 2 * (r // 2) + b, rows, :] for p in range(7)])
            for k in range(2):
                cols[2 * k + b] = jnp.where(i % 2 == 0, c[k], c[2 + k])
        return jnp.concatenate(cols, axis=1)

    def forms(v):
        n = L - 2 * _LATE
        first = jnp.concatenate([v[:n], v[n + _LATE:]], axis=0)
        second = v[:n + _LATE]
        return ((first[:, :dh] + first[:, dh:], first[:, dh:]),
                (second[:, :dh], second[:, :dh] + second[:, dh:]))

    def assemble(p1, q1, p2, q2, c11, c22):
        n = L - 2 * _LATE
        y1, y2 = p1 + q1, p2 + q2
        return (jnp.concatenate([y1[:n], (q1[n:] - q2[n:]) + c11, y1[n:]], axis=0),
                jnp.concatenate([y2, (p2[n:] - p1[n:]) + c22], axis=0))

    def step(i, r, mem):
        rows = _ds((4 * i + r) * seg, seg, seg)
        late = _ds((2 * i + r // 2) * _LATE, _LATE, _LATE)
        h = [[v.astype(_BF16) for v in f]
             for f in forms(jnp.concatenate([mem, _get(xn_v, rows)], axis=0))]
        groups = H // _HG
        qkv, sc, out = {}, {}, {}

        def project_rows(g):
            slabs = range(3 * _HG * g, 3 * _HG * (g + 1))
            y = {}
            for c, k in ((1, 0), (0, 1), (0, 0), (1, 1)):
                y[c, k] = _dot(h[c][k], jnp.concatenate(
                    [_unpack(wa_v[n, pl.ds(k * dq, dq), :]) for n in slabs[c::2]], axis=1))
            c11, c22 = _split(jnp.concatenate(
                [pre_v[n // 2, r % 2, late, :] for n in slabs[::2]], axis=1))
            qkv[g] = assemble(y[0, 0], y[0, 1], y[1, 0], y[1, 1], c11, c22)

        def part(g, n, t):
            k, c = divmod(3 * n + t, 2)
            return qkv[g][c][:, k * E:(k + 1) * E]

        def scores(g):
            sc[g] = [_dot_nt(part(g, n, 0), part(g, n, 1).astype(_BF16)) for n in range(_HG)]

        def attend(g):
            for n in range(_HG):
                z = jnp.where(mask, sc[g][n] * (scale * _LOG2E), -1e9 * _LOG2E)
                e = jnp.exp2(z - jnp.max(z, axis=-1, keepdims=True))
                total = jnp.sum(e, axis=-1, keepdims=True)
                inv = pl.reciprocal(total, approx=True)
                inv = inv * (2.0 - total * inv)
                out[g, n] = _dot(e * inv, part(g, n, 2).astype(_BF16))
                post_v[r, :, pl.ds((g * _HG + n) * E, E)] = out[g, n][L - 2 * _LATE:]
            if g % 2:
                f = forms(jnp.concatenate([out[k, n] for k in (g - 1, g) for n in range(_HG)], axis=1))
                for c in range(2):
                    for k in range(2):
                        att_v[c, k, :, pl.ds(g // 2 * dh, dh)] = _pack(f[c][k])

        def project_out(m):
            for c in range(2):
                for j in range(4):
                    for k in range(2):
                        d = _dot(_unpack(att_v[c, k, :, pl.ds(m * dh, dh)]),
                                 _unpack(wa_v[_wo_slab(H, m, 4 * c + j), pl.ds(k * dq, dq), :]))
                        o[c, k, j] = d + o[c, k, j] if m else d

        o = {}
        for t in range(groups + 4):
            if t < groups:
                project_rows(t)
            else:
                project_out(t - groups)
            if 0 <= t - 2 < groups:
                attend(t - 2)
            if 0 <= t - 1 < groups:
                scores(t - 1)
        o = jnp.concatenate(assemble(*[jnp.concatenate([o[c, k, j] for j in range(4)], axis=1)
                                       for c in range(2) for k in range(2)], 0.0, 0.0), axis=1)
        y = (x_v[rows, :].astype(_F32) + mixer_out(i, r)) + o[n_mem:]
        x_v[rows, :] = y.astype(_BF16)
        _put(acc_v.at[r % 2], late, 0, y[early:early + _LATE, :dh])
        _put(acc_v.at[r % 2], late, dh, y[early + _LATE:, dh:])
        return o[:n_mem]

    def steps(i, mem):
        for r in range(4):
            mem = step(i, r, mem)
        for r in range(2):
            rows = _ds((2 * i + r) * _LATE, _LATE, _LATE)
            for m in range(H * E // D):
                for c in range(0, dq, 128):
                    for n, p in enumerate(_MIXING):
                        for k, v in enumerate(_operands7(_LHS_TERMS, lambda a, b: post_v[
                                2 * r + a % 2, pl.ds(a // 2 * _LATE, _LATE),
                                pl.ds(m * D + b * dq + c, 128)], p)):
                            a2_v[7 * n + k, rows, pl.ds(m * dq + c, 128)] = v
        for r in range(4):
            for r0, n, c0, w in ((0, early, 0, D), (early, _LATE, dh, dh), (early + _LATE, _LATE, 0, dh)):
                at = (_ds((4 * i + r) * seg + r0, n, _LATE), pl.ds(c0, w))
                pltpu.make_async_copy(x_v.at[at], out_hbm.at[at], sem.at[0]).start()
        return mem

    mem0_copy.wait()
    lax.fori_loop(0, n_seg // 4, steps, mem0_v[...].astype(_F32))

    for cp in rest_of_wo:
        cp.wait()

    @pl.loop(0, 2)
    def _(i):
        partial = {}

        def done(m, k, r0, *blocks):
            for c, v in enumerate(blocks):
                j = 4 * c + 2 * i + k % 2
                v = v + (partial.pop((c, k, r0)) if m else acc_v[k // 2, j, pl.ds(r0, _SM), :])
                if m < 3:
                    partial[c, k, r0] = v
                    continue
                for t in range(0, _SM, _LATE):
                    fin_v[k // 2, pl.ds(r0 + t, _LATE), _ds(j * 128, 128, 128)] = (
                        v[t:t + _LATE].astype(_BF16))

        project(lambda m, p, r0: a2_v[p, pl.ds(r0, _SM), pl.ds(m * dq, dq)], done,
                lambda j, b_v: [fill_jobs(b_v, wo_v, jnp.minimum(16 * i + 4 * j + 4, H - 4))])
        for s in range(n_seg):
            for c in range(2):
                cols = _ds(c * dh + i * dq, dq, dq)
                pltpu.make_async_copy(
                    fin_v.at[s % 2, pl.ds(s // 2 * _LATE, _LATE), cols],
                    out_hbm.at[pl.ds(s * seg + early + c * _LATE, _LATE), cols], sem.at[0]).start()

    pltpu.make_async_copy(x_v, out_hbm, sem.at[0]).wait()


def _kernel(x_hbm, mem0_hbm, wq_hbm, wk_hbm, wv_hbm, wo_hbm, w1_hbm, w2_hbm, w3_hbm, w4_hbm,
            out_hbm, *shared, seg):
    S, D = x_hbm.shape
    HE = wo_hbm.shape[0]
    n_mem, n_late = mem0_hbm.shape[0], S // seg * _LATE
    pl.run_scoped(
        functools.partial(_mixer, x_hbm, wq_hbm, wk_hbm, wv_hbm, w1_hbm, w2_hbm, w3_hbm,
                          w4_hbm, *shared, seg),
        pltpu.VMEM((7, D // 4, D // 2), _U32),
        pltpu.VMEM((7, D // 4, D // 2), _U32),
        pltpu.VMEM((2, D // 2, _FC), _U32),
        pltpu.VMEM((2, _FC // 2, D), _U32),
        pltpu.VMEM((49, S // 8, D // 4), _U32),
        pltpu.VMEM((2, 3, _RD * HE // 256, 128), _U32),
        pltpu.VMEM((D // 128, S + 2 * _PAD, 128), _F32),
        pltpu.VMEM((2, 7, _TM // 4, D // 2), _U32),
        pltpu.VMEM((7, _TM // 4, D // 2), _U32),
        pltpu.VMEM((D // 128, _TM, 128), _F32),
        pltpu.VMEM((D // 128, _TM, 128), _F32),
        pltpu.VMEM((D // 128, _TM + _PAD, 128), _F32),
        pltpu.SMEM((1,), jnp.int32),
        pltpu.SemaphoreType.DMA((S // _TM,)),
        pltpu.SemaphoreType.DMA((4,)),
        pltpu.SemaphoreType.DMA((2, 2)),
        pltpu.SemaphoreType.DMA((2, 3)))
    pl.run_scoped(
        functools.partial(_memory, out_hbm, mem0_hbm, wo_hbm, *shared, seg),
        pltpu.VMEM((HE // 128, D // 2, 128), _U32),
        pltpu.VMEM((3 * HE // 256, 2, n_late // 2, 128), _U32),
        pltpu.VMEM((4, 2 * _LATE, HE), _F32),
        pltpu.VMEM((21, n_late // 2, HE // 4), _F32),
        pltpu.VMEM((2, D // 128, n_late // 2, 128), _F32),
        pltpu.VMEM((2, 2, (n_mem + seg - _LATE) // 2, HE // 2), _U32),
        pltpu.VMEM((2, n_late // 2, D), _BF16),
        pltpu.VMEM((n_mem, D), _BF16),
        pltpu.SemaphoreType.DMA((2,)),
        pltpu.SemaphoreType.DMA((8, 8)))


@functools.partial(jax.jit, static_argnames=("A_seg_len",))
def pallas_parallel_sum__memory_aug_recurrent_mem_tr__mixer_s_mlp__prompt_kernel(
    A_x: jax.Array,
    A_mem0: jax.Array,
    A_Wq: jax.Array,
    A_Wk: jax.Array,
    A_Wv: jax.Array,
    A_Wo: jax.Array,
    A_seg_len: int,
    B_x: jax.Array,
    B_w1: jax.Array,
    B_w2: jax.Array,
    B_w3: jax.Array,
    B_w4: jax.Array,
):
    del B_x
    B, S, D = A_x.shape
    _, H, E = A_Wq.shape
    M = A_mem0.shape[1]
    seg = int(A_seg_len)
    assert (B, S, D, H, E, M, seg, B_w3.shape[1]) == (1, 2048, 1024, 32, 128, 8, 32, 3584)

    hbm = pl.BlockSpec(memory_space=pltpu.HBM)
    out = pl.pallas_call(
        functools.partial(_kernel, seg=seg),
        out_shape=jax.ShapeDtypeStruct((S, D), A_x.dtype),
        in_specs=[hbm] * 10,
        out_specs=hbm,
        scratch_shapes=[
            pltpu.VMEM((S, D), _BF16),
            pltpu.VMEM((4 * H, D // 2, E), _U32),
            pltpu.VMEM((21, S // seg * _LATE // 4, D // 4), _U32),
            pltpu.VMEM((D // 128, S + _PAD, 128), _F32),
            pltpu.VMEM((7, 4, S // 4, D // 4), _F32),
            pltpu.VMEM((49, D // 8, 128), _U32),
            pltpu.VMEM((49, D // 8, 128), _U32),
        ],
        compiler_params=pltpu.CompilerParams(vmem_limit_bytes=126 * 1024 * 1024),
    )(A_x.reshape(S, D), A_mem0.reshape(M, D),
      A_Wq.reshape(D * H, E), A_Wk.reshape(D * H, E), A_Wv.reshape(D * H, E),
      A_Wo.reshape(H * E, D), B_w1, B_w2, B_w3, B_w4)
    return out.reshape(B, S, D)
```
